```python
import jax
import jax.numpy as jnp

def _softmax(x, axis=-1):
    return jax.nn.softmax(x, axis=axis)

def _gelu(x):
    return jax.nn.gelu(x, approximate=True)

def _silu(x):
    return jax.nn.silu(x)

def _sigmoid(x):
    return jax.nn.sigmoid(x)

def _layernorm(x, axis=-1, eps=1e-05):
    m = jnp.mean(x, axis=axis, keepdims=True)
    v = jnp.var(x, axis=axis, keepdims=True)
    return (x - m) / jnp.sqrt(v + eps)

def _scatter_add(tgt, idx, src, axis=0):
    return tgt.at[idx].add(src)

def _segment_sum(src, seg, n):
    return jax.ops.segment_sum(src, seg, n)

class _Rng:

    def __init__(self, key):
        self._k = key

    def _next(self):
        self._k, sub = jax.random.split(self._k)
        return sub

    def normal(self, shape):
        return jax.random.normal(self._next(), shape, dtype=jnp.bfloat16)

    def randint(self, lo, hi, shape):
        return jax.random.randint(self._next(), shape, lo, hi, dtype=jnp.int32)

    def uniform(self, shape, lo=0.0, hi=1.0):
        return jax.random.uniform(self._next(), shape, jnp.bfloat16, lo, hi)

    def permutation(self, n):
        return jax.random.permutation(self._next(), n)
kernel_name = 'adaLN_cond__memory_aug_recurrent_mem_tr__glu_gated_swiglu__prompt'

def setup_inputs():
    _rng = _Rng(jax.random.key(int.from_bytes(__import__("os").urandom(4), "little")))
    _w = lambda a: (lambda t: t.astype(jnp.bfloat16) if jnp.issubdtype(t.dtype, jnp.floating) else t)(jnp.asarray(a))

    def _A_setup():
        B, S, Dm = (1, 2048, 1024)
        H, Dh = (32, 128)
        M, seg = (8, 32)
        seg = min(seg, S)
        S = S // seg * seg
        return {'x': _w((lambda *s: _rng.normal(s) * 0.05)(B, S, Dm)), 'mem0': _w((lambda *s: _rng.normal(s) * 0.05)(B, M, Dm)), 'Wq': _w((lambda *s: _rng.normal(s) * 0.05)(Dm, H, Dh) * Dm ** (-0.5)), 'Wk': _w((lambda *s: _rng.normal(s) * 0.05)(Dm, H, Dh) * Dm ** (-0.5)), 'Wv': _w((lambda *s: _rng.normal(s) * 0.05)(Dm, H, Dh) * Dm ** (-0.5)), 'Wo': _w((lambda *s: _rng.normal(s) * 0.05)(H, Dh, Dm) * (H * Dh) ** (-0.5)), 'seg_len': seg}
    _A_in = _A_setup()

    def _B_setup():
        B, S, D, F = (1, 2048, 1024, 3584)
        return {'x': _w((lambda *s: _rng.normal(s) * 0.05)(B, S, D)), 'w1': _w((lambda *s: _rng.normal(s) * 0.05)(D, F) * (2.0 / D) ** 0.5), 'w3': _w((lambda *s: _rng.normal(s) * 0.05)(D, F) * (2.0 / D) ** 0.5), 'w2': _w((lambda *s: _rng.normal(s) * 0.05)(F, D) * (2.0 / F) ** 0.5)}
    _B_in = _B_setup()
    return {'A_x': _A_in['x'], 'A_mem0': _A_in['mem0'], 'A_Wq': _A_in['Wq'], 'A_Wk': _A_in['Wk'], 'A_Wv': _A_in['Wv'], 'A_Wo': _A_in['Wo'], 'A_seg_len': _A_in['seg_len'], 'B_x': _B_in['x'], 'B_w1': _B_in['w1'], 'B_w3': _B_in['w3'], 'B_w2': _B_in['w2'], 'c': _w((lambda *s: _rng.normal(s) * 0.05)(1, 1024)), 'w_mod': _w((lambda *s: _rng.normal(s) * 0.05)(1024, 6 * 1024) * 1024 ** (-0.5))}

def reference(A_x, A_mem0, A_Wq, A_Wk, A_Wv, A_Wo, A_seg_len, B_x, B_w1, B_w3, B_w2, c, w_mod):

    def _A_ref(x, mem0, Wq, Wk, Wv, Wo, seg_len):
        B, S, Dm = x.shape
        H, Dh = (Wq.shape[1], Wq.shape[2])
        M = mem0.shape[1]
        scale = Dh ** (-0.5)
        n_seg = S // seg_len
        L = M + seg_len
        idx = jnp.arange(L)
        mask = (idx[:, None] < M) | (idx[:, None] >= idx[None, :])
        mem = mem0
        outs = []
        for s in range(n_seg):
            xs = x[:, s * seg_len:(s + 1) * seg_len, :].copy()
            h = jnp.concatenate([mem, xs], axis=1)
            q = jnp.einsum('btd,dhe->bhte', h, Wq)
            k = jnp.einsum('btd,dhe->bhte', h, Wk)
            v = jnp.einsum('btd,dhe->bhte', h, Wv)
            scores = jnp.einsum('bhqe,bhke->bhqk', q, k) * scale
            scores = jnp.where(mask[None, None], scores, -1000000000.0)
            p = _softmax(scores, axis=-1)
            o = jnp.einsum('bhqk,bhke->bhqe', p, v)
            o = jnp.einsum('bhte,hed->btd', o, Wo)
            mem = o[:, :M, :].copy()
            outs.append(o[:, M:, :])
        return jnp.concatenate(outs, axis=1)

    def _B_ref(x, w1, w3, w2):
        gate = jnp.einsum('bsd,df->bsf', x, w1)
        up = jnp.einsum('bsd,df->bsf', x, w3)
        h = _silu(gate) * up
        out = jnp.einsum('bsf,fd->bsd', h, w2)
        return out
    x = A_x
    mod = (_silu(c) @ w_mod).reshape(c.shape[0], 6, 1, -1)
    sa, ca, ga, sb, cb, gb = (mod[:, 0].copy(), mod[:, 1].copy(), mod[:, 2].copy(), mod[:, 3].copy(), mod[:, 4].copy(), mod[:, 5].copy())
    h = _layernorm(x, axis=-1) * (1 + ca) + sa
    x = x + ga * _A_ref(h, A_mem0, A_Wq, A_Wk, A_Wv, A_Wo, A_seg_len)
    h = _layernorm(x, axis=-1) * (1 + cb) + sb
    x = x + gb * _B_ref(h, B_w1, B_w3, B_w2)
    return x
```

```python
import functools

import jax
import jax.numpy as jnp
from jax import lax
import jax.experimental.pallas as pl
import jax.experimental.pallas.tpu as pltpu

F32 = jnp.float32
BF16 = jnp.bfloat16
U32 = jnp.uint32

_HG = 4
_FM = 256
_FC = 512


def _mm(a, b):
    return lax.dot_general(a, b, (((1,), (0,)), ((), ())), preferred_element_type=F32)


def _mm_nt(a, b):
    return lax.dot_general(a, b, (((1,), (1,)), ((), ())), preferred_element_type=F32)


def _ln_mod(x, scale1, shift):
    m = jnp.mean(x, axis=-1, keepdims=True)
    d = x - m
    v = jnp.mean(d * d, axis=-1, keepdims=True)
    return d * lax.rsqrt(v + 1e-5) * scale1 + shift


def _body(x_hbm, mem0_ref, wq_hbm, wk_hbm, wv_hbm, wo_hbm, w1_hbm, w3_hbm, w2_hbm, c_ref,
          wmod_hbm, out_hbm,
          xs, wmod, wqkv, wo, w1, w3, w2, mod, hbuf, obuf, x1, h2, ybuf,
          sem_x, sem_mod, sem_w, sem_o, sem_f, sem_out, *, seg, H, Dh):
    S, D = xs.shape
    M = mem0_ref.shape[0]
    L = M + seg
    n_seg = S // seg
    F = w1.shape[1]
    HP = H // 2

    def mod_cp(j):
        return pltpu.make_async_copy(wmod_hbm.at[:, pl.ds(j * 2 * D, 2 * D)],
                                     wmod.at[j], sem_mod.at[j])

    x_cp = pltpu.make_async_copy(x_hbm, xs, sem_x)
    w_hbms = (wq_hbm, wk_hbm, wv_hbm)

    def w_cp(m, hd):
        src = w_hbms[m].bitcast(U32).at[:, (hd % 2) * HP + hd // 2, :]
        return pltpu.make_async_copy(src, wqkv.at[hd, :, pl.ds(m * Dh, Dh)], sem_w.at[m * H + hd])

    wo_cp = pltpu.make_async_copy(wo_hbm.bitcast(U32), wo, sem_o)

    f_cps = [pltpu.make_async_copy(s, d, sem_f.at[i])
             for i, (s, d) in enumerate(((w1_hbm, w1), (w3_hbm, w3), (w2_hbm, w2)))]

    mod_cp(0).start()
    x_cp.start()
    for m in range(3):
        for hd in range(H):
            w_cp(m, hd).start()
    wo_cp.start()
    mod_cp(1).start()
    mod_cp(2).start()
    for cp in f_cps:
        cp.start()

    cv = c_ref[...].astype(F32)
    sc = jnp.broadcast_to(cv * jax.nn.sigmoid(cv), (8, D)).astype(BF16)

    def mod_part(j):
        mod_cp(j).wait()
        mod[:, pl.ds(j * 2 * D, 2 * D)] = _mm(sc, wmod[j])

    mod_part(0)

    for m in range(3):
        for i in range(HP):
            w_cp(m, 2 * i).wait()
            w_cp(m, 2 * i + 1).wait()

        def retile(i, carry, m=m):
            cols = pl.ds(m * Dh, Dh)
            a = wqkv[2 * i, :, cols]
            b = wqkv[2 * i + 1, :, cols]
            wqkv[2 * i, :, cols] = (a & jnp.uint32(0xFFFF)) | (b << 16)
            wqkv[2 * i + 1, :, cols] = (a >> 16) | (b & jnp.uint32(0xFFFF0000))
            return carry

        lax.fori_loop(0, HP, retile, 0)

    wo_cp.wait()
    mod_part(1)
    mod_part(2)
    x_cp.wait()

    def mod_row(j):
        return mod[0:1, pl.ds(j * D, D)]

    def seg_rows(s):
        return pl.ds(pl.multiple_of(s * seg, seg), seg)

    def h_of(s):
        return _ln_mod(xs[seg_rows(s), :].astype(F32), 1.0 + mod_row(1), mod_row(0))

    hbuf[0:M, :] = mem0_ref[...].astype(F32)
    hbuf[M:L, :] = h_of(0)
    scale = Dh ** -0.5
    NG = H // _HG

    def step(s, carry):
        row = lax.broadcasted_iota(jnp.int32, (L, L), 0)
        col = lax.broadcasted_iota(jnp.int32, (L, L), 1)
        mask = (row < M) | (row >= col)
        h = hbuf[...]

        def proj(g):
            return [_mm(h, pltpu.bitcast(wqkv[g * _HG + j], BF16)) for j in range(_HG)]

        def attend(g, qkvs):
            for j, qkv in enumerate(qkvs):
                q = qkv[:, 0:Dh]
                k = qkv[:, Dh:2 * Dh].astype(BF16)
                v = qkv[:, 2 * Dh:3 * Dh].astype(BF16)
                sco = jnp.where(mask, _mm_nt(q, k) * scale, -1e9)
                e = jnp.exp(sco - jnp.max(sco, axis=-1, keepdims=True))
                inv = 1.0 / jnp.sum(e, axis=-1, keepdims=True)
                obuf[:, pl.ds((g * _HG + j) * Dh, Dh)] = _mm(e, v) * inv

        def out_proj(g):
            kk = _HG * Dh
            return _mm(obuf[:, pl.ds(g * kk, kk)],
                       pltpu.bitcast(wo[pl.ds(g * kk // 2, kk // 2), :], BF16))

        acc = None
        pend = proj(0)
        for g in range(NG):
            nxt = proj(g + 1) if g + 1 < NG else None
            attend(g, pend)
            pend = nxt
            if g >= 1:
                part = out_proj(g - 1)
                acc = part if acc is None else acc + part
        acc = acc + out_proj(NG - 1)

        hbuf[0:M, :] = acc[0:M]
        hbuf[M:L, :] = h_of(jnp.minimum(s + 1, n_seg - 1))
        xn = xs[seg_rows(s), :].astype(F32) + mod_row(2) * acc[M:L]
        x1[seg_rows(s), :] = xn
        h2[seg_rows(s), :] = _ln_mod(xn, 1.0 + mod_row(4), mod_row(3)).astype(BF16)
        return carry

    lax.fori_loop(0, n_seg, step, 0)

    for cp in f_cps:
        cp.wait()

    def out_cp(i):
        rows = pl.ds(pl.multiple_of(i * _FM, _FM), _FM)
        return pltpu.make_async_copy(ybuf.at[rows], out_hbm.at[rows], sem_out.at[i])

    def ffn(i, carry):
        rows = pl.ds(pl.multiple_of(i * _FM, _FM), _FM)
        hb = h2[rows, :]
        acc = None
        for f in range(F // _FC):
            cols = pl.ds(f * _FC, _FC)
            gate = _mm(hb, w1[:, cols])
            up = _mm(hb, w3[:, cols])
            act = (gate * jax.nn.sigmoid(gate) * up).astype(BF16)
            part = _mm(act, w2[cols, :])
            acc = part if acc is None else acc + part
        ybuf[rows, :] = (x1[rows, :] + mod_row(5) * acc).astype(ybuf.dtype)
        out_cp(i).start()
        return carry

    lax.fori_loop(0, S // _FM, ffn, 0)
    for i in range(S // _FM):
        out_cp(i).wait()


@functools.partial(jax.jit, static_argnames=("A_seg_len",))
def pallas_adaLN_cond__memory_aug_recurrent_mem_tr__glu_gated_swiglu__prompt_kernel(
        A_x, A_mem0, A_Wq, A_Wk, A_Wv, A_Wo, A_seg_len, B_x, B_w1, B_w3, B_w2, c, w_mod):
    del B_x
    B, S, D = A_x.shape
    _, H, Dh = A_Wq.shape
    M = A_mem0.shape[1]
    F = B_w1.shape[1]
    seg = int(A_seg_len)
    assert B == 1 and S % seg == 0 and S % _FM == 0 and F % _FC == 0
    L = M + seg
    hbm = pl.BlockSpec(memory_space=pl.ANY)
    vmem = pl.BlockSpec(memory_space=pltpu.VMEM)
    dma = pltpu.SemaphoreType.DMA
    out = pl.pallas_call(
        functools.partial(_body, seg=seg, H=H, Dh=Dh),
        out_shape=jax.ShapeDtypeStruct((S, D), A_x.dtype),
        in_specs=[hbm, vmem, hbm, hbm, hbm, hbm, hbm, hbm, hbm, vmem, hbm],
        out_specs=hbm,
        scratch_shapes=[
            pltpu.VMEM((S, D), BF16),
            pltpu.VMEM((3, D, 2 * D), BF16),
            pltpu.VMEM((H, D // 2, 3 * Dh), U32),
            pltpu.VMEM((H * Dh // 2, D), U32),
            pltpu.VMEM((D, F), BF16),
            pltpu.VMEM((D, F), BF16),
            pltpu.VMEM((F, D), BF16),
            pltpu.VMEM((8, 6 * D), F32),
            pltpu.VMEM((L, D), F32),
            pltpu.VMEM((L, H * Dh), F32),
            pltpu.VMEM((S, D), F32),
            pltpu.VMEM((S, D), BF16),
            pltpu.VMEM((S, D), A_x.dtype),
            dma(()), dma((3,)), dma((3 * H,)), dma(()), dma((3,)), dma((S // _FM,)),
        ],
        compiler_params=pltpu.CompilerParams(vmem_limit_bytes=126 * 1024 * 1024),
    )(A_x.reshape(S, D), A_mem0.reshape(M, D), A_Wq.reshape(D // 2, 2 * H, Dh), A_Wk.reshape(D // 2, 2 * H, Dh),
      A_Wv.reshape(D // 2, 2 * H, Dh), A_Wo.reshape(H * Dh, D), B_w1, B_w3, B_w2, c, w_mod)
    return out.reshape(B, S, D)
```

```python
import functools

import jax
import jax.numpy as jnp
from jax import lax
import jax.experimental.pallas as pl
import jax.experimental.pallas.tpu as pltpu

F32 = jnp.float32
BF16 = jnp.bfloat16
U32 = jnp.uint32

_HG = 4
_FM = 256
_FC = 512
_TAIL = 8
_NPRE = 2
_LAG = 1


def _mm(a, b):
    return lax.dot_general(a, b, (((1,), (0,)), ((), ())), preferred_element_type=F32)


def _mm_nt(a, b):
    return lax.dot_general(a, b, (((1,), (1,)), ((), ())), preferred_element_type=F32)


def _ln_mod(x, scale1, shift):
    m = jnp.mean(x, axis=-1, keepdims=True)
    d = x - m
    v = jnp.mean(d * d, axis=-1, keepdims=True)
    return d * lax.rsqrt(v + 1e-5) * scale1 + shift


def _body(x_hbm, mem0_ref, wq_hbm, wk_hbm, wv_hbm, wo_hbm, w1_hbm, w3_hbm, w2_hbm, c_ref,
          wmod_hbm, out_hbm,
          xs, xt, wmod, wqkv, wo, w1, w3, w2, mod, hx, ht, pre, mem, obuf, h2, ybuf,
          sem_x, sem_mod, sem_w, sem_o, sem_f, sem_out, *, H, Dh):
    n_seg, seg, D = xs.shape
    M = mem0_ref.shape[0]
    L = M + seg
    F = w1.shape[1]
    HP = H // 2
    T = _TAIL
    spb = _FM // seg
    n_blk = n_seg // spb

    def mod_cp(j):
        return pltpu.make_async_copy(wmod_hbm.at[:, pl.ds(j * 2 * D, 2 * D)],
                                     wmod.at[j], sem_mod.at[j])

    x_cp = pltpu.make_async_copy(x_hbm, xs, sem_x.at[0])
    xt_cp = pltpu.make_async_copy(x_hbm.at[:, pl.ds(seg - T, T), :], xt, sem_x.at[1])
    w_hbms = (wq_hbm, wk_hbm, wv_hbm)

    def w_cp(m, i, odd):
        src = w_hbms[m].bitcast(U32).at[:, odd * HP + i, :]
        return pltpu.make_async_copy(src, wqkv.at[m, 2 * i + odd], sem_w.at[m * H + 2 * i + odd])

    wo_cp = pltpu.make_async_copy(wo_hbm.bitcast(U32), wo, sem_o)
    f_cps = [pltpu.make_async_copy(s, d, sem_f.at[i])
             for i, (s, d) in enumerate(((w1_hbm, w1), (w3_hbm, w3), (w2_hbm, w2)))]

    def start_w(m):
        for i in range(HP):
            w_cp(m, i, 0).start()
            w_cp(m, i, 1).start()

    mod_cp(0).start()
    xt_cp.start()
    start_w(0)
    x_cp.start()

    cv = c_ref[...].astype(F32)
    sc = jnp.broadcast_to(cv * jax.nn.sigmoid(cv), (8, D)).astype(BF16)

    def mod_part(j):
        mod_cp(j).wait()
        mod[:, pl.ds(j * 2 * D, 2 * D)] = _mm(sc, wmod[j])

    def mod_row(j):
        return mod[0:1, pl.ds(j * D, D)]

    def ln1(xv):
        return _ln_mod(xv.astype(F32), 1.0 + mod_row(1), mod_row(0))

    mod_part(0)
    xt_cp.wait()
    ht[...] = ln1(xt[...].reshape(n_seg * T, D)).astype(BF16)

    def w_tile(m, hd):
        return pltpu.bitcast(wqkv[m, hd], BF16)

    for m in range(3):
        if m == 0:
            start_w(1)
        elif m == 1:
            start_w(2)
            wo_cp.start()
            x_cp.wait()

        def retile(i, carry, m=m):
            w_cp(m, i, 0).wait()
            w_cp(m, i, 1).wait()
            a = wqkv[m, 2 * i]
            b = wqkv[m, 2 * i + 1]
            even = (a & jnp.uint32(0xFFFF)) | (b << 16)
            odd = (a >> 16) | (b & jnp.uint32(0xFFFF0000))
            wqkv[m, 2 * i] = even
            wqkv[m, 2 * i + 1] = odd
            if m < _NPRE:
                w = jnp.concatenate([pltpu.bitcast(even, BF16), pltpu.bitcast(odd, BF16)], axis=1)
                r = _mm(ht[...], w)
                pre[m, 2 * i] = r[:, 0:Dh]
                pre[m, 2 * i + 1] = r[:, Dh:2 * Dh]
            if m == 1:
                n = n_seg // HP
                for j in range(n):
                    hx[i * n + j] = ln1(xs[i * n + j])
            return carry

        lax.fori_loop(0, HP, retile, 0)

    mod_cp(1).start()
    mod_cp(2).start()
    for cp in f_cps:
        cp.start()
    wo_cp.wait()

    mem[...] = mem0_ref[...].astype(F32)
    scale = Dh ** -0.5
    NG = H // _HG

    def step(s, carry):
        row = lax.broadcasted_iota(jnp.int32, (L, L), 0)
        col = lax.broadcasted_iota(jnp.int32, (L, L), 1)
        mask = (row < M) | (row >= col)
        h = jnp.concatenate([mem[...], hx[s]], axis=0)
        tail = pl.ds(pl.multiple_of(s * T, T), T)

        def proj(g):
            heads = range(g * _HG, (g + 1) * _HG)
            res = []
            for m in range(3):
                w = jnp.concatenate([w_tile(m, hd) for hd in heads], axis=1)
                r = _mm(h[0:L - T] if m < _NPRE else h, w)
                r = [r[:, j * Dh:(j + 1) * Dh] for j in range(_HG)]
                if m < _NPRE:
                    r = [jnp.concatenate([r[j], pre[m, hd, tail, :]], axis=0)
                         for j, hd in enumerate(heads)]
                res.append(r)
            return list(zip(*res))

        def attend(g, qkvs):
            for j, (q, k, v) in enumerate(qkvs):
                sco = jnp.where(mask, _mm_nt(q, k.astype(BF16)) * scale, -1e9)
                e = jnp.exp(sco - jnp.max(sco, axis=-1, keepdims=True))
                inv = 1.0 / jnp.sum(e, axis=-1, keepdims=True)
                obuf[:, pl.ds((g * _HG + j) * Dh, Dh)] = _mm(e, v.astype(BF16)) * inv

        def out_proj(g):
            kk = _HG * Dh
            return _mm(obuf[:, pl.ds(g * kk, kk)],
                       pltpu.bitcast(wo[pl.ds(g * kk // 2, kk // 2), :], BF16))

        acc = None
        pend = proj(0)
        for g in range(NG):
            nxt = proj(g + 1) if g + 1 < NG else None
            attend(g, pend)
            pend = nxt
            if g >= _LAG:
                part = out_proj(g - _LAG)
                acc = part if acc is None else acc + part
        for g in range(NG - _LAG, NG):
            part = out_proj(g)
            acc = part if acc is None else acc + part

        mem[...] = acc[0:M]
        hx[s] = acc[M:L]
        return carry

    lax.fori_loop(0, n_seg, step, 0)

    mod_part(1)
    mod_part(2)
    for cp in f_cps:
        cp.wait()

    def out_cp(i):
        blk = pl.ds(i * spb, spb)
        return pltpu.make_async_copy(ybuf.at[blk], out_hbm.at[blk], sem_out.at[i])

    def residual(i):
        blk = pl.ds(i * spb, spb)
        xn = xs[blk].astype(F32).reshape(_FM, D) + mod_row(2) * hx[blk].reshape(_FM, D)
        hx[blk] = xn.reshape(spb, seg, D)
        h2[i] = _ln_mod(xn, 1.0 + mod_row(4), mod_row(3)).astype(BF16)

    def ffn(i, carry, last=False):
        hb = h2[i]
        if not last:
            residual(i + 1)
        acc = None
        for f in range(F // _FC):
            cols = pl.ds(f * _FC, _FC)
            gate = _mm(hb, w1[:, cols])
            up = _mm(hb, w3[:, cols])
            act = (gate * jax.nn.sigmoid(gate) * up).astype(BF16)
            part = _mm(act, w2[cols, :])
            acc = part if acc is None else acc + part
        blk = pl.ds(i * spb, spb)
        y = hx[blk].reshape(_FM, D) + mod_row(5) * acc
        ybuf[blk] = y.astype(ybuf.dtype).reshape(spb, seg, D)
        out_cp(i).start()
        return carry

    residual(0)
    lax.fori_loop(0, n_blk - 1, ffn, 0)
    ffn(n_blk - 1, 0, last=True)
    for i in range(n_blk):
        out_cp(i).wait()


@functools.partial(jax.jit, static_argnames=("A_seg_len",))
def pallas_adaLN_cond__memory_aug_recurrent_mem_tr__glu_gated_swiglu__prompt_kernel(
        A_x, A_mem0, A_Wq, A_Wk, A_Wv, A_Wo, A_seg_len, B_x, B_w1, B_w3, B_w2, c, w_mod):
    del B_x
    B, S, D = A_x.shape
    _, H, Dh = A_Wq.shape
    M = A_mem0.shape[1]
    F = B_w1.shape[1]
    seg = int(A_seg_len)
    assert B == 1 and S % seg == 0 and S % _FM == 0 and F % _FC == 0
    L = M + seg
    hbm = pl.BlockSpec(memory_space=pl.ANY)
    vmem = pl.BlockSpec(memory_space=pltpu.VMEM)
    dma = pltpu.SemaphoreType.DMA
    n_seg = S // seg
    out = pl.pallas_call(
        functools.partial(_body, H=H, Dh=Dh),
        out_shape=jax.ShapeDtypeStruct((n_seg, seg, D), A_x.dtype),
        in_specs=[hbm, vmem, hbm, hbm, hbm, hbm, hbm, hbm, hbm, vmem, hbm],
        out_specs=hbm,
        scratch_shapes=[
            pltpu.VMEM((n_seg, seg, D), BF16),
            pltpu.VMEM((n_seg, _TAIL, D), BF16),
            pltpu.VMEM((3, D, 2 * D), BF16),
            pltpu.VMEM((3, H, D // 2, Dh), U32),
            pltpu.VMEM((H * Dh // 2, D), U32),
            pltpu.VMEM((D, F), BF16),
            pltpu.VMEM((D, F), BF16),
            pltpu.VMEM((F, D), BF16),
            pltpu.VMEM((8, 6 * D), F32),
            pltpu.VMEM((n_seg, seg, D), F32),
            pltpu.VMEM((n_seg * _TAIL, D), BF16),
            pltpu.VMEM((_NPRE, H, n_seg * _TAIL, Dh), F32),
            pltpu.VMEM((M, D), F32),
            pltpu.VMEM((L, H * Dh), F32),
            pltpu.VMEM((S // _FM, _FM, D), BF16),
            pltpu.VMEM((n_seg, seg, D), A_x.dtype),
            dma((2,)), dma((3,)), dma((3 * H,)), dma(()), dma((3,)), dma((S // _FM,)),
        ],
        compiler_params=pltpu.CompilerParams(vmem_limit_bytes=126 * 1024 * 1024),
    )(A_x.reshape(n_seg, seg, D), A_mem0.reshape(M, D), A_Wq.reshape(D // 2, 2 * H, Dh),
      A_Wk.reshape(D // 2, 2 * H, Dh), A_Wv.reshape(D // 2, 2 * H, Dh), A_Wo.reshape(H * Dh, D),
      B_w1, B_w3, B_w2, c, w_mod)
    return out.reshape(B, S, D)
```

```python
import functools

import jax
import jax.numpy as jnp
from jax import lax
import jax.experimental.pallas as pl
import jax.experimental.pallas.tpu as pltpu

F32 = jnp.float32
BF16 = jnp.bfloat16
U32 = jnp.uint32

_HG = 4
_FM = 256
_FC = 512
_TAIL = 8
_NPRE = 2
_LAG = 1
_UNROLL = 1
_AHEAD = 4


def _mm(a, b):
    return lax.dot_general(a, b, (((1,), (0,)), ((), ())), preferred_element_type=F32)


def _mm_nt(a, b):
    return lax.dot_general(a, b, (((1,), (1,)), ((), ())), preferred_element_type=F32)


def _ln_mod(x, scale1, shift):
    m = jnp.mean(x, axis=-1, keepdims=True)
    d = x - m
    v = jnp.mean(d * d, axis=-1, keepdims=True)
    return d * lax.rsqrt(v + 1e-5) * scale1 + shift


def _body(x_hbm, mem0_ref, wq_hbm, wk_hbm, wv_hbm, wo_hbm, w1_hbm, w3_hbm, w2_hbm, c_ref,
          wmod_hbm, out_hbm,
          xs, xt, wmod, wqkv, wo, w1, w3, w2, mod, hx, ht, pre, mem, obuf, h2, ybuf,
          sem_x, sem_mod, sem_w, sem_o, sem_f, sem_out, *, H, Dh):
    n_seg, seg, D = xs.shape
    M = mem0_ref.shape[0]
    L = M + seg
    F = w1.shape[1]
    HP = H // 2
    T = _TAIL
    spb = _FM // seg
    n_blk = n_seg // spb

    def mod_cp(j):
        return pltpu.make_async_copy(wmod_hbm.at[:, pl.ds(j * 2 * D, 2 * D)],
                                     wmod.at[j], sem_mod.at[j])

    def x_cp(i):
        blk = pl.ds(i * (n_seg // HP), n_seg // HP)
        return pltpu.make_async_copy(x_hbm.at[blk], xs.at[blk], sem_x.at[i])

    xt_cp = pltpu.make_async_copy(x_hbm.at[:, pl.ds(seg - T, T), :], xt, sem_x.at[HP])
    w_hbms = (wq_hbm, wk_hbm, wv_hbm)

    def w_cp(m, i, odd):
        src = w_hbms[m].bitcast(U32).at[:, odd * HP + i, :]
        return pltpu.make_async_copy(src, wqkv.at[m, 2 * i + odd], sem_w.at[m * H + 2 * i + odd])

    def wo_cp(i):
        rows = pl.ds(pl.multiple_of(i * Dh, Dh), Dh)
        return pltpu.make_async_copy(wo_hbm.bitcast(U32).at[rows], wo.at[rows], sem_o.at[i])

    f_cps = [pltpu.make_async_copy(s, d, sem_f.at[i])
             for i, (s, d) in enumerate(((w1_hbm, w1), (w3_hbm, w3), (w2_hbm, w2)))]

    def start_pair(m, i):
        w_cp(m, i, 0).start()
        w_cp(m, i, 1).start()

    mod_cp(0).start()
    xt_cp.start()
    start_pair(0, 0)

    cv = c_ref[...].astype(F32)
    sc = jnp.broadcast_to(cv * jax.nn.sigmoid(cv), (8, D)).astype(BF16)

    def mod_part(j):
        mod[:, pl.ds(j * 2 * D, 2 * D)] = _mm(sc, wmod[j])

    def mod_row(j):
        return mod[0:1, pl.ds(j * D, D)]

    def ln1(xv):
        return _ln_mod(xv.astype(F32), 1.0 + mod_row(1), mod_row(0))

    mod_cp(0).wait()
    for i in range(1, _AHEAD):
        start_pair(0, i)
    mod_part(0)
    xt_cp.wait()
    ht[...] = ln1(xt[...].reshape(n_seg * T, D)).astype(BF16)

    def w_tile(m, hd):
        return pltpu.bitcast(wqkv[m, hd], BF16)

    for m in range(3):
        def retile(i, carry, m=m):
            if m == 0:
                pl.when(i + _AHEAD < HP)(lambda: start_pair(0, i + _AHEAD))
                start_pair(1, i)
                x_cp(i).start()
            elif m == 1:
                start_pair(2, i)
                wo_cp(i).start()
                x_cp(i).wait()
            w_cp(m, i, 0).wait()
            w_cp(m, i, 1).wait()
            a = wqkv[m, 2 * i]
            b = wqkv[m, 2 * i + 1]
            even = (a & jnp.uint32(0xFFFF)) | (b << 16)
            odd = (a >> 16) | (b & jnp.uint32(0xFFFF0000))
            wqkv[m, 2 * i] = even
            wqkv[m, 2 * i + 1] = odd
            if m < _NPRE:
                w = jnp.concatenate([pltpu.bitcast(even, BF16), pltpu.bitcast(odd, BF16)], axis=1)
                r = _mm(ht[...], w)
                pre[m, 2 * i] = r[:, 0:Dh]
                pre[m, 2 * i + 1] = r[:, Dh:2 * Dh]
            if m == 1:
                n = n_seg // HP
                for j in range(n):
                    hx[i * n + j] = ln1(xs[i * n + j])
            return carry

        lax.fori_loop(0, HP, retile, 0)

    mod_cp(1).start()
    mod_cp(2).start()
    for cp in f_cps:
        cp.start()
    for i in range(HP):
        wo_cp(i).wait()

    mem[...] = mem0_ref[...].astype(F32)
    scale = Dh ** -0.5
    NG = H // _HG

    def step(s, carry):
        row = lax.broadcasted_iota(jnp.int32, (L, L), 0)
        col = lax.broadcasted_iota(jnp.int32, (L, L), 1)
        mask = (row < M) | (row >= col)
        h = jnp.concatenate([mem[...], hx[s]], axis=0)
        tail = pl.ds(pl.multiple_of(s * T, T), T)

        def proj(m, g):
            heads = range(g * _HG, (g + 1) * _HG)
            w = jnp.concatenate([w_tile(m, hd) for hd in heads], axis=1)
            r = _mm(h[0:L - T] if m < _NPRE else h, w)
            r = [r[:, j * Dh:(j + 1) * Dh] for j in range(_HG)]
            if m < _NPRE:
                r = [jnp.concatenate([r[j], pre[m, hd, tail, :]], axis=0)
                     for j, hd in enumerate(heads)]
            return r

        def probs(qs, ks):
            res = []
            for q, k in zip(qs, ks):
                sco = jnp.where(mask, _mm_nt(q, k.astype(BF16)) * scale, -1e9)
                e = jnp.exp(sco - jnp.max(sco, axis=-1, keepdims=True))
                res.append((e, 1.0 / jnp.sum(e, axis=-1, keepdims=True)))
            return res

        def mix(g, ps, vs):
            for j, ((e, inv), v) in enumerate(zip(ps, vs)):
                obuf[:, pl.ds((g * _HG + j) * Dh, Dh)] = _mm(e, v.astype(BF16)) * inv

        def out_proj(g, acc):
            kk = _HG * Dh
            part = _mm(obuf[:, pl.ds(g * kk, kk)],
                       pltpu.bitcast(wo[pl.ds(g * kk // 2, kk // 2), :], BF16))
            return part if acc is None else acc + part

        acc = ps = vs = None
        for g in range(-1, NG):
            if g + 1 < NG:
                qs, ks = proj(0, g + 1), proj(1, g + 1)
            if g >= 0:
                mix(g, ps, vs)
            if g + 1 < NG:
                vs = proj(2, g + 1)
                ps = probs(qs, ks)
            if g >= _LAG:
                acc = out_proj(g - _LAG, acc)
        for g in range(NG - _LAG, NG):
            acc = out_proj(g, acc)

        mem[...] = acc[0:M]
        hx[s] = acc[M:L]
        return carry

    lax.fori_loop(0, n_seg, step, 0, unroll=_UNROLL)

    for j in (1, 2):
        mod_cp(j).wait()
        mod_part(j)
    for cp in f_cps:
        cp.wait()

    def out_cp(i):
        blk = pl.ds(i * spb, spb)
        return pltpu.make_async_copy(ybuf.at[blk], out_hbm.at[blk], sem_out.at[i])

    def residual(i):
        blk = pl.ds(i * spb, spb)
        xn = xs[blk].astype(F32).reshape(_FM, D) + mod_row(2) * hx[blk].reshape(_FM, D)
        hx[blk] = xn.reshape(spb, seg, D)
        h2[i] = _ln_mod(xn, 1.0 + mod_row(4), mod_row(3)).astype(BF16)

    def ffn(i, carry, last=False):
        hb = h2[i]
        if not last:
            residual(i + 1)
        acc = None
        for f in range(F // _FC):
            cols = pl.ds(f * _FC, _FC)
            gate = _mm(hb, w1[:, cols])
            up = _mm(hb, w3[:, cols])
            act = (gate * jax.nn.sigmoid(gate) * up).astype(BF16)
            part = _mm(act, w2[cols, :])
            acc = part if acc is None else acc + part
        blk = pl.ds(i * spb, spb)
        y = hx[blk].reshape(_FM, D) + mod_row(5) * acc
        ybuf[blk] = y.astype(ybuf.dtype).reshape(spb, seg, D)
        out_cp(i).start()
        return carry

    residual(0)
    lax.fori_loop(0, n_blk - 1, ffn, 0)
    ffn(n_blk - 1, 0, last=True)
    for i in range(n_blk):
        out_cp(i).wait()


@functools.partial(jax.jit, static_argnames=("A_seg_len",))
def pallas_adaLN_cond__memory_aug_recurrent_mem_tr__glu_gated_swiglu__prompt_kernel(
        A_x, A_mem0, A_Wq, A_Wk, A_Wv, A_Wo, A_seg_len, B_x, B_w1, B_w3, B_w2, c, w_mod):
    del B_x
    B, S, D = A_x.shape
    _, H, Dh = A_Wq.shape
    M = A_mem0.shape[1]
    F = B_w1.shape[1]
    seg = int(A_seg_len)
    assert B == 1 and S % seg == 0 and S % _FM == 0 and F % _FC == 0
    L = M + seg
    hbm = pl.BlockSpec(memory_space=pl.ANY)
    vmem = pl.BlockSpec(memory_space=pltpu.VMEM)
    dma = pltpu.SemaphoreType.DMA
    n_seg = S // seg
    out = pl.pallas_call(
        functools.partial(_body, H=H, Dh=Dh),
        out_shape=jax.ShapeDtypeStruct((n_seg, seg, D), A_x.dtype),
        in_specs=[hbm, vmem, hbm, hbm, hbm, hbm, hbm, hbm, hbm, vmem, hbm],
        out_specs=hbm,
        scratch_shapes=[
            pltpu.VMEM((n_seg, seg, D), BF16),
            pltpu.VMEM((n_seg, _TAIL, D), BF16),
            pltpu.VMEM((3, D, 2 * D), BF16),
            pltpu.VMEM((3, H, D // 2, Dh), U32),
            pltpu.VMEM((H * Dh // 2, D), U32),
            pltpu.VMEM((D, F), BF16),
            pltpu.VMEM((D, F), BF16),
            pltpu.VMEM((F, D), BF16),
            pltpu.VMEM((8, 6 * D), F32),
            pltpu.VMEM((n_seg, seg, D), F32),
            pltpu.VMEM((n_seg * _TAIL, D), BF16),
            pltpu.VMEM((_NPRE, H, n_seg * _TAIL, Dh), F32),
            pltpu.VMEM((M, D), F32),
            pltpu.VMEM((L, H * Dh), F32),
            pltpu.VMEM((S // _FM, _FM, D), BF16),
            pltpu.VMEM((n_seg, seg, D), A_x.dtype),
            dma((H // 2 + 1,)), dma((3,)), dma((3 * H,)), dma((H // 2,)), dma((3,)), dma((S // _FM,)),
        ],
        compiler_params=pltpu.CompilerParams(vmem_limit_bytes=126 * 1024 * 1024),
    )(A_x.reshape(n_seg, seg, D), A_mem0.reshape(M, D), A_Wq.reshape(D // 2, 2 * H, Dh),
      A_Wk.reshape(D // 2, 2 * H, Dh), A_Wv.reshape(D // 2, 2 * H, Dh), A_Wo.reshape(H * Dh, D),
      B_w1, B_w3, B_w2, c, w_mod)
    return out.reshape(B, S, D)
```

```python
import functools

import jax
import jax.numpy as jnp
from jax import lax
import jax.experimental.pallas as pl
import jax.experimental.pallas.tpu as pltpu

F32 = jnp.float32
BF16 = jnp.bfloat16
U32 = jnp.uint32

_HG = 4
_FM = 128
_FC = 512
_TAIL = 8
_LAG = 1
_UNROLL = 2
_XA = 8
_AE = 3
_PU = 1
_TPOS = (0, 2)
_NOBC = False
_MC = 512


def _mm(a, b):
    return lax.dot_general(a, b, (((1,), (0,)), ((), ())), preferred_element_type=F32)


def _mm_nt(a, b):
    return lax.dot_general(a, b, (((1,), (1,)), ((), ())), preferred_element_type=F32)


def _normalize(x):
    m = jnp.mean(x, axis=-1, keepdims=True)
    d = x - m
    v = jnp.mean(d * d, axis=-1, keepdims=True)
    return d * lax.rsqrt(v + 1e-5)


def _body(x_hbm, mem0_ref, wq_hbm, wk_hbm, wv_hbm, wo_hbm, w1_hbm, w3_hbm, w2_hbm, c_ref,
          wmod_hbm, out_hbm,
          xs, xt, wmod, wq, wk, wv, wo, w1, w3, w2, mod, att, ht, pre, hbuf, obuf, h2, ybuf,
          sem_x, sem_mod, sem_w, sem_o, sem_f, sem_out, *, H, Dh):
    n_seg, seg, D = xs.shape
    M = mem0_ref.shape[0]
    L = M + seg
    F = w1.shape[1]
    HP = H // 2
    T = _TAIL
    spb = _FM // seg
    n_blk = n_seg // spb

    def mod_cp(j):
        cols = pl.ds(j * _MC, _MC)
        return pltpu.make_async_copy(wmod_hbm.bitcast(U32).at[:, cols], wmod.at[j], sem_mod.at[j])

    xa_cp = pltpu.make_async_copy(x_hbm.at[pl.ds(0, _XA)], xs.at[pl.ds(0, _XA)], sem_x.at[0])
    xb_cp = pltpu.make_async_copy(x_hbm.at[pl.ds(_XA, n_seg - _XA)],
                                  xs.at[pl.ds(_XA, n_seg - _XA)], sem_x.at[1])
    xt_cp = pltpu.make_async_copy(x_hbm.at[:, pl.ds(seg - T, T), :], xt, sem_x.at[2])
    w_hbms = (wq_hbm, wk_hbm, wv_hbm)
    wqkv = (wq, wk, wv)

    def w_cp(m, i, odd):
        src = w_hbms[m].bitcast(U32).at[:, odd * HP + i, :]
        return pltpu.make_async_copy(src, wqkv[m].at[2 * i + odd], sem_w.at[m * H + 2 * i + odd])

    def wo_cp(i):
        rows = pl.ds(pl.multiple_of(i * Dh, Dh), Dh)
        return pltpu.make_async_copy(wo_hbm.bitcast(U32).at[rows], wo.at[rows], sem_o.at[i])

    f_cps = [pltpu.make_async_copy(s, d, sem_f.at[i])
             for i, (s, d) in enumerate(((w1_hbm, w1), (w3_hbm, w3), (w2_hbm, w2)))]

    def start_pair(ms, i):
        for m in ms:
            w_cp(m, i, 0).start()
            w_cp(m, i, 1).start()

    def wait_pair(ms, i):
        for m in ms:
            w_cp(m, i, 0).wait()
            w_cp(m, i, 1).wait()

    def retile(ms, i):
        tiles = []
        for m in ms:
            a = wqkv[m][2 * i]
            b = wqkv[m][2 * i + 1]
            even = (a & jnp.uint32(0xFFFF)) | (b << 16)
            odd = (a >> 16) | (b & jnp.uint32(0xFFFF0000))
            wqkv[m][2 * i] = even
            wqkv[m][2 * i + 1] = odd
            tiles += [pltpu.bitcast(even, BF16), pltpu.bitcast(odd, BF16)]
        return tiles

    def w_tile(m, hd):
        return pltpu.bitcast(wqkv[m][hd], BF16)

    qkv = (0, 1, 2)
    n_mod_a = 2 * D // _MC
    xt_cp.start()
    for j in range(n_mod_a):
        mod_cp(j).start()

    cv = c_ref[...].astype(F32)
    sc = jnp.broadcast_to(cv * jax.nn.sigmoid(cv), (8, D))

    def mod_part(j):
        mod[:, pl.ds(j * _MC, _MC)] = _mm(sc, pltpu.bitcast(wmod[j], BF16))

    def mod_row(j):
        return mod[0:1, pl.ds(j * D, D)]

    def ln1(xv):
        return _normalize(xv.astype(F32)) * (1.0 + mod_row(1)) + mod_row(0)

    xt_cp.wait()
    start_pair(qkv, 0)
    att[0:n_seg * T // seg] = _normalize(xt[...].astype(F32).reshape(n_seg * T, D)).reshape(-1, seg, D)
    for j in range(n_mod_a):
        mod_cp(j).wait()
        if j == n_mod_a - 1:
            start_pair(qkv, 1)
        mod_part(j)
    ht[...] = pltpu.bitcast((att[0:n_seg * T // seg].reshape(n_seg * T, D) * (1.0 + mod_row(1))
                             + mod_row(0)).astype(BF16), U32)
    for i in range(2, _AE):
        start_pair(qkv, i)
    xa_cp.start()

    def arrive(j, carry):
        def traffic():
            for u in range(_PU):
                i = j * _PU + u
                pl.when(i + _AE < HP)(functools.partial(start_pair, qkv, i + _AE))
                wo_cp(i).start()
            for u in range(_PU):
                i = (j + 1) * _PU + u
                pl.when(i < HP)(functools.partial(wait_pair, qkv, i))

        for u in range(_PU):
            i = j * _PU + u
            for m in qkv:
                w = jnp.concatenate(retile((m,), i), axis=1)
                r = _mm(pltpu.bitcast(ht[...], BF16), w)
                if (u, m) == _TPOS:
                    traffic()
                pre[m, 2 * i] = r[:, 0:Dh]
                pre[m, 2 * i + 1] = r[:, Dh:2 * Dh]
        return carry

    for i in range(_PU):
        wait_pair(qkv, i)
    lax.fori_loop(0, HP // _PU, arrive, 0)
    xb_cp.start()
    xa_cp.wait()
    hbuf[0:M] = mem0_ref[...].astype(F32)
    hbuf[M:L] = ln1(xs[0])
    for i in range(HP):
        wo_cp(i).wait()
    for j in range(n_mod_a, 6 * D // _MC):
        mod_cp(j).start()
    for cp in f_cps:
        cp.start()

    scale = Dh ** -0.5
    NG = H // _HG

    def step(s):
        row = lax.broadcasted_iota(jnp.int32, (L, L), 0)
        col = lax.broadcasted_iota(jnp.int32, (L, L), 1)
        mask = (row < M) | (row >= col)
        h = hbuf[0:L - T]
        tail = pl.ds(pl.multiple_of(s * T, T), T)

        def proj(m, g):
            heads = range(g * _HG, (g + 1) * _HG)
            w = jnp.concatenate([w_tile(m, hd) for hd in heads], axis=1)
            r = _mm(h, w)
            r = [r[:, j * Dh:(j + 1) * Dh] for j in range(_HG)]
            return [jnp.concatenate([r[j], pre[m, hd, tail, :]], axis=0)
                    for j, hd in enumerate(heads)]

        def probs(qs, ks):
            res = []
            for q, k in zip(qs, ks):
                sco = jnp.where(mask, _mm_nt(q, k.astype(BF16)) * scale, -1e9)
                e = jnp.exp(sco - jnp.max(sco, axis=-1, keepdims=True))
                res.append((e, 1.0 / jnp.sum(e, axis=-1, keepdims=True)))
            return res

        def mix(g, ps, vs):
            for j, ((e, inv), v) in enumerate(zip(ps, vs)):
                obuf[:, pl.ds((g * _HG + j) * Dh, Dh)] = _mm(e, v.astype(BF16)) * inv

        def out_proj(g, acc):
            kk = _HG * Dh
            part = _mm(obuf[:, pl.ds(g * kk, kk)],
                       pltpu.bitcast(wo[pl.ds(g * kk // 2, kk // 2), :], BF16))
            return part if acc is None else acc + part

        acc = ps = vs = None
        for g in range(-1, NG):
            if g + 1 < NG:
                qs, ks = proj(0, g + 1), proj(1, g + 1)
            if g >= 0:
                mix(g, ps, vs)
            if g + 1 < NG:
                vs = proj(2, g + 1)
                ps = probs(qs, ks)
            if g >= _LAG:
                acc = out_proj(g - _LAG, acc)
        for g in range(NG - _LAG, NG):
            acc = out_proj(g, acc)

        hbuf[M:L] = ln1(xs[jnp.minimum(s + 1, n_seg - 1)])
        hbuf[0:M] = acc[0:M]
        att[s] = acc[M:L]

    def steps(j, carry):
        pl.when(j == _XA // _UNROLL - 1)(xb_cp.wait)
        for u in range(_UNROLL):
            step(j * _UNROLL + u)
        return carry

    lax.fori_loop(0, n_seg // _UNROLL, steps, 0)

    for j in range(n_mod_a, 6 * D // _MC):
        mod_cp(j).wait()
    for j in range(n_mod_a, 6 * D // _MC):
        mod_part(j)
    for cp in f_cps:
        cp.wait()

    def out_cp(i):
        blk = pl.ds(i * spb, spb)
        return pltpu.make_async_copy(ybuf.at[blk], out_hbm.at[blk], sem_out.at[i])

    def residual(i):
        blk = pl.ds(i * spb, spb)
        return xs[blk].astype(F32).reshape(_FM, D) + mod_row(2) * att[blk].reshape(_FM, D)

    def ln2(i, slot):
        h2[slot] = (_normalize(residual(i)) * (1.0 + mod_row(4)) + mod_row(3)).astype(BF16)

    def ffn(i, carry):
        hb = h2[i % 2]
        nf = F // _FC
        acc = act = None
        for f in range(nf + 1):
            prev = act
            if f < nf:
                cols = pl.ds(f * _FC, _FC)
                gate = _mm(hb, w1[:, cols])
                up = _mm(hb, w3[:, cols])
                act = (gate * jax.nn.sigmoid(gate) * up).astype(BF16)
            if f > 0:
                part = _mm(prev, w2[pl.ds((f - 1) * _FC, _FC), :])
                acc = part if acc is None else acc + part
        y = residual(i) + mod_row(5) * acc
        ybuf[pl.ds(i * spb, spb)] = y.astype(ybuf.dtype).reshape(spb, seg, D)
        ln2(jnp.minimum(i + 1, n_blk - 1), (i + 1) % 2)
        out_cp(i).start()
        return carry

    ln2(0, 0)
    lax.fori_loop(0, n_blk, ffn, 0)
    for i in range(n_blk):
        out_cp(i).wait()


@functools.partial(jax.jit, static_argnames=("A_seg_len",))
def pallas_adaLN_cond__memory_aug_recurrent_mem_tr__glu_gated_swiglu__prompt_kernel(
        A_x, A_mem0, A_Wq, A_Wk, A_Wv, A_Wo, A_seg_len, B_x, B_w1, B_w3, B_w2, c, w_mod):
    del B_x
    B, S, D = A_x.shape
    _, H, Dh = A_Wq.shape
    M = A_mem0.shape[1]
    F = B_w1.shape[1]
    seg = int(A_seg_len)
    assert B == 1 and S % seg == 0 and S % _FM == 0 and F % _FC == 0
    L = M + seg
    hbm = pl.BlockSpec(memory_space=pl.ANY)
    vmem = pl.BlockSpec(memory_space=pltpu.VMEM)
    dma = pltpu.SemaphoreType.DMA
    n_seg = S // seg
    out = pl.pallas_call(
        functools.partial(_body, H=H, Dh=Dh),
        out_shape=jax.ShapeDtypeStruct((n_seg, seg, D), A_x.dtype),
        in_specs=[hbm, vmem, hbm, hbm, hbm, hbm, hbm, hbm, hbm, vmem, hbm],
        out_specs=hbm,
        scratch_shapes=[
            pltpu.VMEM((n_seg, seg, D), BF16),
            pltpu.VMEM((n_seg, _TAIL, D), BF16),
            pltpu.VMEM((6 * D // _MC, D // 2, _MC), U32),
            pltpu.VMEM((H, D // 2, Dh), U32),
            pltpu.VMEM((H, D // 2, Dh), U32),
            pltpu.VMEM((H, D // 2, Dh), U32),
            pltpu.VMEM((H * Dh // 2, D), U32),
            pltpu.VMEM((D, F), BF16),
            pltpu.VMEM((D, F), BF16),
            pltpu.VMEM((F, D), BF16),
            pltpu.VMEM((8, 6 * D), F32),
            pltpu.VMEM((n_seg, seg, D), F32),
            pltpu.VMEM((n_seg * _TAIL // 2, D), U32),
            pltpu.VMEM((3, H, n_seg * _TAIL, Dh), F32),
            pltpu.VMEM((L, D), F32),
            pltpu.VMEM((L, H * Dh), F32),
            pltpu.VMEM((2, _FM, D), BF16),
            pltpu.VMEM((n_seg, seg, D), A_x.dtype),
            dma((3,)), dma((6 * D // _MC,)), dma((3 * H,)), dma((H // 2,)), dma((3,)), dma((S // _FM,)),
        ],
        compiler_params=pltpu.CompilerParams(vmem_limit_bytes=126 * 1024 * 1024, disable_bounds_checks=_NOBC),
    )(A_x.reshape(n_seg, seg, D), A_mem0.reshape(M, D), A_Wq.reshape(D // 2, 2 * H, Dh),
      A_Wk.reshape(D // 2, 2 * H, Dh), A_Wv.reshape(D // 2, 2 * H, Dh), A_Wo.reshape(H * Dh, D),
      B_w1, B_w3, B_w2, c, w_mod)
    return out.reshape(B, S, D)
```

```python
import functools

import jax
import jax.numpy as jnp
from jax import lax
import jax.experimental.pallas as pl
import jax.experimental.pallas.tpu as pltpu

F32 = jnp.float32
BF16 = jnp.bfloat16
U32 = jnp.uint32

_HG = 4
_FM = 128
_FC = 896
_TAIL = 8
_LAG = 1
_UNROLL = 2
_CR = 32
_XA = 10
_AE = 3
_PU = 1
_TPOS = (0, 2)
_NOBC = True
_MC = 512


def _mm(a, b):
    return lax.dot_general(a, b, (((1,), (0,)), ((), ())), preferred_element_type=F32)


def _mm_nt(a, b):
    return lax.dot_general(a, b, (((1,), (1,)), ((), ())), preferred_element_type=F32)


def _normalize(x):
    m = jnp.mean(x, axis=-1, keepdims=True)
    d = x - m
    v = jnp.mean(d * d, axis=-1, keepdims=True)
    return d * lax.rsqrt(v + 1e-5)


_RHS = (4, 0, 1, 2, 3, 5, 6)


def _strassen_lhs(a11, a12, a21, a22):
    return [v.astype(BF16) for v in
            (a11 + a22, a21 + a22, a11, a22, a11 + a12, a21 - a11, a12 - a22)]


def _strassen_out(p):
    return p[0] + p[3] - p[4] + p[6], p[2] + p[4], p[1] + p[3], p[0] - p[1] + p[2] + p[5]


def _body(x_hbm, mem0_ref, wq_hbm, wk_hbm, wv_hbm, wo_hbm, w1_hbm, w3_hbm, w2_hbm, c_ref,
          wmod_hbm, out_hbm,
          xs, xt, wmod, wq, wk, wv, wo, wu, wd, mod, att, ht, pre, hbuf, obuf, h2, ybuf,
          sem_x, sem_mod, sem_w, sem_o, sem_f, sem_out, *, H, Dh):
    n_seg, seg, D = xs.shape
    M = mem0_ref.shape[0]
    L = M + seg
    F = w1_hbm.shape[1]
    HP = H // 2
    T = _TAIL
    spb = _FM // seg
    n_blk = n_seg // spb

    n_slot = wmod.shape[0]

    def mod_cp(j):
        cols = pl.ds(j * _MC, _MC)
        return pltpu.make_async_copy(wmod_hbm.bitcast(U32).at[:, cols], wmod.at[j % n_slot], sem_mod.at[j])

    xa_cp = pltpu.make_async_copy(x_hbm.at[pl.ds(0, _XA)], xs.at[pl.ds(0, _XA)], sem_x.at[0])
    xb_cp = pltpu.make_async_copy(x_hbm.at[pl.ds(_XA, n_seg - _XA)],
                                  xs.at[pl.ds(_XA, n_seg - _XA)], sem_x.at[1])
    xt_cp = pltpu.make_async_copy(x_hbm.at[:, pl.ds(seg - T, T), :], xt, sem_x.at[2])
    w_hbms = (wq_hbm, wk_hbm, wv_hbm)
    wqkv = (wq, wk, wv)

    def w_cp(m, i, odd):
        src = w_hbms[m].bitcast(U32).at[:, odd * HP + i, :]
        return pltpu.make_async_copy(src, wqkv[m].at[2 * i + odd], sem_w.at[m * H + 2 * i + odd])

    def wo_cp(i):
        rows = pl.ds(pl.multiple_of(i * Dh, Dh), Dh)
        return pltpu.make_async_copy(wo_hbm.bitcast(U32).at[rows], wo.at[rows], sem_o.at[i])

    w1_w, w3_w, w2_w = (r.bitcast(U32) for r in (w1_hbm, w3_hbm, w2_hbm))
    lo, hi = pl.ds(0, D // 4), pl.ds(D // 4, D // 4)
    f_srcs = [(wu.at[k, :, pl.ds(0, F)], src.at[rows]) for k, (src, rows) in
              enumerate(((w1_w, lo), (w3_w, lo), (w1_w, hi), (w3_w, hi)))]
    f_srcs += [(wd.at[2 * r + q, pl.ds(0, F // 4)],
                w2_w.at[pl.ds(r * F // 4, F // 4), pl.ds(q * D // 2, D // 2)])
               for r in range(2) for q in range(2)]
    f_cps = [pltpu.make_async_copy(src, dst, sem_f.at[n])
             for n, (dst, src) in enumerate(f_srcs)]

    def start_pair(ms, i):
        for m in ms:
            w_cp(m, i, 0).start()
            w_cp(m, i, 1).start()

    def wait_pair(ms, i):
        for m in ms:
            w_cp(m, i, 0).wait()
            w_cp(m, i, 1).wait()

    def retile(ms, i):
        tiles = []
        for m in ms:
            a = wqkv[m][2 * i]
            b = wqkv[m][2 * i + 1]
            even = (a & jnp.uint32(0xFFFF)) | (b << 16)
            odd = (a >> 16) | (b & jnp.uint32(0xFFFF0000))
            wqkv[m][2 * i] = even
            wqkv[m][2 * i + 1] = odd
            tiles += [pltpu.bitcast(even, BF16), pltpu.bitcast(odd, BF16)]
        return tiles

    def w_tile(m, hd):
        return pltpu.bitcast(wqkv[m][hd], BF16)

    qkv = (0, 1, 2)
    n_mod_a = 2 * D // _MC
    xt_cp.start()
    for j in range(n_mod_a):
        mod_cp(j).start()

    cv = c_ref[...].astype(F32)
    sc = jnp.broadcast_to(cv * jax.nn.sigmoid(cv), (8, D))

    def mod_part(j):
        mod[:, pl.ds(j * _MC, _MC)] = _mm(sc, pltpu.bitcast(wmod[j % n_slot], BF16))

    def mod_row(j):
        return mod[0:1, pl.ds(j * D, D)]

    def ln1(xv):
        return _normalize(xv.astype(F32)) * (1.0 + mod_row(1)) + mod_row(0)

    xt_cp.wait()
    start_pair(qkv, 0)
    att[0:n_seg * T // seg] = _normalize(xt[...].astype(F32).reshape(n_seg * T, D)).reshape(-1, seg, D)
    for j in range(n_mod_a):
        mod_cp(j).wait()
        if j == n_mod_a - 1:
            start_pair(qkv, 1)
        mod_part(j)
    ht[...] = pltpu.bitcast((att[0:n_seg * T // seg].reshape(n_seg * T, D) * (1.0 + mod_row(1))
                             + mod_row(0)).astype(BF16), U32)
    for i in range(2, _AE):
        start_pair(qkv, i)
    xa_cp.start()
    wo_cp(0).start()

    def arrive(j, carry):
        def traffic():
            for u in range(_PU):
                i = j * _PU + u
                pl.when(i + _AE < HP)(functools.partial(start_pair, qkv, i + _AE))
                pl.when(i + 1 < HP)(lambda i=i: wo_cp(i + 1).start())
            for u in range(_PU):
                i = (j + 1) * _PU + u
                pl.when(i < HP)(functools.partial(wait_pair, qkv, i))

        for u in range(_PU):
            i = j * _PU + u
            for m in qkv:
                w = jnp.concatenate(retile((m,), i), axis=1)
                r = _mm(pltpu.bitcast(ht[...], BF16), w)
                if (u, m) == _TPOS:
                    traffic()
                pre[m, 2 * i] = r[:, 0:Dh]
                pre[m, 2 * i + 1] = r[:, Dh:2 * Dh]
        return carry

    for i in range(_PU):
        wait_pair(qkv, i)
    lax.fori_loop(0, HP // _PU, arrive, 0)
    xb_cp.start()
    xa_cp.wait()
    hbuf[0:M] = mem0_ref[...].astype(F32)
    hbuf[M:L] = ln1(xs[0])
    for i in range(HP):
        wo_cp(i).wait()
    for j in range(n_mod_a, 6 * D // _MC):
        mod_cp(j).start()
    for cp in f_cps:
        cp.start()

    scale = Dh ** -0.5
    NG = H // _HG

    def step(s, jobs):
        row = lax.broadcasted_iota(jnp.int32, (L, L), 0)
        col = lax.broadcasted_iota(jnp.int32, (L, L), 1)
        mask = (row < M) | (row >= col)
        h = hbuf[0:L - T]
        tail = pl.ds(pl.multiple_of(s * T, T), T)

        def proj(m, g):
            heads = range(g * _HG, (g + 1) * _HG)
            w = jnp.concatenate([w_tile(m, hd) for hd in heads], axis=1)
            r = _mm(h, w)
            r = [r[:, j * Dh:(j + 1) * Dh] for j in range(_HG)]
            return [jnp.concatenate([r[j], pre[m, hd, tail, :]], axis=0)
                    for j, hd in enumerate(heads)]

        def probs(qs, ks):
            res = []
            for q, k in zip(qs, ks):
                sco = jnp.where(mask, _mm_nt(q, k.astype(BF16)) * scale, -1e9)
                e = jnp.exp(sco - jnp.max(sco, axis=-1, keepdims=True))
                res.append((e, 1.0 / jnp.sum(e, axis=-1, keepdims=True)))
            return res

        def mix(g, ps, vs):
            for j, ((e, inv), v) in enumerate(zip(ps, vs)):
                obuf[:, pl.ds((g * _HG + j) * Dh, Dh)] = _mm(e, v.astype(BF16)) * inv

        def out_proj(g, acc):
            kk = _HG * Dh
            part = _mm(obuf[:, pl.ds(g * kk, kk)],
                       pltpu.bitcast(wo[pl.ds(g * kk // 2, kk // 2), :], BF16))
            return part if acc is None else acc + part

        acc = ps = vs = None
        for g in range(-1, NG):
            if g + 1 < NG:
                qs, ks = proj(0, g + 1), proj(1, g + 1)
            if g >= 0:
                mix(g, ps, vs)
            if g + 1 < NG:
                vs = proj(2, g + 1)
                ps = probs(qs, ks)
            for job in jobs[g + 1::NG + 1]:
                job()
            if g >= _LAG:
                acc = out_proj(g - _LAG, acc)
        for g in range(NG - _LAG, NG):
            acc = out_proj(g, acc)

        hbuf[M:L] = ln1(xs[jnp.minimum(s + 1, n_seg - 1)])
        hbuf[0:M] = acc[0:M]
        att[s] = acc[M:L]

    n_it = n_seg // _UNROLL
    n_sl = F // 128
    rd = F // 4 // n_sl
    for k in range(4):
        wu[k, :, pl.ds(F, 128)] = jnp.zeros((D // 4, 128), U32)
        wd[k, pl.ds(F // 4, rd), :] = jnp.zeros((rd, D // 2), U32)

    def combine(ref, idx):
        b11, b12, b21, b22 = (pltpu.bitcast(ref[(k,) + idx], BF16).astype(F32) for k in range(4))
        for k, v in ((1, b12 - b22), (2, b21 - b11), (4, b11 + b22), (5, b11 + b12),
                     (6, b21 + b22)):
            ref[(k,) + idx] = pltpu.bitcast(v.astype(BF16), U32)

    def steps(j, carry):
        @pl.when(j == n_it - n_sl)
        def _():
            xb_cp.wait()
            for cp in f_cps:
                cp.wait()

        sl = jnp.where(j < n_it - n_sl, n_sl, j - (n_it - n_sl))
        cols = pl.ds(pl.multiple_of(sl * 128, 128), 128)
        jobs = [functools.partial(combine, wu, (pl.ds(r, _CR), cols))
                for r in range(0, D // 4, _CR)]
        jobs += [functools.partial(combine, wd, (pl.ds(pl.multiple_of(sl * rd + r, 8), 8),
                                                 slice(None))) for r in range(0, rd, 8)]
        for u in range(_UNROLL):
            step(j * _UNROLL + u, jobs[u::_UNROLL])
        return carry

    lax.fori_loop(0, n_seg // _UNROLL, steps, 0)

    for j in range(n_mod_a, 6 * D // _MC):
        mod_cp(j).wait()
    for j in range(n_mod_a, 6 * D // _MC):
        mod_part(j)

    def out_cp(i):
        blk = pl.ds(i * spb, spb)
        return pltpu.make_async_copy(ybuf.at[blk], out_hbm.at[blk], sem_out.at[i])

    def residual(i):
        blk = pl.ds(i * spb, spb)
        return xs[blk].astype(F32).reshape(_FM, D) + mod_row(2) * att[blk].reshape(_FM, D)

    R = _FM // 2

    def ln2(i, slot):
        hn = _normalize(residual(i)) * (1.0 + mod_row(4)) + mod_row(3)
        ops = _strassen_lhs(hn[0:R, 0:D // 2], hn[0:R, D // 2:D], hn[R:_FM, 0:D // 2],
                            hn[R:_FM, D // 2:D])
        for k, v in enumerate(ops):
            h2[slot, k] = pltpu.bitcast(v, U32)

    def ffn(i, carry):
        def hidden(c0):
            prods = [_mm(pltpu.bitcast(h2[i % 2, k], BF16),
                         pltpu.bitcast(wu[_RHS[k], :, pl.ds(c0, _FC)], BF16)) for k in range(7)]
            g1, u1, g2, u2 = _strassen_out(prods)
            return g1 * jax.nn.sigmoid(g1) * u1, g2 * jax.nn.sigmoid(g2) * u2

        nf = F // 2 // _FC
        acc = [None] * 7
        ops = None
        for f in range(nf + 1):
            prev = ops
            if f < nf:
                a11, a21 = hidden(f * _FC)
                a12, a22 = hidden(F // 2 + f * _FC)
                ops = _strassen_lhs(a11, a12, a21, a22)
            if f > 0:
                rows = pl.ds((f - 1) * _FC // 2, _FC // 2)
                for k in range(7):
                    part = _mm(prev[k], pltpu.bitcast(wd[_RHS[k], rows, :], BF16))
                    acc[k] = part if acc[k] is None else acc[k] + part
        c11, c12, c21, c22 = _strassen_out(acc)
        down = jnp.concatenate([jnp.concatenate([c11, c12], axis=1),
                                jnp.concatenate([c21, c22], axis=1)], axis=0)
        y = residual(i) + mod_row(5) * down
        ybuf[pl.ds(i * spb, spb)] = y.astype(ybuf.dtype).reshape(spb, seg, D)
        ln2(jnp.minimum(i + 1, n_blk - 1), (i + 1) % 2)
        out_cp(i).start()
        return carry

    ln2(0, 0)
    lax.fori_loop(0, n_blk, ffn, 0)
    for i in range(n_blk):
        out_cp(i).wait()


@functools.partial(jax.jit, static_argnames=("A_seg_len",))
def pallas_adaLN_cond__memory_aug_recurrent_mem_tr__glu_gated_swiglu__prompt_kernel(
        A_x, A_mem0, A_Wq, A_Wk, A_Wv, A_Wo, A_seg_len, B_x, B_w1, B_w3, B_w2, c, w_mod):
    del B_x
    B, S, D = A_x.shape
    _, H, Dh = A_Wq.shape
    M = A_mem0.shape[1]
    F = B_w1.shape[1]
    seg = int(A_seg_len)
    assert B == 1 and S % seg == 0 and S % _FM == 0 and F % (2 * _FC) == 0
    L = M + seg
    hbm = pl.BlockSpec(memory_space=pl.ANY)
    vmem = pl.BlockSpec(memory_space=pltpu.VMEM)
    dma = pltpu.SemaphoreType.DMA
    n_seg = S // seg
    out = pl.pallas_call(
        functools.partial(_body, H=H, Dh=Dh),
        out_shape=jax.ShapeDtypeStruct((n_seg, seg, D), A_x.dtype),
        in_specs=[hbm, vmem, hbm, hbm, hbm, hbm, hbm, hbm, hbm, vmem, hbm],
        out_specs=hbm,
        scratch_shapes=[
            pltpu.VMEM((n_seg, seg, D), BF16),
            pltpu.VMEM((n_seg, _TAIL, D), BF16),
            pltpu.VMEM((4 * D // _MC, D // 2, _MC), U32),
            pltpu.VMEM((H, D // 2, Dh), U32),
            pltpu.VMEM((H, D // 2, Dh), U32),
            pltpu.VMEM((H, D // 2, Dh), U32),
            pltpu.VMEM((H * Dh // 2, D), U32),
            pltpu.VMEM((7, D // 4, F + 128), U32),
            pltpu.VMEM((7, F // 4 + 32, D // 2), U32),
            pltpu.VMEM((8, 6 * D), F32),
            pltpu.VMEM((n_seg, seg, D), F32),
            pltpu.VMEM((n_seg * _TAIL // 2, D), U32),
            pltpu.VMEM((3, H, n_seg * _TAIL, Dh), F32),
            pltpu.VMEM((L, D), F32),
            pltpu.VMEM((L, H * Dh), F32),
            pltpu.VMEM((2, 7, _FM // 4, D // 2), U32),
            pltpu.VMEM((n_seg, seg, D), A_x.dtype),
            dma((3,)), dma((6 * D // _MC,)), dma((3 * H,)), dma((H // 2,)), dma((8,)), dma((S // _FM,)),
        ],
        compiler_params=pltpu.CompilerParams(vmem_limit_bytes=127 * 1024 * 1024, disable_bounds_checks=_NOBC),
    )(A_x.reshape(n_seg, seg, D), A_mem0.reshape(M, D), A_Wq.reshape(D // 2, 2 * H, Dh),
      A_Wk.reshape(D // 2, 2 * H, Dh), A_Wv.reshape(D // 2, 2 * H, Dh), A_Wo.reshape(H * Dh, D),
      B_w1, B_w3, B_w2, c, w_mod)
    return out.reshape(B, S, D)
```

```python
import functools

import jax
import jax.numpy as jnp
from jax import lax
import jax.experimental.pallas as pl
import jax.experimental.pallas.tpu as pltpu

F32 = jnp.float32
BF16 = jnp.bfloat16
U32 = jnp.uint32

_HG = 4
_FM = 128
_FC = 896
_TAIL = 8
_LAG = 1
_CR = 16
_XA = 10
_AE = 3
_PU = 1
_TPOS = (0, 2)
_NOBC = True
_MC = 512


def _mm(a, b):
    return lax.dot_general(a, b, (((1,), (0,)), ((), ())), preferred_element_type=F32)


def _mm_nt(a, b):
    return lax.dot_general(a, b, (((1,), (1,)), ((), ())), preferred_element_type=F32)


def _normalize(x):
    m = jnp.mean(x, axis=-1, keepdims=True)
    d = x - m
    v = jnp.mean(d * d, axis=-1, keepdims=True)
    return d * lax.rsqrt(v + 1e-5)


def _unpack(words):
    return (lax.bitcast_convert_type(words << 16, F32),
            lax.bitcast_convert_type(words & jnp.uint32(0xFFFF0000), F32))


def _pack(lo, hi):
    return pltpu.pack_elementwise([lo, hi], packed_dtype=BF16)


def _strassen_rhs(b11, b12, b21, b22):
    return b11 + b22, b12 - b22, b21 - b11, b11 + b12, b21 + b22


def _rhs_refs(raw, sums):
    return sums.at[0], raw.at[0], sums.at[1], sums.at[2], raw.at[3], sums.at[3], sums.at[4]


def _strassen_lhs(a11, a12, a21, a22):
    return [v.astype(BF16) for v in
            (a11 + a22, a21 + a22, a11, a22, a11 + a12, a21 - a11, a12 - a22)]


def _strassen_out(p):
    return p[0] + p[3] - p[4] + p[6], p[2] + p[4], p[1] + p[3], p[0] - p[1] + p[2] + p[5]


def _body(x_hbm, mem0_ref, wq_hbm, wk_hbm, wv_hbm, wo_hbm, w1_hbm, w3_hbm, w2_hbm, c_ref,
          wmod_hbm, out_hbm,
          xs, xt, wmod, wq, wk, wv, wo, wu, wd, wus, wds, mod, att, ht, pre, hbuf, obuf, h2, ybuf,
          sem_x, sem_mod, sem_w, sem_o, sem_f, sem_out, *, H, Dh):
    n_seg, seg, D = xs.shape
    M = mem0_ref.shape[0]
    L = M + seg
    F = w1_hbm.shape[1]
    HP = H // 2
    T = _TAIL
    spb = _FM // seg
    n_blk = n_seg // spb

    n_slot = wmod.shape[0]

    def mod_cp(j):
        cols = pl.ds(j * _MC, _MC)
        return pltpu.make_async_copy(wmod_hbm.bitcast(U32).at[:, cols], wmod.at[j % n_slot], sem_mod.at[j])

    xa_cp = pltpu.make_async_copy(x_hbm.at[pl.ds(0, _XA)], xs.at[pl.ds(0, _XA)], sem_x.at[0])
    xb_cp = pltpu.make_async_copy(x_hbm.at[pl.ds(_XA, n_seg - _XA)],
                                  xs.at[pl.ds(_XA, n_seg - _XA)], sem_x.at[1])
    xt_cp = pltpu.make_async_copy(x_hbm.at[:, pl.ds(seg - T, T), :], xt, sem_x.at[2])
    w_hbms = (wq_hbm, wk_hbm, wv_hbm)
    wqkv = (wq, wk, wv)

    def w_cp(m, i, odd):
        src = w_hbms[m].bitcast(U32).at[:, odd * HP + i, :]
        return pltpu.make_async_copy(src, wqkv[m].at[2 * i + odd], sem_w.at[m * H + 2 * i + odd])

    def wo_cp(i):
        rows = pl.ds(pl.multiple_of(i * Dh, Dh), Dh)
        return pltpu.make_async_copy(wo_hbm.bitcast(U32).at[rows], wo.at[rows], sem_o.at[i])

    w1_w, w3_w, w2_w = (r.bitcast(U32) for r in (w1_hbm, w3_hbm, w2_hbm))
    lo, hi = pl.ds(0, D // 4), pl.ds(D // 4, D // 4)
    f_srcs = [(wu.at[k, :, pl.ds(0, F)], src.at[rows]) for k, (src, rows) in
              enumerate(((w1_w, lo), (w3_w, lo), (w1_w, hi), (w3_w, hi)))]
    f_srcs += [(wd.at[2 * r + q, pl.ds(0, F // 4)],
                w2_w.at[pl.ds(r * F // 4, F // 4), pl.ds(q * D // 2, D // 2)])
               for r in range(2) for q in range(2)]
    f_cps = [pltpu.make_async_copy(src, dst, sem_f.at[n])
             for n, (dst, src) in enumerate(f_srcs)]

    def start_pair(ms, i):
        for m in ms:
            w_cp(m, i, 0).start()
            w_cp(m, i, 1).start()

    def wait_pair(ms, i):
        for m in ms:
            w_cp(m, i, 0).wait()
            w_cp(m, i, 1).wait()

    def retile(m, i):
        a = wqkv[m][2 * i]
        b = wqkv[m][2 * i + 1]
        even = (a & jnp.uint32(0xFFFF)) | (b << 16)
        odd = (a >> 16) | (b & jnp.uint32(0xFFFF0000))
        wqkv[m][2 * i] = even
        wqkv[m][2 * i + 1] = odd
        halves = [_strassen_rhs(*_unpack(w[0:D // 4]), *_unpack(w[D // 4:D // 2])) for w in (a, b)]
        sums = [_pack(lo_v, hi_v) for lo_v, hi_v in zip(*halves)]
        return sums[0], even[0:D // 4], sums[1], sums[2], odd[D // 4:D // 2], sums[3], sums[4]

    def w_tile(m, hd):
        return pltpu.bitcast(wqkv[m][hd], BF16)

    qkv = (0, 1, 2)
    n_mod_a = 2 * D // _MC
    xt_cp.start()
    for j in range(n_mod_a):
        mod_cp(j).start()

    cv = c_ref[...].astype(F32)
    sc = jnp.broadcast_to(cv * jax.nn.sigmoid(cv), (8, D))

    def mod_part(j):
        mod[:, pl.ds(j * _MC, _MC)] = _mm(sc, pltpu.bitcast(wmod[j % n_slot], BF16))

    def mod_row(j):
        return mod[0:1, pl.ds(j * D, D)]

    def ln1(xv):
        return _normalize(xv.astype(F32)) * (1.0 + mod_row(1)) + mod_row(0)

    xt_cp.wait()
    start_pair(qkv, 0)
    att[0:n_seg * T // seg] = _normalize(xt[...].astype(F32).reshape(n_seg * T, D)).reshape(-1, seg, D)
    for j in range(n_mod_a):
        mod_cp(j).wait()
        if j == n_mod_a - 1:
            start_pair(qkv, 1)
        mod_part(j)
    hn = (att[0:n_seg * T // seg].reshape(n_seg * T, D) * (1.0 + mod_row(1))
          + mod_row(0)).reshape(n_seg // 2, 2 * T, D)
    h_ev = hn[:, 0:T].reshape(n_seg // 2 * T, D)
    h_od = hn[:, T:2 * T].reshape(n_seg // 2 * T, D)
    for k, v in enumerate(_strassen_lhs(h_ev[:, 0:D // 2], h_ev[:, D // 2:D],
                                        h_od[:, 0:D // 2], h_od[:, D // 2:D])):
        ht[k] = pltpu.bitcast(v, U32)
    for i in range(2, _AE):
        start_pair(qkv, i)
    xa_cp.start()
    wo_cp(0).start()

    def arrive(j, carry):
        def traffic():
            for u in range(_PU):
                i = j * _PU + u
                pl.when(i + _AE < HP)(functools.partial(start_pair, qkv, i + _AE))
                pl.when(i + 1 < HP)(lambda i=i: wo_cp(i + 1).start())
            for u in range(_PU):
                i = (j + 1) * _PU + u
                pl.when(i < HP)(functools.partial(wait_pair, qkv, i))

        for u in range(_PU):
            i = j * _PU + u
            for m in qkv:
                rhs = retile(m, i)
                p = [_mm(pltpu.bitcast(ht[k], BF16), pltpu.bitcast(rhs[k], BF16))
                     for k in range(7)]
                c11, c12, c21, c22 = _strassen_out(p)
                if (u, m) == _TPOS:
                    traffic()
                pre[m, 2 * i] = _pack(c11, c21)
                pre[m, 2 * i + 1] = _pack(c12, c22)
        return carry

    for i in range(_PU):
        wait_pair(qkv, i)
    lax.fori_loop(0, HP // _PU, arrive, 0)
    xb_cp.start()
    xa_cp.wait()
    hbuf[0:M] = mem0_ref[...].astype(F32)
    hbuf[M:L] = ln1(xs[0])
    for i in range(HP):
        wo_cp(i).wait()
    for cp in f_cps:
        cp.start()

    scale = Dh ** -0.5
    NG = H // _HG

    def step(j, u, jobs):
        s = 2 * j + u
        row = lax.broadcasted_iota(jnp.int32, (L, L), 0)
        col = lax.broadcasted_iota(jnp.int32, (L, L), 1)
        mask = (row < M) | (row >= col)
        h = hbuf[0:L - T]
        tail = pl.ds(pl.multiple_of(j * T, T), T)

        def proj(m, g):
            heads = range(g * _HG, (g + 1) * _HG)
            w = jnp.concatenate([w_tile(m, hd) for hd in heads], axis=1)
            r = _mm(h, w)
            r = [r[:, j * Dh:(j + 1) * Dh] for j in range(_HG)]
            return [jnp.concatenate([r[n], _unpack(pre[m, hd, tail, :])[u]], axis=0)
                    for n, hd in enumerate(heads)]

        def probs(qs, ks):
            res = []
            for q, k in zip(qs, ks):
                sco = jnp.where(mask, _mm_nt(q, k.astype(BF16)) * scale, -1e9)
                e = jnp.exp(sco - jnp.max(sco, axis=-1, keepdims=True))
                res.append((e, 1.0 / jnp.sum(e, axis=-1, keepdims=True)))
            return res

        def mix(g, ps, vs):
            for j, ((e, inv), v) in enumerate(zip(ps, vs)):
                obuf[:, pl.ds((g * _HG + j) * Dh, Dh)] = _mm(e, v.astype(BF16)) * inv

        def out_proj(g, acc):
            kk = _HG * Dh
            part = _mm(obuf[:, pl.ds(g * kk, kk)],
                       pltpu.bitcast(wo[pl.ds(g * kk // 2, kk // 2), :], BF16))
            return part if acc is None else acc + part

        acc = ps = vs = None
        for g in range(-1, NG):
            if g + 1 < NG:
                qs, ks = proj(0, g + 1), proj(1, g + 1)
            if g >= 0:
                mix(g, ps, vs)
            if g + 1 < NG:
                vs = proj(2, g + 1)
                ps = probs(qs, ks)
                for n, job in enumerate(jobs[g + 1::NG]):
                    job((vs, ks, qs)[n % 3][n // 3 % _HG][0:8])
            if g >= _LAG:
                acc = out_proj(g - _LAG, acc)
        for g in range(NG - _LAG, NG):
            acc = out_proj(g, acc)

        hbuf[M:L] = ln1(xs[jnp.minimum(s + 1, n_seg - 1)])
        hbuf[0:M] = acc[0:M]
        att[s] = acc[M:L]

    n_it = n_seg // 2
    n_sl = F // 128
    rd = F // 4 // n_sl
    for k in range(4):
        wu[k, :, pl.ds(F, 128)] = jnp.zeros((D // 4, 128), U32)
        wd[k, pl.ds(F // 4, rd), :] = jnp.zeros((rd, D // 2), U32)

    def combine(raw, sums, idx, anchor):
        raw[0, raw.shape[1] - 8:, raw.shape[2] - 128:] = lax.bitcast_convert_type(anchor, U32)
        halves = zip(*(_unpack(raw[(k,) + idx]) for k in range(4)))
        for k, (lo_v, hi_v) in enumerate(zip(*(_strassen_rhs(*b) for b in halves))):
            sums[(k,) + idx] = _pack(lo_v, hi_v)

    def steps(j, carry):
        sl = jnp.where(j < n_it - n_sl, n_sl, j - (n_it - n_sl))
        cols = pl.ds(pl.multiple_of(sl * 128, 128), 128)
        jobs = [functools.partial(combine, wu, wus, (pl.ds(r, _CR), cols))
                for r in range(0, D // 4, _CR)]
        jobs += [functools.partial(combine, wd, wds, (pl.ds(pl.multiple_of(sl * rd + r, 8), 8),
                                                 slice(None))) for r in range(0, rd, 8)]
        for u in range(2):
            step(j, u, jobs[u::2])
        return carry

    def phase(ph, carry):
        @pl.when(ph == 1)
        def _():
            xb_cp.wait()
            for cp in f_cps:
                cp.wait()
            for n in range(n_mod_a, 6 * D // _MC):
                mod_cp(n).start()

        return lax.fori_loop(ph * (n_it - n_sl), n_it - n_sl + ph * n_sl, steps, carry)

    lax.fori_loop(0, 2, phase, 0)

    for j in range(n_mod_a, 6 * D // _MC):
        mod_cp(j).wait()
    for j in range(n_mod_a, 6 * D // _MC):
        mod_part(j)

    def out_cp(i):
        blk = pl.ds(i * spb, spb)
        return pltpu.make_async_copy(ybuf.at[blk], out_hbm.at[blk], sem_out.at[i])

    def residual(i):
        blk = pl.ds(i * spb, spb)
        return xs[blk].astype(F32).reshape(_FM, D) + mod_row(2) * att[blk].reshape(_FM, D)

    R = _FM // 2

    def ln2(i, slot):
        hn = _normalize(residual(i)) * (1.0 + mod_row(4)) + mod_row(3)
        ops = _strassen_lhs(hn[0:R, 0:D // 2], hn[0:R, D // 2:D], hn[R:_FM, 0:D // 2],
                            hn[R:_FM, D // 2:D])
        for k, v in enumerate(ops):
            h2[slot, k] = pltpu.bitcast(v, U32)

    def ffn(i, carry):
        def hidden(c0):
            prods = [_mm(pltpu.bitcast(h2[i % 2, k], BF16),
                         pltpu.bitcast(_rhs_refs(wu, wus)[k][:, pl.ds(c0, _FC)], BF16)) for k in range(7)]
            g1, u1, g2, u2 = _strassen_out(prods)
            return g1 * jax.nn.sigmoid(g1) * u1, g2 * jax.nn.sigmoid(g2) * u2

        nf = F // 2 // _FC
        acc = [None] * 7
        ops = None
        for f in range(nf + 1):
            prev = ops
            if f < nf:
                a11, a21 = hidden(f * _FC)
                a12, a22 = hidden(F // 2 + f * _FC)
                ops = _strassen_lhs(a11, a12, a21, a22)
            if f > 0:
                rows = pl.ds((f - 1) * _FC // 2, _FC // 2)
                for k in range(7):
                    part = _mm(prev[k], pltpu.bitcast(_rhs_refs(wd, wds)[k][rows, :], BF16))
                    acc[k] = part if acc[k] is None else acc[k] + part
        c11, c12, c21, c22 = _strassen_out(acc)
        down = jnp.concatenate([jnp.concatenate([c11, c12], axis=1),
                                jnp.concatenate([c21, c22], axis=1)], axis=0)
        y = residual(i) + mod_row(5) * down
        ybuf[pl.ds(i * spb, spb)] = y.astype(ybuf.dtype).reshape(spb, seg, D)
        ln2(jnp.minimum(i + 1, n_blk - 1), (i + 1) % 2)
        out_cp(i).start()
        return carry

    ln2(0, 0)
    lax.fori_loop(0, n_blk, ffn, 0)
    for i in range(n_blk):
        out_cp(i).wait()


@functools.partial(jax.jit, static_argnames=("A_seg_len",))
def pallas_adaLN_cond__memory_aug_recurrent_mem_tr__glu_gated_swiglu__prompt_kernel(
        A_x, A_mem0, A_Wq, A_Wk, A_Wv, A_Wo, A_seg_len, B_x, B_w1, B_w3, B_w2, c, w_mod):
    del B_x
    B, S, D = A_x.shape
    _, H, Dh = A_Wq.shape
    M = A_mem0.shape[1]
    F = B_w1.shape[1]
    seg = int(A_seg_len)
    assert B == 1 and S % seg == 0 and S % _FM == 0 and F % (2 * _FC) == 0
    L = M + seg
    hbm = pl.BlockSpec(memory_space=pl.ANY)
    vmem = pl.BlockSpec(memory_space=pltpu.VMEM)
    dma = pltpu.SemaphoreType.DMA
    n_seg = S // seg
    out = pl.pallas_call(
        functools.partial(_body, H=H, Dh=Dh),
        out_shape=jax.ShapeDtypeStruct((n_seg, seg, D), A_x.dtype),
        in_specs=[hbm, vmem, hbm, hbm, hbm, hbm, hbm, hbm, hbm, vmem, hbm],
        out_specs=hbm,
        scratch_shapes=[
            pltpu.VMEM((n_seg, seg, D), BF16),
            pltpu.VMEM((n_seg, _TAIL, D), BF16),
            pltpu.VMEM((4 * D // _MC, D // 2, _MC), U32),
            pltpu.VMEM((H, D // 2, Dh), U32),
            pltpu.VMEM((H, D // 2, Dh), U32),
            pltpu.VMEM((H, D // 2, Dh), U32),
            pltpu.VMEM((H * Dh // 2, D), U32),
            pltpu.VMEM((4, D // 4, F + 128), U32),
            pltpu.VMEM((4, F // 4 + 32, D // 2), U32),
            pltpu.VMEM((5, D // 4, F + 128), U32),
            pltpu.VMEM((5, F // 4 + 32, D // 2), U32),
            pltpu.VMEM((8, 6 * D), F32),
            pltpu.VMEM((n_seg, seg, D), F32),
            pltpu.VMEM((7, n_seg * _TAIL // 4, D // 2), U32),
            pltpu.VMEM((3, H, n_seg * _TAIL // 2, Dh), U32),
            pltpu.VMEM((L, D), F32),
            pltpu.VMEM((L, H * Dh), F32),
            pltpu.VMEM((2, 7, _FM // 4, D // 2), U32),
            pltpu.VMEM((n_seg, seg, D), A_x.dtype),
            dma((3,)), dma((6 * D // _MC,)), dma((3 * H,)), dma((H // 2,)), dma((8,)), dma((S // _FM,)),
        ],
        compiler_params=pltpu.CompilerParams(vmem_limit_bytes=127 * 1024 * 1024, disable_bounds_checks=_NOBC),
    )(A_x.reshape(n_seg, seg, D), A_mem0.reshape(M, D), A_Wq.reshape(D // 2, 2 * H, Dh),
      A_Wk.reshape(D // 2, 2 * H, Dh), A_Wv.reshape(D // 2, 2 * H, Dh), A_Wo.reshape(H * Dh, D),
      B_w1, B_w3, B_w2, c, w_mod)
    return out.reshape(B, S, D)
```

```python
import functools

import jax
import jax.numpy as jnp
from jax import lax
import jax.experimental.pallas as pl
import jax.experimental.pallas.tpu as pltpu

_LOG2E = 1.4426950408889634
F32 = jnp.float32
BF16 = jnp.bfloat16
U32 = jnp.uint32

_HG = 4
_FM = 128
_FC = 896
_TAIL = 8
_LAG = 2
_ORDER = 'kqovpmj'
_ANCH = 'q'
_CR = 8
_LR = 8
_LS = 3
_XA = 10
_AE = 3
_PORD = (1, 4, 0, 2, 3, 5, 6)
_NOBC = True
_MC = 512


def _mm(a, b):
    return lax.dot_general(a, b, (((1,), (0,)), ((), ())), preferred_element_type=F32)


def _mm_nt(a, b):
    return lax.dot_general(a, b, (((1,), (1,)), ((), ())), preferred_element_type=F32)


def _normalize(x):
    m = jnp.mean(x, axis=-1, keepdims=True)
    d = x - m
    v = jnp.mean(d * d, axis=-1, keepdims=True)
    return d * lax.rsqrt(v + 1e-5)


def _silu(x):
    half = 0.5 * x
    return half * jnp.tanh(half) + half


def _unpack(words):
    return (lax.bitcast_convert_type(words << 16, F32),
            lax.bitcast_convert_type(words & jnp.uint32(0xFFFF0000), F32))


def _pack(lo, hi):
    return pltpu.pack_elementwise([lo, hi], packed_dtype=BF16)


def _strassen_rhs(b11, b12, b21, b22):
    return b11 + b22, b12 - b22, b21 - b11, b11 + b12, b21 + b22


def _rhs_refs(raw, sums):
    return sums.at[0], raw.at[0], sums.at[1], sums.at[2], raw.at[3], sums.at[3], sums.at[4]


def _strassen_lhs(a11, a12, a21, a22):
    return a11 + a22, a21 + a22, a11, a22, a11 + a12, a21 - a11, a12 - a22


def _strassen_out(p):
    return p[0] + p[3] - p[4] + p[6], p[2] + p[4], p[1] + p[3], p[0] - p[1] + p[2] + p[5]


def _body(x_hbm, mem0_ref, wq_hbm, wk_hbm, wv_hbm, wo_hbm, w1_hbm, w3_hbm, w2_hbm, c_ref,
          wmod_hbm, out_hbm,
          xs, xt, wmod, wq, wk, wv, wo, wu, wd, wus, wds, mod, att, ht, pre, hbuf, obuf, h2, ybuf,
          sem_x, sem_mod, sem_w, sem_o, sem_f, sem_out, *, H, Dh):
    n_seg, seg, D = xs.shape
    M = mem0_ref.shape[0]
    L = M + seg
    F = w1_hbm.shape[1]
    HP = H // 2
    T = _TAIL
    spb = _FM // seg
    n_blk = n_seg // spb

    n_slot = wmod.shape[0]
    n_mod_a = 2 * D // _MC

    def mod_cp(j):
        cols = pl.ds(j * _MC, _MC)
        return pltpu.make_async_copy(wmod_hbm.bitcast(U32).at[:, cols], wmod.at[j % n_slot], sem_mod.at[min(j, n_mod_a)])

    xa_cp = pltpu.make_async_copy(x_hbm.at[pl.ds(0, _XA)], xs.at[pl.ds(0, _XA)], sem_x.at[0])
    xb_cp = pltpu.make_async_copy(x_hbm.at[pl.ds(_XA, n_seg - _XA)],
                                  xs.at[pl.ds(_XA, n_seg - _XA)], sem_x.at[1])
    xt_cp = pltpu.make_async_copy(x_hbm.at[:, pl.ds(seg - T, T), :], xt, sem_x.at[2])
    w_hbms = (wq_hbm, wk_hbm, wv_hbm)
    wqkv = (wq, wk, wv)

    def w_cp(m, i, odd):
        src = w_hbms[m].bitcast(U32).at[:, odd * HP + i, :]
        return pltpu.make_async_copy(src, wqkv[m].at[2 * i + odd], sem_w.at[i])

    def wo_cp(i):
        rows = pl.ds(pl.multiple_of(i * Dh, Dh), Dh)
        return pltpu.make_async_copy(wo_hbm.bitcast(U32).at[rows], wo.at[rows], sem_o)

    w1_w, w3_w, w2_w = (r.bitcast(U32) for r in (w1_hbm, w3_hbm, w2_hbm))
    lo, hi = pl.ds(0, D // 4), pl.ds(D // 4, D // 4)
    f_srcs = [(wu.at[k, :, pl.ds(0, F)], src.at[rows]) for k, (src, rows) in
              enumerate(((w1_w, lo), (w3_w, lo), (w1_w, hi), (w3_w, hi)))]
    f_srcs += [(wd.at[2 * r + q, pl.ds(0, F // 4)],
                w2_w.at[pl.ds(r * F // 4, F // 4), pl.ds(q * D // 2, D // 2)])
               for r in range(2) for q in range(2)]
    f_cps = [pltpu.make_async_copy(src, dst, sem_f) for dst, src in f_srcs]

    def start_pair(ms, i):
        for m in ms:
            w_cp(m, i, 0).start()
            w_cp(m, i, 1).start()

    def wait_pair(ms, i):
        for m in ms:
            w_cp(m, i, 0).wait()
            w_cp(m, i, 1).wait()

    def retile(m, i):
        a = wqkv[m][2 * i]
        b = wqkv[m][2 * i + 1]
        even = (a & jnp.uint32(0xFFFF)) | (b << 16)
        odd = (a >> 16) | (b & jnp.uint32(0xFFFF0000))
        wqkv[m][2 * i] = even
        wqkv[m][2 * i + 1] = odd
        halves = [_strassen_rhs(*_unpack(w[0:D // 4]), *_unpack(w[D // 4:D // 2])) for w in (a, b)]
        sums = [_pack(lo_v, hi_v) for lo_v, hi_v in zip(*halves)]
        return sums[0], even[0:D // 4], sums[1], sums[2], odd[D // 4:D // 2], sums[3], sums[4]

    def w_tile(m, hd):
        return pltpu.bitcast(wqkv[m][hd], BF16)

    qkv = (0, 1, 2)
    xt_cp.start()
    for j in range(n_mod_a):
        mod_cp(j).start()

    cv = c_ref[...].astype(F32)
    sc = jnp.broadcast_to(cv * jax.nn.sigmoid(cv), (8, D))

    def mod_part(j):
        mod[:, pl.ds(j * _MC, _MC)] = _mm(sc, pltpu.bitcast(wmod[j % n_slot], BF16))

    def mod_row(j):
        return mod[0:1, pl.ds(j * D, D)]

    def ln1(xv):
        return _normalize(xv.astype(F32)) * (1.0 + mod_row(1)) + mod_row(0)

    xt_cp.wait()
    start_pair(qkv, 0)
    att[0:n_seg * T // seg] = _normalize(xt[...].astype(F32).reshape(n_seg * T, D)).reshape(-1, seg, D)
    for j in range(n_mod_a):
        mod_cp(j).wait()
        if j == n_mod_a - 1:
            start_pair(qkv, 1)
        mod_part(j)
    hn = (att[0:n_seg * T // seg].reshape(n_seg * T, D) * (1.0 + mod_row(1))
          + mod_row(0)).reshape(n_seg // 2, 2 * T, D)
    h_ev = hn[:, 0:T].reshape(n_seg // 2 * T, D)
    h_od = hn[:, T:2 * T].reshape(n_seg // 2 * T, D)
    for k, v in enumerate(_strassen_lhs(h_ev[:, 0:D // 2], h_ev[:, D // 2:D],
                                        h_od[:, 0:D // 2], h_od[:, D // 2:D])):
        ht[k] = v
    for i in range(2, _AE):
        start_pair(qkv, i)
    xa_cp.start()
    wo_cp(0).start()

    def arrive(i, carry):
        for m in qkv:
            rhs = retile(m, i)
            p = {k: _mm(ht[k], pltpu.bitcast(rhs[k], BF16)) for k in _PORD}
            c11, c12, c21, c22 = _strassen_out(p)
            if m == qkv[-1]:
                pl.when(i + _AE < HP)(functools.partial(start_pair, qkv, i + _AE))

                @pl.when(i + 1 < HP)
                def _():
                    wo_cp(i + 1).start()
                    wait_pair(qkv, i + 1)

            pre[m, 2 * i] = _pack(c11, c21)
            pre[m, 2 * i + 1] = _pack(c12, c22)
        return carry

    wait_pair(qkv, 0)
    lax.fori_loop(0, HP, arrive, 0)
    xb_cp.start()
    xa_cp.wait()
    hbuf[0:M] = mem0_ref[...].astype(F32)
    hbuf[M:L] = ln1(xs[0])
    for i in range(HP):
        wo_cp(i).wait()
    for cp in f_cps:
        cp.start()

    scale = Dh ** -0.5
    NG = H // _HG

    def step(j, u, jobs):
        s = 2 * j + u
        row = lax.broadcasted_iota(jnp.int32, (L, L), 0)
        col = lax.broadcasted_iota(jnp.int32, (L, L), 1)
        mask = (row < M) | (row >= col)
        h = hbuf[0:L - T]
        tail = pl.ds(pl.multiple_of(j * T, T), T)

        def proj(m, g):
            heads = range(g * _HG, (g + 1) * _HG)
            w = jnp.concatenate([w_tile(m, hd) for hd in heads], axis=1)
            r = _mm(h, w)
            r = [r[:, j * Dh:(j + 1) * Dh] for j in range(_HG)]
            return [jnp.concatenate([r[n], _unpack(pre[m, hd, tail, :])[u]], axis=0)
                    for n, hd in enumerate(heads)]

        def probs(qs, ks):
            res = []
            for q, k in zip(qs, ks):
                sco = jnp.where(mask, _mm_nt(q, k.astype(BF16)) * (scale * _LOG2E), -1e9 * _LOG2E)
                e = jnp.exp2(sco - jnp.max(sco, axis=-1, keepdims=True))
                den = jnp.sum(e, axis=-1, keepdims=True)
                res.append((e, pl.reciprocal(den, full_range=False)))
            return res

        def mix(g, ps, vs):
            for j, ((e, inv), v) in enumerate(zip(ps, vs)):
                obuf[:, pl.ds((g * _HG + j) * Dh, Dh)] = _mm(e, v.astype(BF16)) * inv

        def out_proj(g, acc):
            kk = _HG * Dh
            part = _mm(obuf[:, pl.ds(g * kk, kk)],
                       pltpu.bitcast(wo[pl.ds(g * kk // 2, kk // 2), :], BF16))
            return part if acc is None else acc + part

        acc = None
        val = {}
        for g in range(-1, NG):
            for op in _ORDER:
                if op in "qkv" and g + 1 < NG:
                    val[op, g + 1] = proj("qkv".index(op), g + 1)
                elif op == "p" and g + 1 < NG:
                    val[op, g + 1] = probs(val["q", g + 1], val["k", g + 1])
                elif op == "j" and g + 1 < NG:
                    for n, job in enumerate(jobs[g + 1::NG]):
                        job(val[_ANCH[n % len(_ANCH)], g + 1][n % _HG][0:8])
                elif op == "m" and g >= 0:
                    mix(g, val["p", g], val["v", g])
                elif op == "o" and g >= _LAG:
                    acc = out_proj(g - _LAG, acc)
        for g in range(NG - _LAG, NG):
            acc = out_proj(g, acc)

        hbuf[M:L] = ln1(xs[jnp.minimum(s + 1, n_seg - 1)])
        hbuf[0:M] = acc[0:M]
        att[s] = acc[M:L]

    n_it = n_seg // 2
    n_sl = F // 128
    rd = F // 4 // n_sl
    for k in range(4):
        wu[k, :, pl.ds(F, 128)] = jnp.zeros((D // 4, 128), U32)
        wd[k, pl.ds(F // 4, rd), :] = jnp.zeros((rd, D // 2), U32)

    def combine(raw, sums, idx, anchor):
        raw[0, raw.shape[1] - 8:, raw.shape[2] - 128:] = lax.bitcast_convert_type(anchor, U32)
        halves = zip(*(_unpack(raw[(k,) + idx]) for k in range(4)))
        for k, (lo_v, hi_v) in enumerate(zip(*(_strassen_rhs(*b) for b in halves))):
            sums[(k,) + idx] = _pack(lo_v, hi_v)

    def steps(j, carry):
        sl = jnp.where(j < n_it - n_sl, n_sl, j - (n_it - n_sl))
        cols = pl.ds(pl.multiple_of(sl * 128, 128), 128)
        jobs = [functools.partial(combine, wu, wus, (pl.ds(r, _CR), cols))
                for r in range(0, D // 4, _CR)]
        jobs += [functools.partial(combine, wd, wds, (pl.ds(pl.multiple_of(sl * rd + r, 8), 8),
                                                 slice(None))) for r in range(0, rd, 8)]
        for u in range(2):
            step(j, u, jobs[u::2])
        return carry

    def phase(ph, carry):
        @pl.when(ph == 1)
        def _():
            xb_cp.wait()
            for cp in f_cps:
                cp.wait()
            for n in range(n_mod_a, 6 * D // _MC):
                mod_cp(n).start()

        return lax.fori_loop(ph * (n_it - n_sl), n_it - n_sl + ph * n_sl, steps, carry)

    lax.fori_loop(0, 2, phase, 0)

    for j in range(n_mod_a, 6 * D // _MC):
        mod_cp(j).wait()
    for j in range(n_mod_a, 6 * D // _MC):
        mod_part(j)

    def out_cp(i):
        blk = pl.ds(i * spb, spb)
        return pltpu.make_async_copy(ybuf.at[i % 2], out_hbm.at[blk], sem_out.at[i % 2])

    def residual(i):
        blk = pl.ds(i * spb, spb)
        return xs[blk].astype(F32).reshape(_FM, D) + mod_row(2) * att[blk].reshape(_FM, D)

    R = _FM // 2

    def ln2(i, slot, r):
        top, bot = (
            _normalize(xs[sg, rows, :].astype(F32) + mod_row(2) * att[sg, rows, :])
            * (1.0 + mod_row(4)) + mod_row(3)
            for sg, rows in ((i * spb + q // seg, pl.ds(q % seg, _LR)) for q in (r, R + r)))
        ops = _strassen_lhs(top[:, 0:D // 2], top[:, D // 2:D], bot[:, 0:D // 2], bot[:, D // 2:D])
        for k, v in enumerate(ops):
            h2[slot, k, pl.ds(r, _LR), :] = v

    def ffn(i, carry):
        pl.when(i >= 2)(lambda: out_cp(i - 2).wait())
        pieces = list(range(0, R, _LR))
        count = [0]

        def hidden(c0):
            prods = []
            for k in range(7):
                count[0] += 1
                if count[0] % _LS == 0 and pieces:
                    ln2(jnp.minimum(i + 1, n_blk - 1), (i + 1) % 2, pieces.pop())
                prods.append(_mm(h2[i % 2, k],
                                 pltpu.bitcast(_rhs_refs(wu, wus)[k][:, pl.ds(c0, _FC)], BF16)))
            g1, u1, g2, u2 = _strassen_out(prods)
            return _silu(g1) * u1, _silu(g2) * u2

        nf = F // 2 // _FC
        acc = [None] * 7
        ops = None
        for f in range(nf + 1):
            prev = ops
            if f < nf:
                a11, a21 = hidden(f * _FC)
                a12, a22 = hidden(F // 2 + f * _FC)
                ops = [v.astype(BF16) for v in _strassen_lhs(a11, a12, a21, a22)]
            if f > 0:
                rows = pl.ds((f - 1) * _FC // 2, _FC // 2)
                for k in range(7):
                    part = _mm(prev[k], pltpu.bitcast(_rhs_refs(wd, wds)[k][rows, :], BF16))
                    acc[k] = part if acc[k] is None else acc[k] + part
        assert not pieces
        c11, c12, c21, c22 = _strassen_out(acc)
        down = jnp.concatenate([jnp.concatenate([c11, c12], axis=1),
                                jnp.concatenate([c21, c22], axis=1)], axis=0)
        y = residual(i) + mod_row(5) * down
        ybuf[i % 2] = y.astype(ybuf.dtype).reshape(spb, seg, D)
        out_cp(i).start()
        return carry

    for r in range(0, R, _LR):
        ln2(0, 0, r)
    lax.fori_loop(0, n_blk, ffn, 0)
    for i in range(n_blk - 2, n_blk):
        out_cp(i).wait()


@functools.partial(jax.jit, static_argnames=("A_seg_len",))
def pallas_adaLN_cond__memory_aug_recurrent_mem_tr__glu_gated_swiglu__prompt_kernel(
        A_x, A_mem0, A_Wq, A_Wk, A_Wv, A_Wo, A_seg_len, B_x, B_w1, B_w3, B_w2, c, w_mod):
    del B_x
    B, S, D = A_x.shape
    _, H, Dh = A_Wq.shape
    M = A_mem0.shape[1]
    F = B_w1.shape[1]
    seg = int(A_seg_len)
    assert B == 1 and S % seg == 0 and S % _FM == 0 and F % (2 * _FC) == 0
    L = M + seg
    hbm = pl.BlockSpec(memory_space=pl.ANY)
    vmem = pl.BlockSpec(memory_space=pltpu.VMEM)
    dma = pltpu.SemaphoreType.DMA
    n_seg = S // seg
    out = pl.pallas_call(
        functools.partial(_body, H=H, Dh=Dh),
        out_shape=jax.ShapeDtypeStruct((n_seg, seg, D), A_x.dtype),
        in_specs=[hbm, vmem, hbm, hbm, hbm, hbm, hbm, hbm, hbm, vmem, hbm],
        out_specs=hbm,
        scratch_shapes=[
            pltpu.VMEM((n_seg, seg, D), BF16),
            pltpu.VMEM((n_seg, _TAIL, D), BF16),
            pltpu.VMEM((4 * D // _MC, D // 2, _MC), U32),
            pltpu.VMEM((H, D // 2, Dh), U32),
            pltpu.VMEM((H, D // 2, Dh), U32),
            pltpu.VMEM((H, D // 2, Dh), U32),
            pltpu.VMEM((H * Dh // 2, D), U32),
            pltpu.VMEM((4, D // 4, F + 128), U32),
            pltpu.VMEM((4, F // 4 + 32, D // 2), U32),
            pltpu.VMEM((5, D // 4, F + 128), U32),
            pltpu.VMEM((5, F // 4 + 32, D // 2), U32),
            pltpu.VMEM((8, 6 * D), F32),
            pltpu.VMEM((n_seg, seg, D), F32),
            pltpu.VMEM((7, n_seg * _TAIL // 2, D // 2), F32),
            pltpu.VMEM((3, H, n_seg * _TAIL // 2, Dh), U32),
            pltpu.VMEM((L, D), F32),
            pltpu.VMEM((L, H * Dh), F32),
            pltpu.VMEM((2, 7, _FM // 2, D // 2), F32),
            pltpu.VMEM((2, _FM // seg, seg, D), A_x.dtype),
            dma((3,)), dma((2 * D // _MC + 1,)), dma((H // 2,)), dma(()), dma(()), dma((2,)),
        ],
        compiler_params=pltpu.CompilerParams(vmem_limit_bytes=127 * 1024 * 1024, disable_bounds_checks=_NOBC),
    )(A_x.reshape(n_seg, seg, D), A_mem0.reshape(M, D), A_Wq.reshape(D // 2, 2 * H, Dh),
      A_Wk.reshape(D // 2, 2 * H, Dh), A_Wv.reshape(D // 2, 2 * H, Dh), A_Wo.reshape(H * Dh, D),
      B_w1, B_w3, B_w2, c, w_mod)
    return out.reshape(B, S, D)
```

```python
import functools

import jax
import jax.numpy as jnp
from jax import lax
import jax.experimental.pallas as pl
import jax.experimental.pallas.tpu as pltpu

_LOG2E = 1.4426950408889634
F32 = jnp.float32
BF16 = jnp.bfloat16
U32 = jnp.uint32

_LANES = 128
_TAIL = 8
_HG = 4
_LAG = 2
_AHEAD = 3
_MC = 512
_NA = 6
_PARTS = ((0, 1, 4), (2, 5), (3, 6))
_DT = 1
_LS = 3


def _mm(a, b):
    return lax.dot_general(a, b, (((1,), (0,)), ((), ())), preferred_element_type=F32)


def _mm_nt(a, b):
    return lax.dot_general(a, b, (((1,), (1,)), ((), ())), preferred_element_type=F32)


def _normalize(x):
    m = jnp.mean(x, axis=-1, keepdims=True)
    d = x - m
    v = jnp.mean(d * d, axis=-1, keepdims=True)
    return d * lax.rsqrt(v + 1e-5)


def _silu(x):
    half = 0.5 * x
    return half * jnp.tanh(half) + half


def _unpack(words):
    return (lax.bitcast_convert_type(words << 16, F32),
            lax.bitcast_convert_type(words & jnp.uint32(0xFFFF0000), F32))


def _pack(lo, hi):
    return pltpu.pack_elementwise([lo, hi], packed_dtype=BF16)


def _start(copies):
    for cp in copies:
        cp.start()


def _wait(copies):
    for cp in copies:
        cp.wait()


def _lhs7(a11, a12, a21, a22):
    return a11 + a22, a21 + a22, a11, a22, a11 + a12, a21 - a11, a12 - a22


def _rhs7(b11, b12, b21, b22):
    return b11 + b22, b11, b12 - b22, b21 - b11, b22, b11 + b12, b21 + b22


def _out4(p):
    return p[0] + p[3] - p[4] + p[6], p[2] + p[4], p[1] + p[3], p[0] - p[1] + p[2] + p[5]


def _nested(seven, blk):
    outer = [seven(blk[r][c], blk[r][2 + c], blk[2 + r][c], blk[2 + r][2 + c])
             for r in range(2) for c in range(2)]
    return [v for k in range(7) for v in seven(*(o[k] for o in outer))]


def _packed49(blk, part):
    lo, hi = (_nested(_rhs7, [[b[e] for b in row] for row in blk]) for e in range(2))
    return [(n, _pack(lo[n], hi[n])) for k in part for n in range(7 * k, 7 * k + 7)]


def _out16(product):
    inner = [_out4([product(7 * k + n) for n in range(7)]) for k in range(7)]
    outer = [_out4([v[e] for v in inner]) for e in range(4)]
    return [[outer[2 * (r % 2) + c % 2][2 * (r // 2) + c // 2] for c in range(4)]
            for r in range(4)]


def _body(x_hbm, mem0_ref, wq_hbm, wk_hbm, wv_hbm, wo_hbm, w1_hbm, w3_hbm, w2_hbm, c_ref,
          wmod_hbm, out_hbm,
          xs, wq, wk, wv, wo, mod, att, pre, hbuf,
          sem_x, sem_mod, sem_w, sem_o, sem_ring, sem_out):
    n_seg, seg, D = xs.shape
    H, _, Dh = wq.shape
    M = mem0_ref.shape[0]
    L = M + seg
    F = w1_hbm.shape[2]
    HP = H // 2
    T = _TAIL
    n_it = n_seg // 2
    wqkv = (wq, wk, wv)
    wmod_w = wmod_hbm.bitcast(U32)

    cv = c_ref[...].astype(F32)
    sc = jnp.broadcast_to(_silu(cv), (8, D))

    def mod_row(j):
        per = D // _LANES
        return jnp.concatenate([mod[j * per + n, 0:1, :] for n in range(per)], axis=1)

    def ln1(xv):
        return _normalize(xv.astype(F32)) * (1.0 + mod_row(1)) + mod_row(0)

    def arrival(xt, wmod, nt, ht):
        n_mod = wmod.shape[0]

        def mod_cp(j):
            return pltpu.make_async_copy(wmod_w.at[:, pl.ds(j * _MC, _MC)], wmod.at[j],
                                         sem_mod.at[j])

        def x_cp(i):
            blk = pl.ds(i * (n_seg // HP), n_seg // HP)
            return pltpu.make_async_copy(x_hbm.at[blk], xs.at[blk], sem_x.at[0])

        xt_cp = pltpu.make_async_copy(x_hbm.at[:, pl.ds(seg - T, T), :], xt, sem_x.at[1])

        def pair_cps(i):
            return [pltpu.make_async_copy(src.bitcast(U32).at[:, odd * HP + i, :],
                                          dst.at[2 * i + odd], sem_w.at[i])
                    for src, dst in zip((wq_hbm, wk_hbm, wv_hbm), wqkv) for odd in range(2)]

        def wo_cp(i):
            rows = pl.ds(pl.multiple_of(i * Dh, Dh), Dh)
            return pltpu.make_async_copy(wo_hbm.bitcast(U32).at[rows], wo.at[rows], sem_o)

        xt_cp.start()
        for j in range(n_mod):
            mod_cp(j).start()
        xt_cp.wait()
        _start(pair_cps(0))
        nt[...] = _normalize(xt[...].astype(F32).reshape(n_seg * T, D))
        for j in range(n_mod):
            mod_cp(j).wait()
            if j == n_mod - 1:
                _start(pair_cps(1))
            r = _mm(sc, pltpu.bitcast(wmod[j], BF16))
            for n in range(_MC // _LANES):
                mod[j * (_MC // _LANES) + n] = r[:, n * _LANES:(n + 1) * _LANES]
        hn = (nt[...] * (1.0 + mod_row(1)) + mod_row(0)).reshape(n_it, 2 * T, D)
        h_ev = hn[:, 0:T].reshape(n_it * T, D)
        h_od = hn[:, T:2 * T].reshape(n_it * T, D)
        for k, v in enumerate(_lhs7(h_ev[:, 0:D // 2], h_ev[:, D // 2:D],
                                    h_od[:, 0:D // 2], h_od[:, D // 2:D])):
            ht[k] = v
        for i in range(2, _AHEAD):
            _start(pair_cps(i))
        x_cp(0).start()
        wo_cp(0).start()

        def retile(w, i):
            a = w[2 * i]
            b = w[2 * i + 1]
            even = (a & jnp.uint32(0xFFFF)) | (b << 16)
            odd = (a >> 16) | (b & jnp.uint32(0xFFFF0000))
            w[2 * i] = even
            w[2 * i + 1] = odd
            halves = [_rhs7(*_unpack(v[0:D // 4]), *_unpack(v[D // 4:D // 2])) for v in (a, b)]
            rhs = [_pack(lo, hi) for lo, hi in zip(*halves)]
            rhs[1], rhs[4] = even[0:D // 4], odd[D // 4:D // 2]
            return rhs

        def arrive(i, carry):
            for m in range(3):
                rhs = retile(wqkv[m], i)
                c11, c12, c21, c22 = _out4(
                    {k: _mm(ht[k], pltpu.bitcast(rhs[k], BF16)) for k in (1, 4, 0, 2, 3, 5, 6)})
                if m == 2:
                    pl.when(i + _AHEAD < HP)(lambda: _start(pair_cps(i + _AHEAD)))

                    @pl.when(i + 1 < HP)
                    def _():
                        wo_cp(i + 1).start()
                        x_cp(i + 1).start()
                        _wait(pair_cps(i + 1))

                pre[m, 2 * i] = _pack(c11, c21)
                pre[m, 2 * i + 1] = _pack(c12, c22)
            return carry

        _wait(pair_cps(0))
        lax.fori_loop(0, HP, arrive, 0)
        for i in range(HP):
            x_cp(i).wait()
        for i in range(HP):
            wo_cp(i).wait()

    pl.run_scoped(arrival, pltpu.VMEM((n_seg, T, D), BF16),
                  pltpu.VMEM((2 * D // _MC, D // 2, _MC), U32),
                  pltpu.VMEM((n_seg * T, D), F32), pltpu.VMEM((7, n_it * T, D // 2), F32))

    NT = F // (4 * _LANES)
    mcols = 4 * D // n_it
    drows = 16
    n_dsl = NT * (_LANES // 2) // drows

    def recurrence(wu, wd, obuf, ring_u, ring_d, ring_m):
        def ring_cps(j):
            slot = j % 2
            rows = pl.ds(pl.multiple_of(j // 2 * 8, 8), 8)
            cols = pl.ds(pl.multiple_of(j % 2 * (F // 2), _LANES), F // 2)
            jd = jnp.minimum(j, n_dsl - 1)
            per = _LANES // 2 // drows
            cps = [(src.bitcast(U32).at[:, rows, cols], ring_u.at[slot, n])
                   for n, src in enumerate((w1_hbm, w3_hbm))]
            cps.append((w2_hbm.bitcast(U32).at[:, jd // per, :,
                                               pl.ds(pl.multiple_of(jd % per * drows, 8), drows)],
                        ring_d.at[slot]))
            cps.append((wmod_w.at[:, pl.ds(pl.multiple_of(2 * D + j * mcols, _LANES), mcols)],
                        ring_m.at[slot]))
            return [pltpu.make_async_copy(s, d, sem_ring.at[slot]) for s, d in cps]

        _start(ring_cps(0))
        hbuf[0:M] = mem0_ref[...].astype(F32)
        hbuf[M:L - T] = ln1(xs[0, 0:seg - T])

        def sums_up(j, t, part, anchor):
            ring_u[2, 0, 0, :, 0:_LANES] = lax.bitcast_convert_type(anchor, U32)
            blk = [[_unpack(ring_u[j % 2, n, kq, :, pl.ds((2 * t + par) * _LANES, _LANES)])
                    for n in range(2) for par in range(2)] for kq in range(4)]
            for n, v in _packed49(blk, part):
                wu[n, j % 2, pl.ds(pl.multiple_of(j // 2 * 8, 8), 8), pl.ds(t * _LANES, _LANES)] = v

        def sums_down(j, r, t, part, anchor):
            ring_d[2, 0, 0, 0:8, 0:_LANES] = lax.bitcast_convert_type(anchor, U32)
            blk = [[_unpack(ring_d[j % 2, kq // 2, kq % 2, pl.ds(r, 8),
                                   pl.ds(nq * (D // 4) + t * _LANES, _LANES)])
                    for nq in range(4)] for kq in range(4)]
            rows = pl.ds(pl.multiple_of(jnp.minimum(j, n_dsl - 1) * drows + r, 8), 8)
            for n, v in _packed49(blk, part):
                wd[n, rows, pl.ds(t * _LANES, _LANES)] = v

        def step(j, u, jobs):
            row = lax.broadcasted_iota(jnp.int32, (L, L), 0)
            col = lax.broadcasted_iota(jnp.int32, (L, L), 1)
            mask = (row < M) | (row >= col)
            h = hbuf[...]
            tail = pl.ds(pl.multiple_of(j * T, T), T)

            def proj(m, g):
                heads = range(g * _HG, (g + 1) * _HG)
                r = _mm(h, jnp.concatenate([pltpu.bitcast(wqkv[m][hd], BF16) for hd in heads],
                                           axis=1))
                return [jnp.concatenate([r[:, n * Dh:(n + 1) * Dh],
                                         _unpack(pre[m, hd, tail, :])[u]], axis=0)
                        for n, hd in enumerate(heads)]

            def probs(qs, ks):
                res = []
                for q, k in zip(qs, ks):
                    sco = jnp.where(mask, _mm_nt(q, k.astype(BF16)) * (Dh ** -0.5 * _LOG2E),
                                    -1e9 * _LOG2E)
                    e = jnp.exp2(sco - jnp.max(sco, axis=-1, keepdims=True))
                    den = jnp.sum(e, axis=-1, keepdims=True)
                    res.append((e, pl.reciprocal(den, full_range=False)))
                return res

            def mix(g, ps, vs):
                for n, ((e, inv), v) in enumerate(zip(ps, vs)):
                    obuf[:, pl.ds((g * _HG + n) * Dh, Dh)] = _mm(e, v.astype(BF16)) * inv

            def out_proj(g, acc):
                kk = _HG * Dh
                part = _mm(obuf[:, pl.ds(g * kk, kk)],
                           pltpu.bitcast(wo[pl.ds(g * kk // 2, kk // 2), :], BF16))
                mine = jobs[g::H // _HG]
                for n, job in enumerate(mine):
                    lane = n * _NA // len(mine) * _LANES
                    job(part[0:8, lane:lane + _LANES])
                return part if acc is None else acc + part

            NG = H // _HG
            acc = ps = vs = None
            for g in range(NG + 1):
                if g < NG:
                    ks, qs = proj(1, g), proj(0, g)
                if g > _LAG:
                    acc = out_proj(g - 1 - _LAG, acc)
                prev = ps, vs
                if g < NG:
                    vs = proj(2, g)
                    ps = probs(qs, ks)
                if g > 0:
                    mix(g - 1, *prev)
            for g in range(NG - _LAG, NG):
                acc = out_proj(g, acc)

            hbuf[M:L - T] = ln1(xs[jnp.minimum(2 * j + u + 1, n_seg - 1), 0:seg - T])
            hbuf[0:M] = acc[0:M]
            return acc[M:L]

        def steps(j, carry):
            _wait(ring_cps(j))
            pl.when(j + 1 < n_it)(lambda: _start(ring_cps(j + 1)))
            jobs = [functools.partial(sums_up, j, t, part) for t in range(NT) for part in _PARTS]
            jobs += [functools.partial(sums_down, j, r, t, part) for r in range(0, drows, 8)
                     for t in range(D // 4 // _LANES) for part in _PARTS]
            first = step(j, 0, jobs[0::2])
            mod[2 * D // _LANES + j] = _mm(sc, pltpu.bitcast(ring_m[j % 2], BF16))
            att[j] = _pack(first, step(j, 1, jobs[1::2]))
            return carry

        lax.fori_loop(0, n_it, steps, 0)

    def feed_forward(wu, wd, h2, ybuf):
        n_blk = n_seg // 4

        def out_cp(i):
            return pltpu.make_async_copy(ybuf.at[i % 2], out_hbm.at[pl.ds(i * 4, 4)],
                                         sem_out.at[i % 2])

        def residual(i, q, rows):
            a = _unpack(att[2 * i + q // 2, rows, :])[q % 2]
            return xs[4 * i + q, rows, :].astype(F32) + mod_row(2) * a

        def ln2(i, slot, r):
            hs = [_normalize(residual(i, q, pl.ds(r, 8))) * (1.0 + mod_row(4)) + mod_row(3)
                  for q in range(4)]
            blk = [[v[:, kq * (D // 4):(kq + 1) * (D // 4)] for kq in range(4)] for v in hs]
            for n, v in enumerate(_nested(_lhs7, blk)):
                h2[slot, n, pl.ds(r, 8), :] = v

        def ffn(i, carry):
            pl.when(i >= 2)(lambda: out_cp(i - 2).wait())
            pieces = list(range(0, seg, 8))

            def hidden(half, t):
                if (2 * t + half) % _LS == _LS - 1 and pieces:
                    ln2(jnp.minimum(i + 1, n_blk - 1), (i + 1) % 2, pieces.pop())
                c = _out16(lambda n: _mm(
                    h2[i % 2, n], pltpu.bitcast(wu[n, half, :, pl.ds(t * _LANES, _LANES)], BF16)))
                return [[_silu(c[q][par]) * c[q][2 + par] for par in range(2)] for q in range(4)]

            acc = [None] * 49
            ops = None
            for t0 in range(0, NT + _DT, _DT):
                prev = ops
                ts = range(t0, min(t0 + _DT, NT))
                if ts:
                    acts = [[hidden(half, t) for half in range(2)] for t in ts]
                    ops = _nested(_lhs7, [[jnp.concatenate([a[kq // 2][q][kq % 2] for a in acts],
                                                           axis=1)
                                           for kq in range(4)] for q in range(4)])
                if prev is not None:
                    rows = pl.ds((t0 - _DT) * _LANES // 2, prev[0].shape[1] // 2)
                    for n in range(49):
                        part = _mm(prev[n], pltpu.bitcast(wd[n, rows, :], BF16))
                        acc[n] = part if acc[n] is None else acc[n] + part
            assert not pieces
            down = _out16(lambda n: acc[n])
            for q in range(4):
                y = residual(i, q, slice(None)) + mod_row(5) * jnp.concatenate(down[q], axis=1)
                ybuf[i % 2, q] = y.astype(ybuf.dtype)
            out_cp(i).start()
            return carry

        for r in range(0, seg, 8):
            ln2(0, 0, r)
        lax.fori_loop(0, n_blk, ffn, 0)
        for i in range(n_blk - 2, n_blk):
            out_cp(i).wait()

    def main(wu, wd):
        pl.run_scoped(functools.partial(recurrence, wu, wd),
                      pltpu.VMEM((L, H * Dh), F32), pltpu.VMEM((3, 2, 4, 8, F // 2), U32),
                      pltpu.VMEM((3, 2, 2, drows, D), U32), pltpu.VMEM((2, D // 2, mcols), U32))
        pl.run_scoped(functools.partial(feed_forward, wu, wd),
                      pltpu.VMEM((2, 49, seg, D // 4), F32),
                      pltpu.VMEM((2, 4, seg, D), out_hbm.dtype))

    pl.run_scoped(main, pltpu.VMEM((49, 2, D // 8, F // 4), U32),
                  pltpu.VMEM((49, F // 8, D // 4), U32))


@functools.partial(jax.jit, static_argnames=("A_seg_len",))
def pallas_adaLN_cond__memory_aug_recurrent_mem_tr__glu_gated_swiglu__prompt_kernel(
        A_x, A_mem0, A_Wq, A_Wk, A_Wv, A_Wo, A_seg_len, B_x, B_w1, B_w3, B_w2, c, w_mod):
    del B_x
    B, S, D = A_x.shape
    _, H, Dh = A_Wq.shape
    M = A_mem0.shape[1]
    F = B_w1.shape[1]
    seg = int(A_seg_len)
    n_seg = S // seg
    assert (B, S, D, H, Dh, M, F, seg) == (1, 2048, 1024, 32, 128, 8, 3584, 32)
    hbm = pl.BlockSpec(memory_space=pl.ANY)
    vmem = pl.BlockSpec(memory_space=pltpu.VMEM)
    dma = pltpu.SemaphoreType.DMA
    out = pl.pallas_call(
        _body,
        out_shape=jax.ShapeDtypeStruct((n_seg, seg, D), A_x.dtype),
        in_specs=[hbm, vmem, hbm, hbm, hbm, hbm, hbm, hbm, hbm, vmem, hbm],
        out_specs=hbm,
        scratch_shapes=[
            pltpu.VMEM((n_seg, seg, D), BF16),
            pltpu.VMEM((H, D // 2, Dh), U32),
            pltpu.VMEM((H, D // 2, Dh), U32),
            pltpu.VMEM((H, D // 2, Dh), U32),
            pltpu.VMEM((H * Dh // 2, D), U32),
            pltpu.VMEM((6 * D // _LANES, 8, _LANES), F32),
            pltpu.VMEM((n_seg // 2, seg, D), U32),
            pltpu.VMEM((3, H, n_seg // 2 * _TAIL, Dh), U32),
            pltpu.VMEM((M + seg - _TAIL, D), F32),
            dma((2,)), dma((2 * D // _MC,)), dma((H // 2,)), dma(()), dma((2,)), dma((2,)),
        ],
        compiler_params=pltpu.CompilerParams(vmem_limit_bytes=127 * 1024 * 1024,
                                             disable_bounds_checks=True),
    )(A_x.reshape(n_seg, seg, D), A_mem0.reshape(M, D), A_Wq.reshape(D // 2, 2 * H, Dh),
      A_Wk.reshape(D // 2, 2 * H, Dh), A_Wv.reshape(D // 2, 2 * H, Dh), A_Wo.reshape(H * Dh, D),
      B_w1.reshape(4, D // 4, F), B_w3.reshape(4, D // 4, F),
      B_w2.reshape(2, F // (4 * _LANES), 2, _LANES, D), c, w_mod)
    return out.reshape(B, S, D)
```

```python
import functools

import jax
import jax.numpy as jnp
from jax import lax
import jax.experimental.pallas as pl
import jax.experimental.pallas.tpu as pltpu

_LOG2E = 1.4426950408889634
F32 = jnp.float32
BF16 = jnp.bfloat16
U32 = jnp.uint32

_LANES = 128
_TAIL = 8
_HG = 4
_LAG = 2
_AHEAD = 3
_MC = 512
_NA = 8
_INNER = 4
_PARTS = ((0, 1, 4), (2, 5), (3, 6))
_DT = 1
_LS = 3


def _mm(a, b):
    return lax.dot_general(a, b, (((1,), (0,)), ((), ())), preferred_element_type=F32)


def _mm_nt(a, b):
    return lax.dot_general(a, b, (((1,), (1,)), ((), ())), preferred_element_type=F32)


def _normalize(x):
    m = jnp.mean(x, axis=-1, keepdims=True)
    d = x - m
    v = jnp.mean(d * d, axis=-1, keepdims=True)
    return d * lax.rsqrt(v + 1e-5)


def _silu(x):
    half = 0.5 * x
    return half * jnp.tanh(half) + half


def _unpack(words):
    return (lax.bitcast_convert_type(words << 16, F32),
            lax.bitcast_convert_type(words & jnp.uint32(0xFFFF0000), F32))


def _pack(lo, hi):
    return pltpu.pack_elementwise([lo, hi], packed_dtype=BF16)


def _start(copies):
    for cp in copies:
        cp.start()


def _wait(copies):
    for cp in copies:
        cp.wait()


def _lhs7(a11, a12, a21, a22):
    return a11 + a22, a21 + a22, a11, a22, a11 + a12, a21 - a11, a12 - a22


def _rhs7(b11, b12, b21, b22):
    return b11 + b22, b11, b12 - b22, b21 - b11, b22, b11 + b12, b21 + b22


def _out4(p):
    return p[0] + p[3] - p[4] + p[6], p[2] + p[4], p[1] + p[3], p[0] - p[1] + p[2] + p[5]


def _nested(seven, blk):
    outer = [seven(blk[r][c], blk[r][2 + c], blk[2 + r][c], blk[2 + r][2 + c])
             for r in range(2) for c in range(2)]
    return [v for k in range(7) for v in seven(*(o[k] for o in outer))]


def _packed49(blk, part):
    lo, hi = (_nested(_rhs7, [[b[e] for b in row] for row in blk]) for e in range(2))
    return [(n, _pack(lo[n], hi[n])) for k in part for n in range(7 * k, 7 * k + 7)]


def _out16(product):
    inner = [_out4([product(7 * k + n) for n in range(7)]) for k in range(7)]
    outer = [_out4([v[e] for v in inner]) for e in range(4)]
    return [[outer[2 * (r % 2) + c % 2][2 * (r // 2) + c // 2] for c in range(4)]
            for r in range(4)]


def _body(x_hbm, mem0_ref, wq_hbm, wk_hbm, wv_hbm, wo_hbm, w1_hbm, w3_hbm, w2_hbm, c_ref,
          wmod_hbm, out_hbm,
          xs, wq, wk, wv, wo, mod, att, pre, hbuf, obuf, ring_u, ring_d, ring_m,
          sem_x, sem_mod, sem_w, sem_o, sem_ring, sem_out):
    n_seg, seg, D = xs.shape
    H, _, Dh = wq.shape
    M = mem0_ref.shape[0]
    L = M + seg
    F = w1_hbm.shape[2]
    HP = H // 2
    T = _TAIL
    n_it = n_seg // 2
    wqkv = (wq, wk, wv)
    wmod_w = wmod_hbm.bitcast(U32)

    cv = c_ref[...].astype(F32)
    sc = jnp.broadcast_to(_silu(cv), (8, D))

    def mod_row(j):
        per = D // _LANES
        return jnp.concatenate([mod[j * per + n, 0:1, :] for n in range(per)], axis=1)

    def ln1(xv):
        return _normalize(xv.astype(F32)) * (1.0 + mod_row(1)) + mod_row(0)

    NT = F // (4 * _LANES)
    n_out = n_it // _INNER
    urows = D // 8 // n_out
    drows = _LANES // 2 // _INNER

    def ring_cps(o):
        slot = o % 2
        rows = pl.ds(pl.multiple_of(o * urows, urows), urows)
        cps = [(src.bitcast(U32).at[:, rows], ring_u.at[pl.ds(slot * 8 + n * 4, 4)])
               for n, src in enumerate((w1_hbm, w3_hbm))]
        cps += [(w2_hbm.bitcast(U32).at[half * NT + jnp.minimum(o, NT - 1)],
                 ring_d.at[pl.ds(pl.multiple_of((slot * 2 + half) * _LANES, _LANES), _LANES)])
                for half in range(2)]
        mc = _INNER * _LANES
        cps.append((wmod_w.at[:, pl.ds(pl.multiple_of(2 * D + o * mc, mc), mc)],
                    ring_m.at[slot]))
        return [pltpu.make_async_copy(s, d, sem_ring.at[slot]) for s, d in cps]

    def arrival(xt, wmod, nt, ht):
        n_mod = wmod.shape[0]

        def mod_cp(j):
            return pltpu.make_async_copy(wmod_w.at[:, pl.ds(j * _MC, _MC)], wmod.at[j],
                                         sem_mod.at[j])

        def x_cp(i):
            blk = pl.ds(i * (n_seg // HP), n_seg // HP)
            return pltpu.make_async_copy(x_hbm.at[blk], xs.at[blk], sem_x.at[0])

        xt_cp = pltpu.make_async_copy(x_hbm.at[:, pl.ds(seg - T, T), :], xt, sem_x.at[1])

        def pair_cps(i):
            return [pltpu.make_async_copy(src.bitcast(U32).at[:, odd * HP + i, :],
                                          dst.at[2 * i + odd], sem_w.at[i])
                    for src, dst in zip((wq_hbm, wk_hbm, wv_hbm), wqkv) for odd in range(2)]

        def wo_cp(i):
            rows = pl.ds(pl.multiple_of(i * Dh, Dh), Dh)
            return pltpu.make_async_copy(wo_hbm.bitcast(U32).at[rows], wo.at[rows], sem_o)

        xt_cp.start()
        for j in range(n_mod):
            mod_cp(j).start()
        xt_cp.wait()
        _start(pair_cps(0))
        nt[...] = _normalize(xt[...].astype(F32).reshape(n_seg * T, D))
        for j in range(n_mod):
            mod_cp(j).wait()
            if j == n_mod - 1:
                _start(pair_cps(1))
            r = _mm(sc, pltpu.bitcast(wmod[j], BF16))
            for n in range(_MC // _LANES):
                mod[j * (_MC // _LANES) + n] = r[:, n * _LANES:(n + 1) * _LANES]
        hn = (nt[...] * (1.0 + mod_row(1)) + mod_row(0)).reshape(n_it, 2 * T, D)
        h_ev = hn[:, 0:T].reshape(n_it * T, D)
        h_od = hn[:, T:2 * T].reshape(n_it * T, D)
        for k, v in enumerate(_lhs7(h_ev[:, 0:D // 2], h_ev[:, D // 2:D],
                                    h_od[:, 0:D // 2], h_od[:, D // 2:D])):
            ht[k] = v
        for i in range(2, _AHEAD):
            _start(pair_cps(i))
        x_cp(0).start()
        wo_cp(0).start()

        def retile(w, i):
            a = w[2 * i]
            b = w[2 * i + 1]
            even = (a & jnp.uint32(0xFFFF)) | (b << 16)
            odd = (a >> 16) | (b & jnp.uint32(0xFFFF0000))
            w[2 * i] = even
            w[2 * i + 1] = odd
            halves = [_rhs7(*_unpack(v[0:D // 4]), *_unpack(v[D // 4:D // 2])) for v in (a, b)]
            rhs = [_pack(lo, hi) for lo, hi in zip(*halves)]
            rhs[1], rhs[4] = even[0:D // 4], odd[D // 4:D // 2]
            return rhs

        def arrive(i, carry):
            for m in range(3):
                rhs = retile(wqkv[m], i)
                c11, c12, c21, c22 = _out4(
                    {k: _mm(ht[k], pltpu.bitcast(rhs[k], BF16)) for k in (1, 4, 0, 2, 3, 5, 6)})
                if m == 2:
                    pl.when(i + _AHEAD < HP)(lambda: _start(pair_cps(i + _AHEAD)))
                    pl.when(i + _AHEAD == HP)(lambda: _start(ring_cps(0)))

                    @pl.when(i + 1 < HP)
                    def _():
                        wo_cp(i + 1).start()
                        x_cp(i + 1).start()
                        _wait(pair_cps(i + 1))

                pre[m, 2 * i] = _pack(c11, c21)
                pre[m, 2 * i + 1] = _pack(c12, c22)
            return carry

        _wait(pair_cps(0))
        lax.fori_loop(0, HP, arrive, 0)
        for i in range(HP):
            x_cp(i).wait()
        for i in range(HP):
            wo_cp(i).wait()

    pl.run_scoped(arrival, pltpu.VMEM((n_seg, T, D), BF16),
                  pltpu.VMEM((2 * D // _MC, D // 2, _MC), U32),
                  pltpu.VMEM((n_seg * T, D), F32), pltpu.VMEM((7, n_it * T, D // 2), F32))

    def recurrence(wu, wd):
        hbuf[0:M] = mem0_ref[...].astype(F32)
        hbuf[M:L - T] = ln1(xs[0, 0:seg - T])

        def weight_jobs(j):
            slot = j // _INNER % 2
            src_u = ring_u.at[pl.ds(slot * 8, 8), pl.ds(pl.multiple_of(j % _INNER // 2 * 8, 8), 8),
                              pl.ds(pl.multiple_of(j % 2 * (F // 2), _LANES), F // 2)]
            dst_u = wu.at[:, j % 2, pl.ds(pl.multiple_of(j // 2 * 8, 8), 8)]
            r0 = j % _INNER * drows
            src_d = ring_d.at[pl.ds(pl.multiple_of(slot * 2 * _LANES + r0, drows),
                                    3 * _LANES // 2 + drows)]
            tile = jnp.minimum(j // _INNER, NT - 1)
            dst_d = wd.at[:, pl.ds(pl.multiple_of(tile * (_LANES // 2) + r0, drows), drows)]

            def up(t, part, anchor):
                ring_u[16, 0:8, 0:_LANES] = lax.bitcast_convert_type(anchor, U32)
                blk = [[_unpack(src_u[n * 4 + kq, :, pl.ds((2 * t + par) * _LANES, _LANES)])
                        for n in range(2) for par in range(2)] for kq in range(4)]
                for n, v in _packed49(blk, part):
                    dst_u[n, :, pl.ds(t * _LANES, _LANES)] = v

            def down(r, t, part, anchor):
                ring_d[4 * _LANES:, 0:_LANES] = lax.bitcast_convert_type(anchor, U32)
                blk = [[_unpack(src_d[pl.ds(kq * (_LANES // 2) + r, 8),
                                      pl.ds(nq * (D // 4) + t * _LANES, _LANES)])
                        for nq in range(4)] for kq in range(4)]
                for n, v in _packed49(blk, part):
                    dst_d[n, pl.ds(r, 8), pl.ds(t * _LANES, _LANES)] = v

            return ([functools.partial(up, t, part) for t in range(NT) for part in _PARTS]
                    + [functools.partial(down, r, t, part) for r in range(0, drows, 8)
                       for t in range(D // 4 // _LANES) for part in _PARTS])

        def step(j, u, jobs):
            row = lax.broadcasted_iota(jnp.int32, (L, L), 0)
            col = lax.broadcasted_iota(jnp.int32, (L, L), 1)
            mask = (row < M) | (row >= col)
            h = hbuf[...]
            tail = pl.ds(pl.multiple_of(j * T, T), T)

            def proj(m, g):
                heads = range(g * _HG, (g + 1) * _HG)
                r = _mm(h, jnp.concatenate([pltpu.bitcast(wqkv[m][hd], BF16) for hd in heads],
                                           axis=1))
                return [jnp.concatenate([r[:, n * Dh:(n + 1) * Dh],
                                         _unpack(pre[m, hd, tail, :])[u]], axis=0)
                        for n, hd in enumerate(heads)]

            def probs(qs, ks):
                res = []
                for q, k in zip(qs, ks):
                    sco = jnp.where(mask, _mm_nt(q, k.astype(BF16)) * (Dh ** -0.5 * _LOG2E),
                                    -1e9 * _LOG2E)
                    e = jnp.exp2(sco - jnp.max(sco, axis=-1, keepdims=True))
                    den = jnp.sum(e, axis=-1, keepdims=True)
                    res.append((e, pl.reciprocal(den, full_range=False)))
                return res

            def mix(g, ps, vs):
                for n, ((e, inv), v) in enumerate(zip(ps, vs)):
                    obuf[:, pl.ds((g * _HG + n) * Dh, Dh)] = _mm(e, v.astype(BF16)) * inv

            def out_proj(g, acc):
                kk = _HG * Dh
                part = _mm(obuf[:, pl.ds(g * kk, kk)],
                           pltpu.bitcast(wo[pl.ds(g * kk // 2, kk // 2), :], BF16))
                mine = jobs[g::H // _HG]
                for n, job in enumerate(mine):
                    lane = n * _NA // len(mine) * _LANES
                    job(part[0:8, lane:lane + _LANES])
                return part if acc is None else acc + part

            NG = H // _HG
            acc = ps = vs = None
            for g in range(NG + 1):
                if g < NG:
                    ks, qs = proj(1, g), proj(0, g)
                if g > _LAG:
                    acc = out_proj(g - 1 - _LAG, acc)
                prev = ps, vs
                if g < NG:
                    vs = proj(2, g)
                    ps = probs(qs, ks)
                if g > 0:
                    mix(g - 1, *prev)
            for g in range(NG - _LAG, NG):
                acc = out_proj(g, acc)

            hbuf[M:L - T] = ln1(xs[jnp.minimum(2 * j + u + 1, n_seg - 1), 0:seg - T])
            hbuf[0:M] = acc[0:M]
            return acc[M:L]

        def steps(j, carry):
            jobs = weight_jobs(j)
            first = step(j, 0, jobs[0::2])
            mod[2 * D // _LANES + j] = _mm(sc, pltpu.bitcast(ring_m[
                j // _INNER % 2, :, pl.ds(pl.multiple_of(j % _INNER * _LANES, _LANES), _LANES)], BF16))
            att[j] = _pack(first, step(j, 1, jobs[1::2]))
            return carry

        def outer(o, carry):
            _wait(ring_cps(o))
            pl.when(o + 1 < n_out)(lambda: _start(ring_cps(o + 1)))
            return lax.fori_loop(o * _INNER, (o + 1) * _INNER, steps, carry)

        lax.fori_loop(0, n_out, outer, 0)

    def feed_forward(wu, wd):
        n_blk = n_seg // 4

        def out_cp(i):
            blk = pl.ds(i * 4, 4)
            return pltpu.make_async_copy(xs.at[blk], out_hbm.at[blk], sem_out)

        def residual(i, q, rows):
            a = _unpack(att[2 * i + q // 2, rows, :])[q % 2]
            return xs[4 * i + q, rows, :].astype(F32) + mod_row(2) * a

        def operands(slot):
            return wo.at[pl.ds(pl.multiple_of(slot * 13 * seg, seg), 13 * seg)]

        def place(n, r, size):
            return pl.ds(n // 4 * seg + r, size), pl.ds(n % 4 * (D // 4), D // 4)

        def ln2(i, dst, r):
            hs = [_normalize(residual(i, q, pl.ds(r, 8))) * (1.0 + mod_row(4)) + mod_row(3)
                  for q in range(4)]
            blk = [[v[:, kq * (D // 4):(kq + 1) * (D // 4)] for kq in range(4)] for v in hs]
            for n, v in enumerate(_nested(_lhs7, blk)):
                dst[place(n, r, 8)] = lax.bitcast_convert_type(v, U32)

        def ffn(i, carry):
            pieces = list(range(0, seg, 8))
            cur, nxt = operands(i % 2), operands((i + 1) % 2)

            def hidden(half, t):
                if (2 * t + half) % _LS == _LS - 1 and pieces:
                    ln2(jnp.minimum(i + 1, n_blk - 1), nxt, pieces.pop())
                c = _out16(lambda n: _mm(
                    lax.bitcast_convert_type(cur[place(n, 0, seg)], F32),
                    pltpu.bitcast(wu[n, half, :, pl.ds(t * _LANES, _LANES)], BF16)))
                return [[_silu(c[q][par]) * c[q][2 + par] for par in range(2)] for q in range(4)]

            acc = [None] * 49
            ops = None
            for t0 in range(0, NT + _DT, _DT):
                prev = ops
                ts = range(t0, min(t0 + _DT, NT))
                if ts:
                    acts = [[hidden(half, t) for half in range(2)] for t in ts]
                    ops = _nested(_lhs7, [[jnp.concatenate([a[kq // 2][q][kq % 2] for a in acts],
                                                           axis=1)
                                           for kq in range(4)] for q in range(4)])
                if prev is not None:
                    rows = pl.ds((t0 - _DT) * _LANES // 2, prev[0].shape[1] // 2)
                    for n in range(49):
                        part = _mm(prev[n], pltpu.bitcast(wd[n, rows, :], BF16))
                        acc[n] = part if acc[n] is None else acc[n] + part
            assert not pieces
            down = _out16(lambda n: acc[n])
            ys = [residual(i, q, slice(None)) + mod_row(5) * jnp.concatenate(down[q], axis=1)
                  for q in range(4)]
            for q in range(4):
                xs[4 * i + q] = ys[q].astype(xs.dtype)
            out_cp(i).start()
            return carry

        for r in range(0, seg, 8):
            ln2(0, operands(0), r)
        lax.fori_loop(0, n_blk, ffn, 0)
        for i in range(n_blk):
            out_cp(i).wait()

    def main(wu, wd):
        recurrence(wu, wd)
        feed_forward(wu, wd)

    pl.run_scoped(main, pltpu.VMEM((49, 2, D // 8, F // 4), U32),
                  pltpu.VMEM((49, F // 8, D // 4), U32))


@functools.partial(jax.jit, static_argnames=("A_seg_len",))
def pallas_adaLN_cond__memory_aug_recurrent_mem_tr__glu_gated_swiglu__prompt_kernel(
        A_x, A_mem0, A_Wq, A_Wk, A_Wv, A_Wo, A_seg_len, B_x, B_w1, B_w3, B_w2, c, w_mod):
    del B_x
    B, S, D = A_x.shape
    _, H, Dh = A_Wq.shape
    M = A_mem0.shape[1]
    F = B_w1.shape[1]
    seg = int(A_seg_len)
    n_seg = S // seg
    assert (B, S, D, H, Dh, M, F, seg) == (1, 2048, 1024, 32, 128, 8, 3584, 32)
    hbm = pl.BlockSpec(memory_space=pl.ANY)
    vmem = pl.BlockSpec(memory_space=pltpu.VMEM)
    dma = pltpu.SemaphoreType.DMA
    out = pl.pallas_call(
        _body,
        out_shape=jax.ShapeDtypeStruct((n_seg, seg, D), A_x.dtype),
        in_specs=[hbm, vmem, hbm, hbm, hbm, hbm, hbm, hbm, hbm, vmem, hbm],
        out_specs=hbm,
        scratch_shapes=[
            pltpu.VMEM((n_seg, seg, D), BF16),
            pltpu.VMEM((H, D // 2, Dh), U32),
            pltpu.VMEM((H, D // 2, Dh), U32),
            pltpu.VMEM((H, D // 2, Dh), U32),
            pltpu.VMEM((H * Dh // 2, D), U32),
            pltpu.VMEM((6 * D // _LANES, 8, _LANES), F32),
            pltpu.VMEM((n_seg // 2, seg, D), U32),
            pltpu.VMEM((3, H, n_seg // 2 * _TAIL, Dh), U32),
            pltpu.VMEM((M + seg - _TAIL, D), F32),
            pltpu.VMEM((M + seg, H * Dh), F32),
            pltpu.VMEM((17, D // 4 * _INNER // n_seg, F), U32),
            pltpu.VMEM((4 * _LANES + 8, D), U32),
            pltpu.VMEM((2, D // 2, _INNER * _LANES), U32),
            dma((2,)), dma((2 * D // _MC,)), dma((H // 2,)), dma(()), dma((2,)), dma(()),
        ],
        compiler_params=pltpu.CompilerParams(vmem_limit_bytes=128 * 1024 * 1024,
                                             disable_bounds_checks=True),
    )(A_x.reshape(n_seg, seg, D), A_mem0.reshape(M, D), A_Wq.reshape(D // 2, 2 * H, Dh),
      A_Wk.reshape(D // 2, 2 * H, Dh), A_Wv.reshape(D // 2, 2 * H, Dh), A_Wo.reshape(H * Dh, D),
      B_w1.reshape(4, D // 4, F), B_w3.reshape(4, D // 4, F),
      B_w2.reshape(F // (2 * _LANES), 2 * _LANES, D), c, w_mod)
    return out.reshape(B, S, D)
```

```python
import functools

import jax
import jax.numpy as jnp
from jax import lax
import jax.experimental.pallas as pl
import jax.experimental.pallas.tpu as pltpu

_LOG2E = 1.4426950408889634
F32 = jnp.float32
BF16 = jnp.bfloat16
U32 = jnp.uint32

_LANES = 128
_TAIL = 8
_HG = 4
_LAG = 2
_AHEAD = 3
_MC = 512
_NA = 8
_INNER = 4
_PARTS = ((0, 1, 4), (2, 5), (3, 6))
_DT = 4
_LR = 32
_LPOS = (8,)


def _mm(a, b):
    return lax.dot_general(a, b, (((1,), (0,)), ((), ())), preferred_element_type=F32)


def _mm_nt(a, b):
    return lax.dot_general(a, b, (((1,), (1,)), ((), ())), preferred_element_type=F32)


def _normalize(x):
    m = jnp.mean(x, axis=-1, keepdims=True)
    d = x - m
    v = jnp.mean(d * d, axis=-1, keepdims=True)
    return d * lax.rsqrt(v + 1e-5)


def _silu(x):
    half = 0.5 * x
    return half * jnp.tanh(half) + half


def _unpack(words):
    return (lax.bitcast_convert_type(words << 16, F32),
            lax.bitcast_convert_type(words & jnp.uint32(0xFFFF0000), F32))


def _pack(lo, hi):
    return pltpu.pack_elementwise([lo, hi], packed_dtype=BF16)


def _start(copies):
    for cp in copies:
        cp.start()


def _wait(copies):
    for cp in copies:
        cp.wait()


def _lhs7(a11, a12, a21, a22):
    return a11 + a22, a21 + a22, a11, a22, a11 + a12, a21 - a11, a12 - a22


def _rhs7(b11, b12, b21, b22):
    return b11 + b22, b11, b12 - b22, b21 - b11, b22, b11 + b12, b21 + b22


def _out4(p):
    return p[0] + p[3] - p[4] + p[6], p[2] + p[4], p[1] + p[3], p[0] - p[1] + p[2] + p[5]


def _nested(seven, blk):
    outer = [seven(blk[r][c], blk[r][2 + c], blk[2 + r][c], blk[2 + r][2 + c])
             for r in range(2) for c in range(2)]
    return [v for k in range(7) for v in seven(*(o[k] for o in outer))]


def _packed49(blk, part):
    lo, hi = (_nested(_rhs7, [[b[e] for b in row] for row in blk]) for e in range(2))
    return [(n, _pack(lo[n], hi[n])) for k in part for n in range(7 * k, 7 * k + 7)]


def _out16(product):
    inner = [_out4([product(7 * k + n) for n in range(7)]) for k in range(7)]
    outer = [_out4([v[e] for v in inner]) for e in range(4)]
    return [[outer[2 * (r % 2) + c % 2][2 * (r // 2) + c // 2] for c in range(4)]
            for r in range(4)]


def _body(x_hbm, mem0_ref, wq_hbm, wk_hbm, wv_hbm, wo_hbm, w1_hbm, w3_hbm, w2_hbm, c_ref,
          wmod_hbm, out_hbm,
          xs, wq, wk, wv, wo, mod, pre, hbuf, obuf, ring_u, ring_d, ring_m,
          sem_x, sem_mod, sem_w, sem_o, sem_ring, sem_out):
    n_seg, seg, D = xs.shape
    H, _, Dh = wq.shape
    M = mem0_ref.shape[0]
    L = M + seg
    F = w1_hbm.shape[2]
    HP = H // 2
    T = _TAIL
    n_it = n_seg // 2
    wqkv = (wq, wk, wv)
    wmod_w = wmod_hbm.bitcast(U32)

    cv = c_ref[...].astype(F32)
    sc = jnp.broadcast_to(_silu(cv), (8, D))

    def mod_row(j):
        per = D // _LANES
        return jnp.concatenate([mod[j * per + n, 0:1, :] for n in range(per)], axis=1)

    def attended(j):
        return pre.at[0, :, pl.ds(pl.multiple_of(j * T, T), T)]

    def ln1(xv):
        return _normalize(xv.astype(F32)) * (1.0 + mod_row(1)) + mod_row(0)

    NT = F // (4 * _LANES)
    n_out = n_it // _INNER
    urows = D // 8 // n_out
    drows = _LANES // 2 // _INNER

    def ring_cps(o):
        slot = o % 2
        rows = pl.ds(pl.multiple_of(o * urows, urows), urows)
        cps = [(src.bitcast(U32).at[:, rows], ring_u.at[pl.ds(slot * 8 + n * 4, 4)])
               for n, src in enumerate((w1_hbm, w3_hbm))]
        cps += [(w2_hbm.bitcast(U32).at[half * NT + jnp.minimum(o, NT - 1)],
                 ring_d.at[pl.ds(pl.multiple_of((slot * 2 + half) * _LANES, _LANES), _LANES)])
                for half in range(2)]
        mc = _INNER * _LANES
        cps.append((wmod_w.at[:, pl.ds(pl.multiple_of(2 * D + o * mc, mc), mc)],
                    ring_m.at[slot]))
        return [pltpu.make_async_copy(s, d, sem_ring.at[slot]) for s, d in cps]

    def arrival(xt, wmod, nt, ht):
        n_mod = wmod.shape[0]

        def mod_cp(j):
            return pltpu.make_async_copy(wmod_w.at[:, pl.ds(j * _MC, _MC)], wmod.at[j],
                                         sem_mod.at[j])

        def x_cp(i):
            blk = pl.ds(i * (n_seg // HP), n_seg // HP)
            return pltpu.make_async_copy(x_hbm.at[blk], xs.at[blk], sem_x.at[0])

        xt_cp = pltpu.make_async_copy(x_hbm.at[:, pl.ds(seg - T, T), :], xt, sem_x.at[1])

        def pair_cps(i):
            return [pltpu.make_async_copy(src.bitcast(U32).at[:, odd * HP + i, :],
                                          dst.at[2 * i + odd], sem_w.at[i])
                    for src, dst in zip((wq_hbm, wk_hbm, wv_hbm), wqkv) for odd in range(2)]

        def wo_cp(i):
            rows = pl.ds(pl.multiple_of(i * Dh, Dh), Dh)
            return pltpu.make_async_copy(wo_hbm.bitcast(U32).at[rows], wo.at[rows], sem_o)

        xt_cp.start()
        for j in range(n_mod):
            mod_cp(j).start()
        xt_cp.wait()
        _start(pair_cps(0))
        nt[...] = _normalize(xt[...].astype(F32).reshape(n_seg * T, D))
        for j in range(n_mod):
            mod_cp(j).wait()
            if j == n_mod - 1:
                _start(pair_cps(1))
            r = _mm(sc, pltpu.bitcast(wmod[j], BF16))
            for n in range(_MC // _LANES):
                mod[j * (_MC // _LANES) + n] = r[:, n * _LANES:(n + 1) * _LANES]
        hn = (nt[...] * (1.0 + mod_row(1)) + mod_row(0)).reshape(n_it, 2 * T, D)
        h_ev = hn[:, 0:T].reshape(n_it * T, D)
        h_od = hn[:, T:2 * T].reshape(n_it * T, D)
        for k, v in enumerate(_lhs7(h_ev[:, 0:D // 2], h_ev[:, D // 2:D],
                                    h_od[:, 0:D // 2], h_od[:, D // 2:D])):
            ht[k] = v
        for i in range(2, _AHEAD):
            _start(pair_cps(i))
        x_cp(0).start()
        wo_cp(0).start()

        def retile(w, i):
            a = w[2 * i]
            b = w[2 * i + 1]
            even = (a & jnp.uint32(0xFFFF)) | (b << 16)
            odd = (a >> 16) | (b & jnp.uint32(0xFFFF0000))
            w[2 * i] = even
            w[2 * i + 1] = odd
            halves = [_rhs7(*_unpack(v[0:D // 4]), *_unpack(v[D // 4:D // 2])) for v in (a, b)]
            rhs = [_pack(lo, hi) for lo, hi in zip(*halves)]
            rhs[1], rhs[4] = even[0:D // 4], odd[D // 4:D // 2]
            return rhs

        def arrive(i, carry):
            for m in range(3):
                rhs = retile(wqkv[m], i)
                c11, c12, c21, c22 = _out4(
                    {k: _mm(ht[k], pltpu.bitcast(rhs[k], BF16)) for k in (1, 4, 0, 2, 3, 5, 6)})
                if m == 2:
                    pl.when(i + _AHEAD < HP)(lambda: _start(pair_cps(i + _AHEAD)))
                    pl.when(i + _AHEAD == HP)(lambda: _start(ring_cps(0)))

                    @pl.when(i + 1 < HP)
                    def _():
                        wo_cp(i + 1).start()
                        x_cp(i + 1).start()
                        _wait(pair_cps(i + 1))

                pre[m, 2 * i] = _pack(c11, c21)
                pre[m, 2 * i + 1] = _pack(c12, c22)
            return carry

        _wait(pair_cps(0))
        lax.fori_loop(0, HP, arrive, 0)
        for i in range(HP):
            x_cp(i).wait()
        for i in range(HP):
            wo_cp(i).wait()

    pl.run_scoped(arrival, pltpu.VMEM((n_seg, T, D), BF16),
                  pltpu.VMEM((2 * D // _MC, D // 2, _MC), U32),
                  pltpu.VMEM((n_seg * T, D), F32), pltpu.VMEM((7, n_it * T, D // 2), F32))

    def recurrence(wu, wd):
        hbuf[0:M] = mem0_ref[...].astype(F32)
        hbuf[M:L - T] = ln1(xs[0, 0:seg - T])

        def weight_jobs(j):
            slot = j // _INNER % 2
            src_u = ring_u.at[pl.ds(slot * 8, 8), pl.ds(pl.multiple_of(j % _INNER // 2 * 8, 8), 8),
                              pl.ds(pl.multiple_of(j % 2 * (F // 2), _LANES), F // 2)]
            dst_u = wu.at[:, j % 2, pl.ds(pl.multiple_of(j // 2 * 8, 8), 8)]
            r0 = j % _INNER * drows
            src_d = ring_d.at[pl.ds(pl.multiple_of(slot * 2 * _LANES + r0, drows),
                                    3 * _LANES // 2 + drows)]
            tile = jnp.minimum(j // _INNER, NT - 1)
            dst_d = wd.at[:, pl.ds(pl.multiple_of(tile * (_LANES // 2) + r0, drows), drows)]

            def up(t, part, anchor):
                ring_u[16, 0:8, 0:_LANES] = lax.bitcast_convert_type(anchor, U32)
                blk = [[_unpack(src_u[n * 4 + kq, :, pl.ds((2 * t + par) * _LANES, _LANES)])
                        for n in range(2) for par in range(2)] for kq in range(4)]
                for n, v in _packed49(blk, part):
                    dst_u[n, :, pl.ds(t * _LANES, _LANES)] = v

            def down(r, t, part, anchor):
                ring_d[4 * _LANES:, 0:_LANES] = lax.bitcast_convert_type(anchor, U32)
                blk = [[_unpack(src_d[pl.ds(kq * (_LANES // 2) + r, 8),
                                      pl.ds(nq * (D // 4) + t * _LANES, _LANES)])
                        for nq in range(4)] for kq in range(4)]
                for n, v in _packed49(blk, part):
                    dst_d[n, pl.ds(r, 8), pl.ds(t * _LANES, _LANES)] = v

            return ([functools.partial(up, t, part) for t in range(NT) for part in _PARTS]
                    + [functools.partial(down, r, t, part) for r in range(0, drows, 8)
                       for t in range(D // 4 // _LANES) for part in _PARTS])

        def step(j, u, jobs):
            row = lax.broadcasted_iota(jnp.int32, (L, L), 0)
            col = lax.broadcasted_iota(jnp.int32, (L, L), 1)
            mask = (row < M) | (row >= col)
            h = hbuf[...]
            tail = pl.ds(pl.multiple_of(j * T, T), T)

            def proj(m, g):
                heads = range(g * _HG, (g + 1) * _HG)
                r = _mm(h, jnp.concatenate([pltpu.bitcast(wqkv[m][hd], BF16) for hd in heads],
                                           axis=1))
                return [jnp.concatenate([r[:, n * Dh:(n + 1) * Dh],
                                         _unpack(pre[m, hd, tail, :])[u]], axis=0)
                        for n, hd in enumerate(heads)]

            def probs(qs, ks):
                res = []
                for q, k in zip(qs, ks):
                    sco = jnp.where(mask, _mm_nt(q, k.astype(BF16)) * (Dh ** -0.5 * _LOG2E),
                                    -1e9 * _LOG2E)
                    e = jnp.exp2(sco - jnp.max(sco, axis=-1, keepdims=True))
                    den = jnp.sum(e, axis=-1, keepdims=True)
                    res.append((e, pl.reciprocal(den, full_range=False)))
                return res

            def mix(g, ps, vs):
                for n, ((e, inv), v) in enumerate(zip(ps, vs)):
                    obuf[:, pl.ds((g * _HG + n) * Dh, Dh)] = _mm(e, v.astype(BF16)) * inv

            def out_proj(g, acc):
                kk = _HG * Dh
                part = _mm(obuf[:, pl.ds(g * kk, kk)],
                           pltpu.bitcast(wo[pl.ds(g * kk // 2, kk // 2), :], BF16))
                mine = jobs[g::H // _HG]
                for n, job in enumerate(mine):
                    lane = n * _NA // len(mine) * _LANES
                    job(part[0:8, lane:lane + _LANES])
                return part if acc is None else acc + part

            NG = H // _HG
            acc = ps = vs = None
            for g in range(NG + 1):
                if g < NG:
                    ks, qs = proj(1, g), proj(0, g)
                if g > _LAG:
                    acc = out_proj(g - 1 - _LAG, acc)
                prev = ps, vs
                if g < NG:
                    vs = proj(2, g)
                    ps = probs(qs, ks)
                if g > 0:
                    mix(g - 1, *prev)
            for g in range(NG - _LAG, NG):
                acc = out_proj(g, acc)

            hbuf[M:L - T] = ln1(xs[jnp.minimum(2 * j + u + 1, n_seg - 1), 0:seg - T])
            hbuf[0:M] = acc[0:M]
            return acc[M:L]

        def steps(j, carry):
            jobs = weight_jobs(j)
            first = step(j, 0, jobs[0::2])
            mod[2 * D // _LANES + j] = _mm(sc, pltpu.bitcast(ring_m[
                j // _INNER % 2, :, pl.ds(pl.multiple_of(j % _INNER * _LANES, _LANES), _LANES)], BF16))
            both = _pack(first, step(j, 1, jobs[1::2]))
            dst = attended(j)
            for r in range(seg // T):
                for n in range(D // Dh):
                    dst[r * (D // Dh) + n] = both[r * T:(r + 1) * T, n * Dh:(n + 1) * Dh]
            return carry

        def outer(o, carry):
            _wait(ring_cps(o))
            pl.when(o + 1 < n_out)(lambda: _start(ring_cps(o + 1)))
            return lax.fori_loop(o * _INNER, (o + 1) * _INNER, steps, carry)

        lax.fori_loop(0, n_out, outer, 0)

    def feed_forward(wu, wd):
        n_blk = n_seg // 4

        def out_cp(i):
            blk = pl.ds(i * 4, 4)
            return pltpu.make_async_copy(xs.at[blk], out_hbm.at[blk], sem_out)

        def residual(i, q, r, size):
            src = attended(2 * i + q // 2)
            a = jnp.concatenate(
                [jnp.concatenate([_unpack(src[g * (D // Dh) + n])[q % 2] for n in range(D // Dh)],
                                 axis=1) for g in range(r // T, (r + size) // T)], axis=0)
            return xs[4 * i + q, pl.ds(r, size), :].astype(F32) + mod_row(2) * a

        def operands(slot):
            return wo.at[pl.ds(pl.multiple_of(slot * 13 * seg, seg), 13 * seg)]

        def place(n, r, size):
            return pl.ds(n // 4 * seg + r, size), pl.ds(n % 4 * (D // 4), D // 4)

        def ln2(i, dst, r):
            hs = [_normalize(residual(i, q, r, _LR)) * (1.0 + mod_row(4)) + mod_row(3)
                  for q in range(4)]
            blk = [[v[:, kq * (D // 4):(kq + 1) * (D // 4)] for kq in range(4)] for v in hs]
            for n, v in enumerate(_nested(_lhs7, blk)):
                dst[place(n, r, _LR)] = lax.bitcast_convert_type(v, U32)

        def ffn(i, carry):
            pieces = list(range(0, seg, _LR))
            cur, nxt = operands(i % 2), operands((i + 1) % 2)

            def hidden(half, t):
                if 2 * t + half in _LPOS:
                    ln2(jnp.minimum(i + 1, n_blk - 1), nxt, pieces.pop())
                c = _out16(lambda n: _mm(
                    lax.bitcast_convert_type(cur[place(n, 0, seg)], F32),
                    pltpu.bitcast(wu[n, half, :, pl.ds(t * _LANES, _LANES)], BF16)))
                return [[_silu(c[q][par]) * c[q][2 + par] for par in range(2)] for q in range(4)]

            acc = [None] * 49
            ops = None
            for t0 in range(0, NT + _DT, _DT):
                prev = ops
                ts = range(t0, min(t0 + _DT, NT))
                if ts:
                    acts = [[hidden(half, t) for half in range(2)] for t in ts]
                    ops = _nested(_lhs7, [[jnp.concatenate([a[kq // 2][q][kq % 2] for a in acts],
                                                           axis=1)
                                           for kq in range(4)] for q in range(4)])
                if prev is not None:
                    rows = pl.ds((t0 - _DT) * _LANES // 2, prev[0].shape[1] // 2)
                    for n in range(49):
                        part = _mm(prev[n], pltpu.bitcast(wd[n, rows, :], BF16))
                        acc[n] = part if acc[n] is None else acc[n] + part
            assert not pieces
            down = _out16(lambda n: acc[n])
            ys = [residual(i, q, 0, seg) + mod_row(5) * jnp.concatenate(down[q], axis=1)
                  for q in range(4)]
            for q in range(4):
                xs[4 * i + q] = ys[q].astype(xs.dtype)
            out_cp(i).start()
            return carry

        for r in range(0, seg, _LR):
            ln2(0, operands(0), r)
        lax.fori_loop(0, n_blk, ffn, 0)
        for i in range(n_blk):
            out_cp(i).wait()

    def main(wu, wd):
        recurrence(wu, wd)
        feed_forward(wu, wd)

    pl.run_scoped(main, pltpu.VMEM((49, 2, D // 8, F // 4), U32),
                  pltpu.VMEM((49, F // 8, D // 4), U32))


@functools.partial(jax.jit, static_argnames=("A_seg_len",))
def pallas_adaLN_cond__memory_aug_recurrent_mem_tr__glu_gated_swiglu__prompt_kernel(
        A_x, A_mem0, A_Wq, A_Wk, A_Wv, A_Wo, A_seg_len, B_x, B_w1, B_w3, B_w2, c, w_mod):
    del B_x
    B, S, D = A_x.shape
    _, H, Dh = A_Wq.shape
    M = A_mem0.shape[1]
    F = B_w1.shape[1]
    seg = int(A_seg_len)
    n_seg = S // seg
    assert (B, S, D, H, Dh, M, F, seg) == (1, 2048, 1024, 32, 128, 8, 3584, 32)
    hbm = pl.BlockSpec(memory_space=pl.ANY)
    vmem = pl.BlockSpec(memory_space=pltpu.VMEM)
    dma = pltpu.SemaphoreType.DMA
    out = pl.pallas_call(
        _body,
        out_shape=jax.ShapeDtypeStruct((n_seg, seg, D), A_x.dtype),
        in_specs=[hbm, vmem, hbm, hbm, hbm, hbm, hbm, hbm, hbm, vmem, hbm],
        out_specs=hbm,
        scratch_shapes=[
            pltpu.VMEM((n_seg, seg, D), BF16),
            pltpu.VMEM((H, D // 2, Dh), U32),
            pltpu.VMEM((H, D // 2, Dh), U32),
            pltpu.VMEM((H, D // 2, Dh), U32),
            pltpu.VMEM((H * Dh // 2, D), U32),
            pltpu.VMEM((6 * D // _LANES, 8, _LANES), F32),
            pltpu.VMEM((3, H, n_seg // 2 * _TAIL, Dh), U32),
            pltpu.VMEM((M + seg - _TAIL, D), F32),
            pltpu.VMEM((M + seg, H * Dh), F32),
            pltpu.VMEM((17, D // 4 * _INNER // n_seg, F), U32),
            pltpu.VMEM((4 * _LANES + 8, D), U32),
            pltpu.VMEM((2, D // 2, _INNER * _LANES), U32),
            dma((2,)), dma((2 * D // _MC,)), dma((H // 2,)), dma(()), dma((2,)), dma(()),
        ],
        compiler_params=pltpu.CompilerParams(vmem_limit_bytes=127 * 1024 * 1024,
                                             disable_bounds_checks=True),
    )(A_x.reshape(n_seg, seg, D), A_mem0.reshape(M, D), A_Wq.reshape(D // 2, 2 * H, Dh),
      A_Wk.reshape(D // 2, 2 * H, Dh), A_Wv.reshape(D // 2, 2 * H, Dh), A_Wo.reshape(H * Dh, D),
      B_w1.reshape(4, D // 4, F), B_w3.reshape(4, D // 4, F),
      B_w2.reshape(F // (2 * _LANES), 2 * _LANES, D), c, w_mod)
    return out.reshape(B, S, D)
```

```python
import functools

import jax
import jax.numpy as jnp
import numpy as np
from jax import lax
import jax.experimental.pallas as pl
import jax.experimental.pallas.tpu as pltpu

_LOG2E = 1.4426950408889634
F32 = jnp.float32
BF16 = jnp.bfloat16
U32 = jnp.uint32

_HI16 = np.uint32(0xFFFF0000)
_LO16 = np.uint32(0x0000FFFF)
_HALF = np.uint32(0x00008000)
_LANES = 128
_TAIL = 8
_HG = 4
_LAG = 2
_AHEAD = 3
_MC = 512
_NA = 6
_INNER = 4
_PARTS = tuple((k,) for k in range(7))
_DT = 4
_LR = 32
_LPOS = (8,)


def _mm(a, b):
    return lax.dot_general(a, b, (((1,), (0,)), ((), ())), preferred_element_type=F32)


def _mm_nt(a, b):
    return lax.dot_general(a, b, (((1,), (1,)), ((), ())), preferred_element_type=F32)


def _normalize(x):
    m = jnp.mean(x, axis=-1, keepdims=True)
    d = x - m
    v = jnp.mean(d * d, axis=-1, keepdims=True)
    return d * lax.rsqrt(v + 1e-5)


def _silu(x):
    half = 0.5 * x
    return half * jnp.tanh(half) + half


def _unpack(words):
    return (lax.bitcast_convert_type(words << 16, F32),
            lax.bitcast_convert_type(words & _HI16, F32))


def _pack(lo, hi):
    lo, hi = (lax.bitcast_convert_type(v, U32) + _HALF for v in (lo, hi))
    return (lo >> 16) | (hi & _HI16)


def _start(copies):
    for cp in copies:
        cp.start()


def _wait(copies):
    for cp in copies:
        cp.wait()


def _lhs7(a11, a12, a21, a22):
    return a11 + a22, a21 + a22, a11, a22, a11 + a12, a21 - a11, a12 - a22


def _rhs7(b11, b12, b21, b22):
    return b11 + b22, b11, b12 - b22, b21 - b11, b22, b11 + b12, b21 + b22


def _out4(p):
    return p[0] + p[3] - p[4] + p[6], p[2] + p[4], p[1] + p[3], p[0] - p[1] + p[2] + p[5]


def _nested(seven, blk):
    outer = [seven(blk[r][c], blk[r][2 + c], blk[2 + r][c], blk[2 + r][2 + c])
             for r in range(2) for c in range(2)]
    return [v for k in range(7) for v in seven(*(o[k] for o in outer))]


def _packed49(blk, part):
    lo, hi = (_nested(_rhs7, [[b[e] for b in row] for row in blk]) for e in range(2))
    return [(n, _pack(lo[n], hi[n])) for k in part for n in range(7 * k, 7 * k + 7)]


def _out16(product):
    inner = [_out4([product(7 * k + n) for n in range(7)]) for k in range(7)]
    outer = [_out4([v[e] for v in inner]) for e in range(4)]
    return [[outer[2 * (r % 2) + c % 2][2 * (r // 2) + c // 2] for c in range(4)]
            for r in range(4)]


def _body(x_hbm, mem0_ref, wq_hbm, wk_hbm, wv_hbm, wo_hbm, w1_hbm, w3_hbm, w2_hbm, c_ref,
          wmod_hbm, out_hbm,
          xs, wq, wk, wv, wo, mod, pre, hbuf, obuf, ring_u, ring_d, ring_m,
          sem_x, sem_mod, sem_w, sem_o, sem_ring, sem_out):
    n_seg, seg, D = xs.shape
    H, _, Dh = wq.shape
    M = mem0_ref.shape[0]
    L = M + seg
    F = w1_hbm.shape[2]
    HP = H // 2
    T = _TAIL
    n_it = n_seg // 2
    wqkv = (wq, wk, wv)
    wmod_w = wmod_hbm.bitcast(U32)

    cv = c_ref[...].astype(F32)
    sc = jnp.broadcast_to(_silu(cv), (8, D))

    def mod_row(j):
        per = D // _LANES
        return jnp.concatenate([mod[j * per + n, 0:1, :] for n in range(per)], axis=1)

    def attended(j):
        return pre.at[0, :, pl.ds(pl.multiple_of(j * T, T), T)]

    def ln1(xv):
        return _normalize(xv.astype(F32)) * (1.0 + mod_row(1)) + mod_row(0)

    NT = F // (4 * _LANES)
    n_out = n_it // _INNER
    urows = D // 8 // n_out
    drows = _LANES // 2 // _INNER

    def ring_cps(o):
        slot = o % 2
        rows = pl.ds(pl.multiple_of(o * urows, urows), urows)
        cps = [(src.bitcast(U32).at[:, rows], ring_u.at[pl.ds(slot * 8 + n * 4, 4)])
               for n, src in enumerate((w1_hbm, w3_hbm))]
        cps += [(w2_hbm.bitcast(U32).at[half * NT + jnp.minimum(o, NT - 1)],
                 ring_d.at[pl.ds(pl.multiple_of((slot * 2 + half) * _LANES, _LANES), _LANES)])
                for half in range(2)]
        mc = _INNER * _LANES
        cps.append((wmod_w.at[:, pl.ds(pl.multiple_of(2 * D + o * mc, mc), mc)],
                    ring_m.at[slot]))
        return [pltpu.make_async_copy(s, d, sem_ring.at[slot]) for s, d in cps]

    def arrival(xt, wmod, nt, ht):
        n_mod = wmod.shape[0]

        def mod_cp(j):
            return pltpu.make_async_copy(wmod_w.at[:, pl.ds(j * _MC, _MC)], wmod.at[j],
                                         sem_mod.at[j])

        def x_cp(i):
            blk = pl.ds(i * (n_seg // HP), n_seg // HP)
            return pltpu.make_async_copy(x_hbm.at[blk], xs.at[blk], sem_x.at[0])

        xt_cp = pltpu.make_async_copy(x_hbm.at[:, pl.ds(seg - T, T), :], xt, sem_x.at[1])

        def pair_cps(i):
            return [pltpu.make_async_copy(src.bitcast(U32).at[:, odd * HP + i, :],
                                          dst.at[2 * i + odd], sem_w.at[i])
                    for src, dst in zip((wq_hbm, wk_hbm, wv_hbm), wqkv) for odd in range(2)]

        def wo_cp(i):
            rows = pl.ds(pl.multiple_of(i * Dh, Dh), Dh)
            return pltpu.make_async_copy(wo_hbm.bitcast(U32).at[rows], wo.at[rows], sem_o)

        xt_cp.start()
        for j in range(n_mod):
            mod_cp(j).start()
        xt_cp.wait()
        _start(pair_cps(0))
        nt[...] = _normalize(xt[...].astype(F32).reshape(n_seg * T, D))
        for j in range(n_mod):
            mod_cp(j).wait()
            if j == n_mod - 1:
                _start(pair_cps(1))
            r = _mm(sc, pltpu.bitcast(wmod[j], BF16))
            for n in range(_MC // _LANES):
                mod[j * (_MC // _LANES) + n] = r[:, n * _LANES:(n + 1) * _LANES]
        hn = (nt[...] * (1.0 + mod_row(1)) + mod_row(0)).reshape(n_it, 2 * T, D)
        h_ev = hn[:, 0:T].reshape(n_it * T, D)
        h_od = hn[:, T:2 * T].reshape(n_it * T, D)
        for k, v in enumerate(_lhs7(h_ev[:, 0:D // 2], h_ev[:, D // 2:D],
                                    h_od[:, 0:D // 2], h_od[:, D // 2:D])):
            ht[k] = v
        for i in range(2, _AHEAD):
            _start(pair_cps(i))
        x_cp(0).start()
        wo_cp(0).start()

        def retile(w, i):
            a = w[2 * i]
            b = w[2 * i + 1]
            even = (a & _LO16) | (b << 16)
            odd = (a >> 16) | (b & _HI16)
            w[2 * i] = even
            w[2 * i + 1] = odd
            halves = [_rhs7(*_unpack(v[0:D // 4]), *_unpack(v[D // 4:D // 2])) for v in (a, b)]
            rhs = [_pack(lo, hi) for lo, hi in zip(*halves)]
            rhs[1], rhs[4] = even[0:D // 4], odd[D // 4:D // 2]
            return rhs

        def arrive(i, carry):
            for m in range(3):
                rhs = retile(wqkv[m], i)
                c11, c12, c21, c22 = _out4(
                    {k: _mm(ht[k], pltpu.bitcast(rhs[k], BF16)) for k in (1, 4, 0, 2, 3, 5, 6)})
                if m == 2:
                    pl.when(i + _AHEAD < HP)(lambda: _start(pair_cps(i + _AHEAD)))
                    pl.when(i + _AHEAD == HP)(lambda: _start(ring_cps(0)))

                    @pl.when(i + 1 < HP)
                    def _():
                        wo_cp(i + 1).start()
                        x_cp(i + 1).start()
                        _wait(pair_cps(i + 1))

                pre[m, 2 * i] = _pack(c11, c21)
                pre[m, 2 * i + 1] = _pack(c12, c22)
            return carry

        _wait(pair_cps(0))
        lax.fori_loop(0, HP, arrive, 0)
        for i in range(HP):
            x_cp(i).wait()
        for i in range(HP):
            wo_cp(i).wait()

    pl.run_scoped(arrival, pltpu.VMEM((n_seg, T, D), BF16),
                  pltpu.VMEM((2 * D // _MC, D // 2, _MC), U32),
                  pltpu.VMEM((n_seg * T, D), F32), pltpu.VMEM((7, n_it * T, D // 2), F32))

    def recurrence(wu, wd):
        hbuf[0:M] = mem0_ref[...].astype(F32)
        hbuf[M:L - T] = ln1(xs[0, 0:seg - T])

        def weight_jobs(j):
            slot = j // _INNER % 2
            src_u = ring_u.at[pl.ds(slot * 8, 8), pl.ds(pl.multiple_of(j % _INNER // 2 * 8, 8), 8),
                              pl.ds(pl.multiple_of(j % 2 * (F // 2), _LANES), F // 2)]
            dst_u = wu.at[:, j % 2, pl.ds(pl.multiple_of(j // 2 * 8, 8), 8)]
            r0 = j % _INNER * drows
            src_d = ring_d.at[pl.ds(pl.multiple_of(slot * 2 * _LANES + r0, drows),
                                    3 * _LANES // 2 + drows)]
            tile = jnp.minimum(j // _INNER, NT - 1)
            dst_d = wd.at[:, pl.ds(pl.multiple_of(tile * (_LANES // 2) + r0, drows), drows)]

            def up(t, part, anchor):
                ring_u[16, 0:8, 0:_LANES] = lax.bitcast_convert_type(anchor, U32)
                blk = [[_unpack(src_u[n * 4 + kq, :, pl.ds((2 * t + par) * _LANES, _LANES)])
                        for n in range(2) for par in range(2)] for kq in range(4)]
                for n, v in _packed49(blk, part):
                    dst_u[n, :, pl.ds(t * _LANES, _LANES)] = v

            def down(r, t, part, anchor):
                ring_d[4 * _LANES:, 0:_LANES] = lax.bitcast_convert_type(anchor, U32)
                blk = [[_unpack(src_d[pl.ds(kq * (_LANES // 2) + r, 8),
                                      pl.ds(nq * (D // 4) + t * _LANES, _LANES)])
                        for nq in range(4)] for kq in range(4)]
                for n, v in _packed49(blk, part):
                    dst_d[n, pl.ds(r, 8), pl.ds(t * _LANES, _LANES)] = v

            return ([functools.partial(up, t, part) for t in range(NT) for part in _PARTS]
                    + [functools.partial(down, r, t, part) for r in range(0, drows, 8)
                       for t in range(D // 4 // _LANES) for part in _PARTS])

        def step(j, u, jobs):
            row = lax.broadcasted_iota(jnp.int32, (L, L), 0)
            col = lax.broadcasted_iota(jnp.int32, (L, L), 1)
            mask = (row < M) | (row >= col)
            h = hbuf[...]
            tail = pl.ds(pl.multiple_of(j * T, T), T)

            def proj(m, g):
                heads = range(g * _HG, (g + 1) * _HG)
                r = _mm(h, jnp.concatenate([pltpu.bitcast(wqkv[m][hd], BF16) for hd in heads],
                                           axis=1))
                return [jnp.concatenate([r[:, n * Dh:(n + 1) * Dh],
                                         _unpack(pre[m, hd, tail, :])[u]], axis=0)
                        for n, hd in enumerate(heads)]

            def probs(qs, ks):
                res = []
                for q, k in zip(qs, ks):
                    sco = jnp.where(mask, _mm_nt(q, k.astype(BF16)) * (Dh ** -0.5 * _LOG2E),
                                    -1e9 * _LOG2E)
                    e = jnp.exp2(sco - jnp.max(sco, axis=-1, keepdims=True))
                    den = jnp.sum(e, axis=-1, keepdims=True)
                    res.append((e, pl.reciprocal(den, full_range=False)))
                return res

            def mix(g, ps, vs):
                for n, ((e, inv), v) in enumerate(zip(ps, vs)):
                    obuf[:, pl.ds((g * _HG + n) * Dh, Dh)] = _mm(e, v.astype(BF16)) * inv

            def out_proj(g, acc):
                kk = _HG * Dh
                part = _mm(obuf[:, pl.ds(g * kk, kk)],
                           pltpu.bitcast(wo[pl.ds(g * kk // 2, kk // 2), :], BF16))
                mine = jobs[g::H // _HG]
                for n, job in enumerate(mine):
                    lane = n * _NA // len(mine) * _LANES
                    job(part[0:8, lane:lane + _LANES])
                return part if acc is None else acc + part

            NG = H // _HG
            acc = ps = vs = None
            for g in range(NG + 1):
                if g < NG:
                    ks, qs = proj(1, g), proj(0, g)
                if g > _LAG:
                    acc = out_proj(g - 1 - _LAG, acc)
                prev = ps, vs
                if g < NG:
                    vs = proj(2, g)
                    ps = probs(qs, ks)
                if g > 0:
                    mix(g - 1, *prev)
            for g in range(NG - _LAG, NG):
                acc = out_proj(g, acc)

            hbuf[M:L - T] = ln1(xs[jnp.minimum(2 * j + u + 1, n_seg - 1), 0:seg - T])
            hbuf[0:M] = acc[0:M]
            return acc[M:L]

        def steps(j, carry):
            jobs = weight_jobs(j)
            first = step(j, 0, jobs[0::2])
            mod[2 * D // _LANES + j] = _mm(sc, pltpu.bitcast(ring_m[
                j // _INNER % 2, :, pl.ds(pl.multiple_of(j % _INNER * _LANES, _LANES), _LANES)], BF16))
            both = _pack(first, step(j, 1, jobs[1::2]))
            dst = attended(j)
            for r in range(seg // T):
                for n in range(D // Dh):
                    dst[r * (D // Dh) + n] = both[r * T:(r + 1) * T, n * Dh:(n + 1) * Dh]
            return carry

        def outer(o, carry):
            _wait(ring_cps(o))
            pl.when(o + 1 < n_out)(lambda: _start(ring_cps(o + 1)))
            return lax.fori_loop(o * _INNER, (o + 1) * _INNER, steps, carry)

        lax.fori_loop(0, n_out, outer, 0)

    def feed_forward(wu, wd):
        n_blk = n_seg // 4

        def out_cp(i):
            blk = pl.ds(i * 4, 4)
            return pltpu.make_async_copy(xs.at[blk], out_hbm.at[blk], sem_out)

        def residual(i, q, r, size):
            src = attended(2 * i + q // 2)
            a = jnp.concatenate(
                [jnp.concatenate([_unpack(src[g * (D // Dh) + n])[q % 2] for n in range(D // Dh)],
                                 axis=1) for g in range(r // T, (r + size) // T)], axis=0)
            return xs[4 * i + q, pl.ds(r, size), :].astype(F32) + mod_row(2) * a

        def operands(slot):
            return wo.at[pl.ds(pl.multiple_of(slot * 13 * seg, seg), 13 * seg)]

        def place(n, r, size):
            return pl.ds(n // 4 * seg + r, size), pl.ds(n % 4 * (D // 4), D // 4)

        def ln2(i, dst, r):
            hs = [_normalize(residual(i, q, r, _LR)) * (1.0 + mod_row(4)) + mod_row(3)
                  for q in range(4)]
            blk = [[v[:, kq * (D // 4):(kq + 1) * (D // 4)] for kq in range(4)] for v in hs]
            for n, v in enumerate(_nested(_lhs7, blk)):
                dst[place(n, r, _LR)] = lax.bitcast_convert_type(v, U32)

        def ffn(i, carry):
            pieces = list(range(0, seg, _LR))
            cur, nxt = operands(i % 2), operands((i + 1) % 2)

            def hidden(half, t):
                if 2 * t + half in _LPOS:
                    ln2(jnp.minimum(i + 1, n_blk - 1), nxt, pieces.pop())
                c = _out16(lambda n: _mm(
                    lax.bitcast_convert_type(cur[place(n, 0, seg)], F32),
                    pltpu.bitcast(wu[n, half, :, pl.ds(t * _LANES, _LANES)], BF16)))
                return [[_silu(c[q][par]) * c[q][2 + par] for par in range(2)] for q in range(4)]

            acc = [None] * 49
            ops = None
            for t0 in range(0, NT + _DT, _DT):
                prev = ops
                ts = range(t0, min(t0 + _DT, NT))
                if ts:
                    acts = [[hidden(half, t) for half in range(2)] for t in ts]
                    ops = _nested(_lhs7, [[jnp.concatenate([a[kq // 2][q][kq % 2] for a in acts],
                                                           axis=1)
                                           for kq in range(4)] for q in range(4)])
                if prev is not None:
                    rows = pl.ds((t0 - _DT) * _LANES // 2, prev[0].shape[1] // 2)
                    for n in range(49):
                        part = _mm(prev[n], pltpu.bitcast(wd[n, rows, :], BF16))
                        acc[n] = part if acc[n] is None else acc[n] + part
            assert not pieces
            down = _out16(lambda n: acc[n])
            ys = [residual(i, q, 0, seg) + mod_row(5) * jnp.concatenate(down[q], axis=1)
                  for q in range(4)]
            for q in range(4):
                xs[4 * i + q] = ys[q].astype(xs.dtype)
            out_cp(i).start()
            return carry

        for r in range(0, seg, _LR):
            ln2(0, operands(0), r)
        lax.fori_loop(0, n_blk, ffn, 0)
        for i in range(n_blk):
            out_cp(i).wait()

    def main(wu, wd):
        recurrence(wu, wd)
        feed_forward(wu, wd)

    pl.run_scoped(main, pltpu.VMEM((49, 2, D // 8, F // 4), U32),
                  pltpu.VMEM((49, F // 8, D // 4), U32))


@functools.partial(jax.jit, static_argnames=("A_seg_len",))
def pallas_adaLN_cond__memory_aug_recurrent_mem_tr__glu_gated_swiglu__prompt_kernel(
        A_x, A_mem0, A_Wq, A_Wk, A_Wv, A_Wo, A_seg_len, B_x, B_w1, B_w3, B_w2, c, w_mod):
    del B_x
    B, S, D = A_x.shape
    _, H, Dh = A_Wq.shape
    M = A_mem0.shape[1]
    F = B_w1.shape[1]
    seg = int(A_seg_len)
    n_seg = S // seg
    assert (B, S, D, H, Dh, M, F, seg) == (1, 2048, 1024, 32, 128, 8, 3584, 32)
    hbm = pl.BlockSpec(memory_space=pl.ANY)
    vmem = pl.BlockSpec(memory_space=pltpu.VMEM)
    dma = pltpu.SemaphoreType.DMA
    out = pl.pallas_call(
        _body,
        out_shape=jax.ShapeDtypeStruct((n_seg, seg, D), A_x.dtype),
        in_specs=[hbm, vmem, hbm, hbm, hbm, hbm, hbm, hbm, hbm, vmem, hbm],
        out_specs=hbm,
        scratch_shapes=[
            pltpu.VMEM((n_seg, seg, D), BF16),
            pltpu.VMEM((H, D // 2, Dh), U32),
            pltpu.VMEM((H, D // 2, Dh), U32),
            pltpu.VMEM((H, D // 2, Dh), U32),
            pltpu.VMEM((H * Dh // 2, D), U32),
            pltpu.VMEM((6 * D // _LANES, 8, _LANES), F32),
            pltpu.VMEM((3, H, n_seg // 2 * _TAIL, Dh), U32),
            pltpu.VMEM((M + seg - _TAIL, D), F32),
            pltpu.VMEM((M + seg, H * Dh), F32),
            pltpu.VMEM((17, D // 4 * _INNER // n_seg, F), U32),
            pltpu.VMEM((4 * _LANES + 8, D), U32),
            pltpu.VMEM((2, D // 2, _INNER * _LANES), U32),
            dma((2,)), dma((2 * D // _MC,)), dma((H // 2,)), dma(()), dma((2,)), dma(()),
        ],
        compiler_params=pltpu.CompilerParams(vmem_limit_bytes=127 * 1024 * 1024,
                                             disable_bounds_checks=True),
    )(A_x.reshape(n_seg, seg, D), A_mem0.reshape(M, D), A_Wq.reshape(D // 2, 2 * H, Dh),
      A_Wk.reshape(D // 2, 2 * H, Dh), A_Wv.reshape(D // 2, 2 * H, Dh), A_Wo.reshape(H * Dh, D),
      B_w1.reshape(4, D // 4, F), B_w3.reshape(4, D // 4, F),
      B_w2.reshape(F // (2 * _LANES), 2 * _LANES, D), c, w_mod)
    return out.reshape(B, S, D)
```

```python
import functools

import jax
import jax.numpy as jnp
import numpy as np
from jax import lax
import jax.experimental.pallas as pl
import jax.experimental.pallas.tpu as pltpu

_LOG2E = 1.4426950408889634
F32 = jnp.float32
BF16 = jnp.bfloat16
U32 = jnp.uint32

_HI16 = np.uint32(0xFFFF0000)
_LO16 = np.uint32(0x0000FFFF)
_HALF = np.uint32(0x00008000)
_LANES = 128
_TAIL = 8
_HG = 4
_LAG = 2
_AHEAD = 3
_MC = 512
_NA = 6
_INNER = 4
_PARTS = tuple((k,) for k in range(7))
_DT = 4
_LPOS = 4


def _mm(a, b):
    return lax.dot_general(a, b, (((1,), (0,)), ((), ())), preferred_element_type=F32)


def _mm_nt(a, b):
    return lax.dot_general(a, b, (((1,), (1,)), ((), ())), preferred_element_type=F32)


def _normalize(x):
    m = jnp.mean(x, axis=-1, keepdims=True)
    d = x - m
    v = jnp.mean(d * d, axis=-1, keepdims=True)
    return d * lax.rsqrt(v + 1e-5)


def _silu(x):
    half = 0.5 * x
    return half * jnp.tanh(half) + half


def _unpack(words):
    return (lax.bitcast_convert_type(words << 16, F32),
            lax.bitcast_convert_type(words & _HI16, F32))


def _pack(lo, hi):
    lo, hi = (lax.bitcast_convert_type(v, U32) + _HALF for v in (lo, hi))
    return (lo >> 16) | (hi & _HI16)


def _start(copies):
    for cp in copies:
        cp.start()


def _wait(copies):
    for cp in copies:
        cp.wait()


def _lhs7(a11, a12, a21, a22):
    return a11 + a22, a21 + a22, a11, a22, a11 + a12, a21 - a11, a12 - a22


def _rhs7(b11, b12, b21, b22):
    return b11 + b22, b11, b12 - b22, b21 - b11, b22, b11 + b12, b21 + b22


def _out4(p):
    return p[0] + p[3] - p[4] + p[6], p[2] + p[4], p[1] + p[3], p[0] - p[1] + p[2] + p[5]


def _nested(seven, blk):
    outer = [seven(blk[r][c], blk[r][2 + c], blk[2 + r][c], blk[2 + r][2 + c])
             for r in range(2) for c in range(2)]
    return [v for k in range(7) for v in seven(*(o[k] for o in outer))]


def _packed49(blk, part):
    lo, hi = (_nested(_rhs7, [[b[e] for b in row] for row in blk]) for e in range(2))
    return [(n, _pack(lo[n], hi[n])) for k in part for n in range(7 * k, 7 * k + 7)]


def _out16(product):
    inner = [_out4([product(7 * k + n) for n in range(7)]) for k in range(7)]
    outer = [_out4([v[e] for v in inner]) for e in range(4)]
    return [[outer[2 * (r % 2) + c % 2][2 * (r // 2) + c // 2] for c in range(4)]
            for r in range(4)]


def _body(x_hbm, mem0_ref, wq_hbm, wk_hbm, wv_hbm, wo_hbm, w1_hbm, w3_hbm, w2_hbm, c_ref,
          wmod_hbm, out_hbm,
          xs, wq, wk, wv, wo, mod, pre, hbuf, obuf, ring_u, ring_d, ring_m,
          sem_x, sem_mod, sem_w, sem_o, sem_ring, sem_out):
    n_seg, seg, D = xs.shape
    H, _, Dh = wq.shape
    M = mem0_ref.shape[0]
    L = M + seg
    F = w1_hbm.shape[2]
    HP = H // 2
    T = _TAIL
    n_it = n_seg // 2
    wqkv = (wq, wk, wv)
    wmod_w = wmod_hbm.bitcast(U32)

    cv = c_ref[...].astype(F32)
    sc = jnp.broadcast_to(_silu(cv), (8, D))

    def mod_row(j):
        per = D // _LANES
        return jnp.concatenate([mod[j * per + n, 0:1, :] for n in range(per)], axis=1)

    def attended(j):
        return pre.at[0, :, pl.ds(pl.multiple_of(j * T, T), T)]

    def ln1(xv):
        return _normalize(xv.astype(F32)) * (1.0 + mod_row(1)) + mod_row(0)

    NT = F // (4 * _LANES)
    n_out = n_it // _INNER
    urows = D // 8 // n_out
    drows = _LANES // 2 // _INNER

    def ring_cps(o):
        slot = o % 2
        rows = pl.ds(pl.multiple_of(o * urows, urows), urows)
        cps = [(src.bitcast(U32).at[:, rows], ring_u.at[pl.ds(slot * 8 + n * 4, 4)])
               for n, src in enumerate((w1_hbm, w3_hbm))]
        cps += [(w2_hbm.bitcast(U32).at[half * NT + jnp.minimum(o, NT - 1)],
                 ring_d.at[pl.ds(pl.multiple_of((slot * 2 + half) * _LANES, _LANES), _LANES)])
                for half in range(2)]
        mc = _INNER * _LANES
        cps.append((wmod_w.at[:, pl.ds(pl.multiple_of(2 * D + o * mc, mc), mc)],
                    ring_m.at[slot]))
        return [pltpu.make_async_copy(s, d, sem_ring.at[slot]) for s, d in cps]

    def arrival(xt, wmod, nt, ht):
        n_mod = wmod.shape[0]

        def mod_cp(j):
            return pltpu.make_async_copy(wmod_w.at[:, pl.ds(j * _MC, _MC)], wmod.at[j],
                                         sem_mod.at[j])

        def x_cp(i):
            blk = pl.ds(i * (n_seg // HP), n_seg // HP)
            return pltpu.make_async_copy(x_hbm.at[blk], xs.at[blk], sem_x.at[0])

        xt_cp = pltpu.make_async_copy(x_hbm.at[:, pl.ds(seg - T, T), :], xt, sem_x.at[1])

        def pair_cps(i):
            return [pltpu.make_async_copy(src.bitcast(U32).at[:, odd * HP + i, :],
                                          dst.at[2 * i + odd], sem_w.at[i])
                    for src, dst in zip((wq_hbm, wk_hbm, wv_hbm), wqkv) for odd in range(2)]

        def wo_cp(i):
            rows = pl.ds(pl.multiple_of(i * Dh, Dh), Dh)
            return pltpu.make_async_copy(wo_hbm.bitcast(U32).at[rows], wo.at[rows], sem_o)

        xt_cp.start()
        for j in range(n_mod):
            mod_cp(j).start()
        xt_cp.wait()
        _start(pair_cps(0))
        nt[...] = _normalize(xt[...].astype(F32).reshape(n_seg * T, D))
        for j in range(n_mod):
            mod_cp(j).wait()
            if j == n_mod - 1:
                _start(pair_cps(1))
            r = _mm(sc, pltpu.bitcast(wmod[j], BF16))
            for n in range(_MC // _LANES):
                mod[j * (_MC // _LANES) + n] = r[:, n * _LANES:(n + 1) * _LANES]
        hn = (nt[...] * (1.0 + mod_row(1)) + mod_row(0)).reshape(n_it, 2 * T, D)
        h_ev = hn[:, 0:T].reshape(n_it * T, D)
        h_od = hn[:, T:2 * T].reshape(n_it * T, D)
        for k, v in enumerate(_lhs7(h_ev[:, 0:D // 2], h_ev[:, D // 2:D],
                                    h_od[:, 0:D // 2], h_od[:, D // 2:D])):
            ht[k] = v
        for i in range(2, _AHEAD):
            _start(pair_cps(i))
        x_cp(0).start()
        wo_cp(0).start()

        def retile(w, i):
            a = w[2 * i]
            b = w[2 * i + 1]
            even = (a & _LO16) | (b << 16)
            odd = (a >> 16) | (b & _HI16)
            w[2 * i] = even
            w[2 * i + 1] = odd
            halves = [_rhs7(*_unpack(v[0:D // 4]), *_unpack(v[D // 4:D // 2])) for v in (a, b)]
            rhs = [_pack(lo, hi) for lo, hi in zip(*halves)]
            rhs[1], rhs[4] = even[0:D // 4], odd[D // 4:D // 2]
            return rhs

        def arrive(i, carry):
            for m in range(3):
                rhs = retile(wqkv[m], i)
                c11, c12, c21, c22 = _out4(
                    {k: _mm(ht[k], pltpu.bitcast(rhs[k], BF16)) for k in (1, 4, 0, 2, 3, 5, 6)})
                if m == 2:
                    pl.when(i + _AHEAD < HP)(lambda: _start(pair_cps(i + _AHEAD)))
                    pl.when(i + _AHEAD == HP)(lambda: _start(ring_cps(0)))

                    @pl.when(i + 1 < HP)
                    def _():
                        wo_cp(i + 1).start()
                        x_cp(i + 1).start()
                        _wait(pair_cps(i + 1))

                pre[m, 2 * i] = _pack(c11, c21)
                pre[m, 2 * i + 1] = _pack(c12, c22)
            return carry

        _wait(pair_cps(0))
        lax.fori_loop(0, HP, arrive, 0)
        for i in range(HP):
            x_cp(i).wait()
        for i in range(HP):
            wo_cp(i).wait()

    pl.run_scoped(arrival, pltpu.VMEM((n_seg, T, D), BF16),
                  pltpu.VMEM((2 * D // _MC, D // 2, _MC), U32),
                  pltpu.VMEM((n_seg * T, D), F32), pltpu.VMEM((7, n_it * T, D // 2), F32))

    def recurrence(wu, wd):
        hbuf[0:M] = mem0_ref[...].astype(F32)
        hbuf[M:L - T] = ln1(xs[0, 0:seg - T])

        def weight_jobs(j):
            slot = j // _INNER % 2
            src_u = ring_u.at[pl.ds(slot * 8, 8), pl.ds(pl.multiple_of(j % _INNER // 2 * 8, 8), 8),
                              pl.ds(pl.multiple_of(j % 2 * (F // 2), _LANES), F // 2)]
            dst_u = wu.at[:, j % 2, pl.ds(pl.multiple_of(j // 2 * 8, 8), 8)]
            r0 = j % _INNER * drows
            src_d = ring_d.at[pl.ds(pl.multiple_of(slot * 2 * _LANES + r0, drows),
                                    3 * _LANES // 2 + drows)]
            tile = jnp.minimum(j // _INNER, NT - 1)
            dst_d = wd.at[:, pl.ds(pl.multiple_of(tile * (_LANES // 2) + r0, drows), drows)]

            def up(t, part, anchor):
                ring_u[16, 0:8, 0:_LANES] = lax.bitcast_convert_type(anchor, U32)
                blk = [[_unpack(src_u[n * 4 + kq, :, pl.ds((2 * t + par) * _LANES, _LANES)])
                        for n in range(2) for par in range(2)] for kq in range(4)]
                for n, v in _packed49(blk, part):
                    dst_u[n, :, pl.ds(t * _LANES, _LANES)] = v

            def down(r, t, part, anchor):
                ring_d[4 * _LANES:, 0:_LANES] = lax.bitcast_convert_type(anchor, U32)
                blk = [[_unpack(src_d[pl.ds(kq * (_LANES // 2) + r, 8),
                                      pl.ds(nq * (D // 4) + t * _LANES, _LANES)])
                        for nq in range(4)] for kq in range(4)]
                for n, v in _packed49(blk, part):
                    dst_d[n, pl.ds(r, 8), pl.ds(t * _LANES, _LANES)] = v

            return ([functools.partial(up, t, part) for t in range(NT) for part in _PARTS]
                    + [functools.partial(down, r, t, part) for r in range(0, drows, 8)
                       for t in range(D // 4 // _LANES) for part in _PARTS])

        def step(j, u, jobs):
            row = lax.broadcasted_iota(jnp.int32, (L, L), 0)
            col = lax.broadcasted_iota(jnp.int32, (L, L), 1)
            mask = (row < M) | (row >= col)
            h = hbuf[...].astype(BF16)
            tail = pl.ds(pl.multiple_of(j * T, T), T)

            def proj(m, g):
                heads = range(g * _HG, (g + 1) * _HG)
                r = _mm(h, jnp.concatenate([pltpu.bitcast(wqkv[m][hd], BF16) for hd in heads],
                                           axis=1))
                return [jnp.concatenate([r[:, n * Dh:(n + 1) * Dh],
                                         _unpack(pre[m, hd, tail, :])[u]], axis=0)
                        for n, hd in enumerate(heads)]

            def probs(qs, ks):
                res = []
                for q, k in zip(qs, ks):
                    sco = jnp.where(mask, _mm_nt(q, k.astype(BF16)) * (Dh ** -0.5 * _LOG2E),
                                    -1e9 * _LOG2E)
                    e = jnp.exp2(sco - jnp.max(sco, axis=-1, keepdims=True))
                    den = jnp.sum(e, axis=-1, keepdims=True)
                    res.append((e, pl.reciprocal(den, full_range=False)))
                return res

            def mix(g, ps, vs):
                for n, ((e, inv), v) in enumerate(zip(ps, vs)):
                    obuf[:, pl.ds((g * _HG + n) * Dh, Dh)] = _mm(e, v.astype(BF16)) * inv

            def out_proj(g, acc):
                kk = _HG * Dh
                part = _mm(obuf[:, pl.ds(g * kk, kk)],
                           pltpu.bitcast(wo[pl.ds(g * kk // 2, kk // 2), :], BF16))
                mine = jobs[g::H // _HG]
                for n, job in enumerate(mine):
                    lane = n * _NA // len(mine) * _LANES
                    job(part[0:8, lane:lane + _LANES])
                return part if acc is None else acc + part

            NG = H // _HG
            acc = ps = vs = None
            for g in range(NG + 1):
                if g < NG:
                    ks, qs = proj(1, g), proj(0, g)
                if g > _LAG:
                    acc = out_proj(g - 1 - _LAG, acc)
                prev = ps, vs
                if g < NG:
                    vs = proj(2, g)
                    ps = probs(qs, ks)
                if g > 0:
                    mix(g - 1, *prev)
            for g in range(NG - _LAG, NG):
                acc = out_proj(g, acc)

            hbuf[M:L - T] = ln1(xs[jnp.minimum(2 * j + u + 1, n_seg - 1), 0:seg - T])
            hbuf[0:M] = acc[0:M]
            return acc[M:L]

        def steps(j, carry):
            jobs = weight_jobs(j)
            first = step(j, 0, jobs[0::2])
            mod[2 * D // _LANES + j] = _mm(sc, pltpu.bitcast(ring_m[
                j // _INNER % 2, :, pl.ds(pl.multiple_of(j % _INNER * _LANES, _LANES), _LANES)], BF16))
            both = _pack(first, step(j, 1, jobs[1::2]))
            dst = attended(j)
            for r in range(seg // T):
                for n in range(D // Dh):
                    dst[r * (D // Dh) + n] = both[r * T:(r + 1) * T, n * Dh:(n + 1) * Dh]
            return carry

        def outer(o, carry):
            _wait(ring_cps(o))
            pl.when(o + 1 < n_out)(lambda: _start(ring_cps(o + 1)))
            return lax.fori_loop(o * _INNER, (o + 1) * _INNER, steps, carry)

        lax.fori_loop(0, n_out, outer, 0)

    def feed_forward(wu, wd):
        n_blk = n_seg // 4

        def out_cp(i):
            blk = pl.ds(i * 4, 4)
            return pltpu.make_async_copy(xs.at[blk], out_hbm.at[blk], sem_out)

        def residual(i, q):
            src = attended(2 * i + q // 2)
            a = jnp.concatenate(
                [jnp.concatenate([_unpack(src[g * (D // Dh) + n])[q % 2] for n in range(D // Dh)],
                                 axis=1) for g in range(seg // T)], axis=0)
            return xs[4 * i + q].astype(F32) + mod_row(2) * a

        def operands(slot):
            return wo.at[pl.ds(pl.multiple_of(slot * 7 * seg, seg), 7 * seg)]

        def place(n):
            return pl.ds(n // 4 * (seg // 2), seg // 2), pl.ds(n % 4 * (D // 4), D // 4)

        def ln2(i, dst):
            hs = [_normalize(residual(i, q)) * (1.0 + mod_row(4)) + mod_row(3)
                  for q in range(4)]
            blk = [[v[:, kq * (D // 4):(kq + 1) * (D // 4)] for kq in range(4)] for v in hs]
            for n, v in enumerate(_nested(_lhs7, blk)):
                dst[place(n)] = pltpu.bitcast(v.astype(BF16), U32)

        def ffn(i, carry):
            cur, nxt = operands(i % 2), operands((i + 1) % 2)

            def hidden(half, t):
                if 2 * t + half == _LPOS:
                    ln2(jnp.minimum(i + 1, n_blk - 1), nxt)
                c = _out16(lambda n: _mm(
                    pltpu.bitcast(cur[place(n)], BF16),
                    pltpu.bitcast(wu[n, half, :, pl.ds(t * _LANES, _LANES)], BF16)))
                return [[_silu(c[q][par]) * c[q][2 + par] for par in range(2)] for q in range(4)]

            acc = [None] * 49
            ops = None
            for t0 in range(0, NT + _DT, _DT):
                prev = ops
                ts = range(t0, min(t0 + _DT, NT))
                if ts:
                    acts = [[hidden(half, t) for half in range(2)] for t in ts]
                    ops = _nested(_lhs7, [[jnp.concatenate([a[kq // 2][q][kq % 2] for a in acts],
                                                           axis=1)
                                           for kq in range(4)] for q in range(4)])
                if prev is not None:
                    rows = pl.ds((t0 - _DT) * _LANES // 2, prev[0].shape[1] // 2)
                    for n in range(49):
                        part = _mm(prev[n], pltpu.bitcast(wd[n, rows, :], BF16))
                        acc[n] = part if acc[n] is None else acc[n] + part
            down = _out16(lambda n: acc[n])
            ys = [residual(i, q) + mod_row(5) * jnp.concatenate(down[q], axis=1)
                  for q in range(4)]
            for q in range(4):
                xs[4 * i + q] = ys[q].astype(xs.dtype)
            out_cp(i).start()
            return carry

        ln2(0, operands(0))
        lax.fori_loop(0, n_blk, ffn, 0)
        for i in range(n_blk):
            out_cp(i).wait()

    def main(wu, wd):
        recurrence(wu, wd)
        feed_forward(wu, wd)

    pl.run_scoped(main, pltpu.VMEM((49, 2, D // 8, F // 4), U32),
                  pltpu.VMEM((49, F // 8, D // 4), U32))


@functools.partial(jax.jit, static_argnames=("A_seg_len",))
def pallas_adaLN_cond__memory_aug_recurrent_mem_tr__glu_gated_swiglu__prompt_kernel(
        A_x, A_mem0, A_Wq, A_Wk, A_Wv, A_Wo, A_seg_len, B_x, B_w1, B_w3, B_w2, c, w_mod):
    del B_x
    B, S, D = A_x.shape
    _, H, Dh = A_Wq.shape
    M = A_mem0.shape[1]
    F = B_w1.shape[1]
    seg = int(A_seg_len)
    n_seg = S // seg
    assert (B, S, D, H, Dh, M, F, seg) == (1, 2048, 1024, 32, 128, 8, 3584, 32)
    hbm = pl.BlockSpec(memory_space=pl.ANY)
    vmem = pl.BlockSpec(memory_space=pltpu.VMEM)
    dma = pltpu.SemaphoreType.DMA
    out = pl.pallas_call(
        _body,
        out_shape=jax.ShapeDtypeStruct((n_seg, seg, D), A_x.dtype),
        in_specs=[hbm, vmem, hbm, hbm, hbm, hbm, hbm, hbm, hbm, vmem, hbm],
        out_specs=hbm,
        scratch_shapes=[
            pltpu.VMEM((n_seg, seg, D), BF16),
            pltpu.VMEM((H, D // 2, Dh), U32),
            pltpu.VMEM((H, D // 2, Dh), U32),
            pltpu.VMEM((H, D // 2, Dh), U32),
            pltpu.VMEM((H * Dh // 2, D), U32),
            pltpu.VMEM((6 * D // _LANES, 8, _LANES), F32),
            pltpu.VMEM((3, H, n_seg // 2 * _TAIL, Dh), U32),
            pltpu.VMEM((M + seg - _TAIL, D), F32),
            pltpu.VMEM((M + seg, H * Dh), F32),
            pltpu.VMEM((17, D // 4 * _INNER // n_seg, F), U32),
            pltpu.VMEM((4 * _LANES + 8, D), U32),
            pltpu.VMEM((2, D // 2, _INNER * _LANES), U32),
            dma((2,)), dma((2 * D // _MC,)), dma((H // 2,)), dma(()), dma((2,)), dma(()),
        ],
        compiler_params=pltpu.CompilerParams(vmem_limit_bytes=127 * 1024 * 1024,
                                             disable_bounds_checks=True),
    )(A_x.reshape(n_seg, seg, D), A_mem0.reshape(M, D), A_Wq.reshape(D // 2, 2 * H, Dh),
      A_Wk.reshape(D // 2, 2 * H, Dh), A_Wv.reshape(D // 2, 2 * H, Dh), A_Wo.reshape(H * Dh, D),
      B_w1.reshape(4, D // 4, F), B_w3.reshape(4, D // 4, F),
      B_w2.reshape(F // (2 * _LANES), 2 * _LANES, D), c, w_mod)
    return out.reshape(B, S, D)
```

```python
import functools

import jax
import jax.numpy as jnp
import numpy as np
from jax import lax
import jax.experimental.pallas as pl
import jax.experimental.pallas.tpu as pltpu

_LOG2E = 1.4426950408889634
F32 = jnp.float32
BF16 = jnp.bfloat16
U32 = jnp.uint32

_HI16 = np.uint32(0xFFFF0000)
_LO16 = np.uint32(0x0000FFFF)
_HALF = np.uint32(0x00008000)
_LANES = 128
_TAIL = 8
_HG = 4
_LAG = 2
_AHEAD = 4
_MC = 512
_NA = 6
_INNER = 4
_DT = 4
_LPOS = 4


def _mm(a, b):
    return lax.dot_general(a, b, (((1,), (0,)), ((), ())), preferred_element_type=F32)


def _mm_nt(a, b):
    return lax.dot_general(a, b, (((1,), (1,)), ((), ())), preferred_element_type=F32)


def _normalize(x):
    m = jnp.mean(x, axis=-1, keepdims=True)
    d = x - m
    v = jnp.mean(d * d, axis=-1, keepdims=True)
    return d * lax.rsqrt(v + 1e-5)


def _silu(x):
    half = 0.5 * x
    return half * jnp.tanh(half) + half


def _unpack(words):
    return (lax.bitcast_convert_type(words << 16, F32),
            lax.bitcast_convert_type(words & _HI16, F32))


def _pack(lo, hi):
    lo, hi = (lax.bitcast_convert_type(v, U32) + _HALF for v in (lo, hi))
    return (lo >> 16) | (hi & _HI16)


def _start(copies):
    for cp in copies:
        cp.start()


def _wait(copies):
    for cp in copies:
        cp.wait()


def _lhs7(a11, a12, a21, a22):
    return a11 + a22, a21 + a22, a11, a22, a11 + a12, a21 - a11, a12 - a22


def _rhs7(b11, b12, b21, b22):
    return b11 + b22, b11, b12 - b22, b21 - b11, b22, b11 + b12, b21 + b22


def _out4(p):
    return p[0] + p[3] - p[4] + p[6], p[2] + p[4], p[1] + p[3], p[0] - p[1] + p[2] + p[5]


def _nested(seven, blk):
    outer = [seven(blk[r][c], blk[r][2 + c], blk[2 + r][c], blk[2 + r][2 + c])
             for r in range(2) for c in range(2)]
    return [v for k in range(7) for v in seven(*(o[k] for o in outer))]


def _packed49(blk, part):
    lo, hi = (_nested(_rhs7, [[b[e] for b in row] for row in blk]) for e in range(2))
    return [(n, _pack(lo[n], hi[n])) for n in range(7 * part, 7 * part + 7)]


def _out16(product):
    inner = [_out4([product(7 * k + n) for n in range(7)]) for k in range(7)]
    outer = [_out4([v[e] for v in inner]) for e in range(4)]
    return [[outer[2 * (r % 2) + c % 2][2 * (r // 2) + c // 2] for c in range(4)]
            for r in range(4)]


def _body(x_hbm, mem0_ref, wq_hbm, wk_hbm, wv_hbm, wo_hbm, w1_hbm, w3_hbm, w2_hbm, c_ref,
          wmod_hbm, out_hbm,
          xs, wq, wk, wv, wo, mod, pre, hbuf, obuf, ring_u, ring_d, ring_m,
          sem_x, sem_mod, sem_w, sem_o, sem_ring, sem_out):
    n_seg, seg, D = xs.shape
    H, _, Dh = wq.shape
    M = mem0_ref.shape[0]
    L = M + seg
    F = w1_hbm.shape[2]
    HP = H // 2
    T = _TAIL
    n_it = n_seg // 2
    wqkv = (wq, wk, wv)
    wmod_w = wmod_hbm.bitcast(U32)

    cv = c_ref[...].astype(F32)
    sc = jnp.broadcast_to(_silu(cv), (8, D))

    def mod_row(j):
        per = D // _LANES
        return jnp.concatenate([mod[j * per + n, 0:1, :] for n in range(per)], axis=1)

    def attended(j):
        return pre.at[0, :, pl.ds(pl.multiple_of(j * T, T), T)]

    def ln1(xv):
        return _normalize(xv.astype(F32)) * (1.0 + mod_row(1)) + mod_row(0)

    NT = F // (4 * _LANES)
    n_out = n_it // _INNER
    urows = D // 8 // n_out
    drows = _LANES // 2 // _INNER

    def x_cp(part):
        first = 4 * _INNER
        blk = pl.ds(first, n_seg - first) if part else pl.ds(0, first)
        return pltpu.make_async_copy(x_hbm.at[blk], xs.at[blk], sem_x.at[0])

    def ring_cps(o):
        slot = o % 2
        rows = pl.ds(pl.multiple_of(o * urows, urows), urows)
        cps = [(src.bitcast(U32).at[:, rows], ring_u.at[pl.ds(slot * 8 + n * 4, 4)])
               for n, src in enumerate((w1_hbm, w3_hbm))]
        cps += [(w2_hbm.bitcast(U32).at[half * NT + jnp.minimum(o, NT - 1)],
                 ring_d.at[pl.ds(pl.multiple_of((slot * 2 + half) * _LANES, _LANES), _LANES)])
                for half in range(2)]
        mc = _INNER * _LANES
        cps.append((wmod_w.at[:, pl.ds(pl.multiple_of(2 * D + o * mc, mc), mc)],
                    ring_m.at[slot]))
        return [pltpu.make_async_copy(s, d, sem_ring.at[slot]) for s, d in cps]

    def arrival(xt, wmod, nt, ht):
        n_mod = wmod.shape[0]

        def mod_cp(j):
            return pltpu.make_async_copy(wmod_w.at[:, pl.ds(j * _MC, _MC)], wmod.at[j],
                                         sem_mod.at[j])

        xt_cp = pltpu.make_async_copy(x_hbm.at[:, pl.ds(seg - T, T), :], xt, sem_x.at[1])

        def pair_cps(i):
            return [pltpu.make_async_copy(src.bitcast(U32).at[:, odd * HP + i, :],
                                          dst.at[2 * i + odd], sem_w.at[i])
                    for src, dst in zip((wq_hbm, wk_hbm, wv_hbm), wqkv) for odd in range(2)]

        def wo_cp(i):
            rows = pl.ds(pl.multiple_of(i * Dh, Dh), Dh)
            return pltpu.make_async_copy(wo_hbm.bitcast(U32).at[rows], wo.at[rows], sem_o)

        xt_cp.start()
        for j in range(n_mod):
            mod_cp(j).start()
        xt_cp.wait()
        _start(pair_cps(0))
        nt[...] = _normalize(xt[...].astype(F32).reshape(n_seg * T, D))
        for j in range(n_mod):
            mod_cp(j).wait()
            if j == n_mod - 1:
                _start(pair_cps(1))
            r = _mm(sc, pltpu.bitcast(wmod[j], BF16))
            for n in range(_MC // _LANES):
                mod[j * (_MC // _LANES) + n] = r[:, n * _LANES:(n + 1) * _LANES]
        hn = (nt[...] * (1.0 + mod_row(1)) + mod_row(0)).reshape(n_it, 2 * T, D)
        h_ev = hn[:, 0:T].reshape(n_it * T, D)
        h_od = hn[:, T:2 * T].reshape(n_it * T, D)
        for k, v in enumerate(_lhs7(h_ev[:, 0:D // 2], h_ev[:, D // 2:D],
                                    h_od[:, 0:D // 2], h_od[:, D // 2:D])):
            ht[k] = v
        for i in range(2, _AHEAD):
            _start(pair_cps(i))
        wo_cp(0).start()

        def retile(w, i):
            a = w[2 * i]
            b = w[2 * i + 1]
            even = (a & _LO16) | (b << 16)
            odd = (a >> 16) | (b & _HI16)
            w[2 * i] = even
            w[2 * i + 1] = odd
            halves = [_rhs7(*_unpack(v[0:D // 4]), *_unpack(v[D // 4:D // 2])) for v in (a, b)]
            rhs = [_pack(lo, hi) for lo, hi in zip(*halves)]
            rhs[1], rhs[4] = even[0:D // 4], odd[D // 4:D // 2]
            return rhs

        def arrive(i, carry):
            for m in range(3):
                rhs = retile(wqkv[m], i)
                c11, c12, c21, c22 = _out4(
                    {k: _mm(ht[k], pltpu.bitcast(rhs[k], BF16)) for k in (1, 4, 0, 2, 3, 5, 6)})
                if m == 2:
                    pl.when(i + _AHEAD < HP)(lambda: _start(pair_cps(i + _AHEAD)))
                    pl.when(i + _AHEAD == HP)(lambda: _start(ring_cps(0) + [x_cp(0)]))

                    @pl.when(i + 1 < HP)
                    def _():
                        wo_cp(i + 1).start()
                        _wait(pair_cps(i + 1))

                pre[m, 2 * i] = _pack(c11, c21)
                pre[m, 2 * i + 1] = _pack(c12, c22)
            return carry

        _wait(pair_cps(0))
        lax.fori_loop(0, HP, arrive, 0)
        x_cp(0).wait()
        for i in range(HP):
            wo_cp(i).wait()

    pl.run_scoped(arrival, pltpu.VMEM((n_seg, T, D), BF16),
                  pltpu.VMEM((2 * D // _MC, D // 2, _MC), U32),
                  pltpu.VMEM((n_seg * T, D), F32), pltpu.VMEM((7, n_it * T, D // 2), F32))

    def recurrence(wu, wd):
        x_cp(1).start()
        hbuf[0:M] = mem0_ref[...].astype(F32)
        hbuf[M:L - T] = ln1(xs[0, 0:seg - T])

        def weight_jobs(j):
            slot = j // _INNER % 2
            src_u = ring_u.at[pl.ds(slot * 8, 8), pl.ds(pl.multiple_of(j % _INNER // 2 * 8, 8), 8),
                              pl.ds(pl.multiple_of(j % 2 * (F // 2), _LANES), F // 2)]
            dst_u = wu.at[:, j % 2, pl.ds(pl.multiple_of(j // 2 * 8, 8), 8)]
            r0 = j % _INNER * drows
            src_d = ring_d.at[pl.ds(pl.multiple_of(slot * 2 * _LANES + r0, drows),
                                    3 * _LANES // 2 + drows)]
            tile = jnp.minimum(j // _INNER, NT - 1)
            dst_d = wd.at[:, pl.ds(pl.multiple_of(tile * (_LANES // 2) + r0, drows), drows)]

            def up(t, part, anchor):
                ring_u[16, 0:8, 0:_LANES] = lax.bitcast_convert_type(anchor, U32)
                blk = [[_unpack(src_u[n * 4 + kq, :, pl.ds((2 * t + par) * _LANES, _LANES)])
                        for n in range(2) for par in range(2)] for kq in range(4)]
                for n, v in _packed49(blk, part):
                    dst_u[n, :, pl.ds(t * _LANES, _LANES)] = v

            def down(r, t, part, anchor):
                ring_d[4 * _LANES:, 0:_LANES] = lax.bitcast_convert_type(anchor, U32)
                blk = [[_unpack(src_d[pl.ds(kq * (_LANES // 2) + r, 8),
                                      pl.ds(nq * (D // 4) + t * _LANES, _LANES)])
                        for nq in range(4)] for kq in range(4)]
                for n, v in _packed49(blk, part):
                    dst_d[n, pl.ds(r, 8), pl.ds(t * _LANES, _LANES)] = v

            return ([functools.partial(up, t, part) for t in range(NT) for part in range(7)]
                    + [functools.partial(down, r, t, part) for r in range(0, drows, 8)
                       for t in range(D // 4 // _LANES) for part in range(7)])

        def step(j, u, jobs):
            row = lax.broadcasted_iota(jnp.int32, (L, L), 0)
            col = lax.broadcasted_iota(jnp.int32, (L, L), 1)
            mask = (row < M) | (row >= col)
            h = hbuf[...].astype(BF16)
            tail = pl.ds(pl.multiple_of(j * T, T), T)

            def proj(m, g):
                heads = range(g * _HG, (g + 1) * _HG)
                r = _mm(h, jnp.concatenate([pltpu.bitcast(wqkv[m][hd], BF16) for hd in heads],
                                           axis=1))
                return [jnp.concatenate([r[:, n * Dh:(n + 1) * Dh],
                                         _unpack(pre[m, hd, tail, :])[u]], axis=0)
                        for n, hd in enumerate(heads)]

            def probs(qs, ks):
                res = []
                for q, k in zip(qs, ks):
                    sco = jnp.where(mask, _mm_nt(q, k.astype(BF16)) * (Dh ** -0.5 * _LOG2E),
                                    -1e9 * _LOG2E)
                    e = jnp.exp2(sco - jnp.max(sco, axis=-1, keepdims=True))
                    den = jnp.sum(e, axis=-1, keepdims=True)
                    res.append((e, pl.reciprocal(den, full_range=False)))
                return res

            def mix(g, ps, vs):
                for n, ((e, inv), v) in enumerate(zip(ps, vs)):
                    obuf[:, pl.ds((g * _HG + n) * Dh, Dh)] = _mm(e, v.astype(BF16)) * inv

            def out_proj(g, acc):
                kk = _HG * Dh
                part = _mm(obuf[:, pl.ds(g * kk, kk)],
                           pltpu.bitcast(wo[pl.ds(g * kk // 2, kk // 2), :], BF16))
                mine = jobs[g::H // _HG]
                for n, job in enumerate(mine):
                    lane = n * _NA // len(mine) * _LANES
                    job(part[0:8, lane:lane + _LANES])
                return part if acc is None else acc + part

            NG = H // _HG
            acc = ps = vs = None
            for g in range(NG + 1):
                if g < NG:
                    ks, qs = proj(1, g), proj(0, g)
                if g > _LAG:
                    acc = out_proj(g - 1 - _LAG, acc)
                prev = ps, vs
                if g < NG:
                    vs = proj(2, g)
                    ps = probs(qs, ks)
                if g > 0:
                    mix(g - 1, *prev)
            for g in range(NG - _LAG, NG):
                acc = out_proj(g, acc)

            hbuf[M:L - T] = ln1(xs[jnp.minimum(2 * j + u + 1, n_seg - 1), 0:seg - T])
            hbuf[0:M] = acc[0:M]
            return acc[M:L]

        def steps(j, carry):
            jobs = weight_jobs(j)
            first = step(j, 0, jobs[0::2])
            mod[2 * D // _LANES + j] = _mm(sc, pltpu.bitcast(ring_m[
                j // _INNER % 2, :, pl.ds(pl.multiple_of(j % _INNER * _LANES, _LANES), _LANES)], BF16))
            both = _pack(first, step(j, 1, jobs[1::2]))
            dst = attended(j)
            for r in range(seg // T):
                for n in range(D // Dh):
                    dst[r * (D // Dh) + n] = both[r * T:(r + 1) * T, n * Dh:(n + 1) * Dh]
            return carry

        def outer(o, carry):
            _wait(ring_cps(o))
            pl.when(o == 1)(x_cp(1).wait)
            pl.when(o + 1 < n_out)(lambda: _start(ring_cps(o + 1)))
            return lax.fori_loop(o * _INNER, (o + 1) * _INNER, steps, carry)

        lax.fori_loop(0, n_out, outer, 0)

    def feed_forward(wu, wd):
        n_blk = n_seg // 4

        def out_cp(i):
            blk = pl.ds(i * 4, 4)
            return pltpu.make_async_copy(xs.at[blk], out_hbm.at[blk], sem_out)

        def residual(i, q):
            src = attended(2 * i + q // 2)
            a = jnp.concatenate(
                [jnp.concatenate([_unpack(src[g * (D // Dh) + n])[q % 2] for n in range(D // Dh)],
                                 axis=1) for g in range(seg // T)], axis=0)
            return xs[4 * i + q].astype(F32) + mod_row(2) * a

        def operands(slot):
            return wo.at[pl.ds(pl.multiple_of(slot * 7 * seg, seg), 7 * seg)]

        def place(n):
            return pl.ds(n // 4 * (seg // 2), seg // 2), pl.ds(n % 4 * (D // 4), D // 4)

        def ln2(i, dst):
            hs = [_normalize(residual(i, q)) * (1.0 + mod_row(4)) + mod_row(3)
                  for q in range(4)]
            blk = [[v[:, kq * (D // 4):(kq + 1) * (D // 4)] for kq in range(4)] for v in hs]
            for n, v in enumerate(_nested(_lhs7, blk)):
                dst[place(n)] = pltpu.bitcast(v.astype(BF16), U32)

        def ffn(i, carry):
            cur, nxt = operands(i % 2), operands((i + 1) % 2)

            def hidden(half, t):
                if 2 * t + half == _LPOS:
                    ln2(jnp.minimum(i + 1, n_blk - 1), nxt)
                c = _out16(lambda n: _mm(
                    pltpu.bitcast(cur[place(n)], BF16),
                    pltpu.bitcast(wu[n, half, :, pl.ds(t * _LANES, _LANES)], BF16)))
                return [[_silu(c[q][par]) * c[q][2 + par] for par in range(2)] for q in range(4)]

            acc = [None] * 49
            ops = None
            for t0 in range(0, NT + _DT, _DT):
                prev = ops
                ts = range(t0, min(t0 + _DT, NT))
                if ts:
                    acts = [[hidden(half, t) for half in range(2)] for t in ts]
                    ops = _nested(_lhs7, [[jnp.concatenate([a[kq // 2][q][kq % 2] for a in acts],
                                                           axis=1)
                                           for kq in range(4)] for q in range(4)])
                if prev is not None:
                    rows = pl.ds((t0 - _DT) * _LANES // 2, prev[0].shape[1] // 2)
                    for n in range(49):
                        part = _mm(prev[n], pltpu.bitcast(wd[n, rows, :], BF16))
                        acc[n] = part if acc[n] is None else acc[n] + part
            down = _out16(lambda n: acc[n])
            ys = [residual(i, q) + mod_row(5) * jnp.concatenate(down[q], axis=1)
                  for q in range(4)]
            for q in range(4):
                xs[4 * i + q] = ys[q].astype(xs.dtype)
            out_cp(i).start()
            return carry

        ln2(0, operands(0))
        lax.fori_loop(0, n_blk, ffn, 0)
        for i in range(n_blk):
            out_cp(i).wait()

    def main(wu, wd):
        recurrence(wu, wd)
        feed_forward(wu, wd)

    pl.run_scoped(main, pltpu.VMEM((49, 2, D // 8, F // 4), U32),
                  pltpu.VMEM((49, F // 8, D // 4), U32))


@functools.partial(jax.jit, static_argnames=("A_seg_len",))
def pallas_adaLN_cond__memory_aug_recurrent_mem_tr__glu_gated_swiglu__prompt_kernel(
        A_x, A_mem0, A_Wq, A_Wk, A_Wv, A_Wo, A_seg_len, B_x, B_w1, B_w3, B_w2, c, w_mod):
    del B_x
    B, S, D = A_x.shape
    _, H, Dh = A_Wq.shape
    M = A_mem0.shape[1]
    F = B_w1.shape[1]
    seg = int(A_seg_len)
    n_seg = S // seg
    assert (B, S, D, H, Dh, M, F, seg) == (1, 2048, 1024, 32, 128, 8, 3584, 32)
    hbm = pl.BlockSpec(memory_space=pl.ANY)
    vmem = pl.BlockSpec(memory_space=pltpu.VMEM)
    dma = pltpu.SemaphoreType.DMA
    out = pl.pallas_call(
        _body,
        out_shape=jax.ShapeDtypeStruct((n_seg, seg, D), A_x.dtype),
        in_specs=[hbm, vmem, hbm, hbm, hbm, hbm, hbm, hbm, hbm, vmem, hbm],
        out_specs=hbm,
        scratch_shapes=[
            pltpu.VMEM((n_seg, seg, D), BF16),
            pltpu.VMEM((H, D // 2, Dh), U32),
            pltpu.VMEM((H, D // 2, Dh), U32),
            pltpu.VMEM((H, D // 2, Dh), U32),
            pltpu.VMEM((H * Dh // 2, D), U32),
            pltpu.VMEM((6 * D // _LANES, 8, _LANES), F32),
            pltpu.VMEM((3, H, n_seg // 2 * _TAIL, Dh), U32),
            pltpu.VMEM((M + seg - _TAIL, D), F32),
            pltpu.VMEM((M + seg, H * Dh), F32),
            pltpu.VMEM((17, D // 4 * _INNER // n_seg, F), U32),
            pltpu.VMEM((4 * _LANES + 8, D), U32),
            pltpu.VMEM((2, D // 2, _INNER * _LANES), U32),
            dma((2,)), dma((2 * D // _MC,)), dma((H // 2,)), dma(()), dma((2,)), dma(()),
        ],
        compiler_params=pltpu.CompilerParams(vmem_limit_bytes=127 * 1024 * 1024,
                                             disable_bounds_checks=True),
    )(A_x.reshape(n_seg, seg, D), A_mem0.reshape(M, D), A_Wq.reshape(D // 2, 2 * H, Dh),
      A_Wk.reshape(D // 2, 2 * H, Dh), A_Wv.reshape(D // 2, 2 * H, Dh), A_Wo.reshape(H * Dh, D),
      B_w1.reshape(4, D // 4, F), B_w3.reshape(4, D // 4, F),
      B_w2.reshape(F // (2 * _LANES), 2 * _LANES, D), c, w_mod)
    return out.reshape(B, S, D)
```

```python
import functools

import jax
import jax.numpy as jnp
import numpy as np
from jax import lax
import jax.experimental.pallas as pl
import jax.experimental.pallas.tpu as pltpu

_LOG2E = 1.4426950408889634
F32 = jnp.float32
BF16 = jnp.bfloat16
U32 = jnp.uint32

_HI16 = np.uint32(0xFFFF0000)
_LO16 = np.uint32(0x0000FFFF)
_HALF = np.uint32(0x00008000)
_LANES = 128
_TAIL = 8
_HG = 4
_LAG = 2
_AHEAD = 4
_MC = 512
_NA = 6
_INNER = 4
_DT = 3
_LPOS = 7


def _mm(a, b):
    return lax.dot_general(a, b, (((1,), (0,)), ((), ())), preferred_element_type=F32)


def _mm_nt(a, b):
    return lax.dot_general(a, b, (((1,), (1,)), ((), ())), preferred_element_type=F32)


def _normalize(x):
    m = jnp.mean(x, axis=-1, keepdims=True)
    d = x - m
    v = jnp.mean(d * d, axis=-1, keepdims=True)
    return d * lax.rsqrt(v + 1e-5)


def _silu(x):
    half = 0.5 * x
    return half * jnp.tanh(half) + half


def _unpack(words):
    return (lax.bitcast_convert_type(words << 16, F32),
            lax.bitcast_convert_type(words & _HI16, F32))


def _pack(lo, hi):
    lo, hi = (lax.bitcast_convert_type(v, U32) + _HALF for v in (lo, hi))
    return (lo >> 16) | (hi & _HI16)


def _start(copies):
    for cp in copies:
        cp.start()


def _wait(copies):
    for cp in copies:
        cp.wait()


def _lhs7(a11, a12, a21, a22):
    return a11 + a22, a21 + a22, a11, a22, a11 + a12, a21 - a11, a12 - a22


def _rhs7(b11, b12, b21, b22):
    return b11 + b22, b11, b12 - b22, b21 - b11, b22, b11 + b12, b21 + b22


def _out4(p):
    return p[0] + p[3] - p[4] + p[6], p[2] + p[4], p[1] + p[3], p[0] - p[1] + p[2] + p[5]


def _nested(seven, blk):
    outer = [seven(blk[r][c], blk[r][2 + c], blk[2 + r][c], blk[2 + r][2 + c])
             for r in range(2) for c in range(2)]
    return [v for k in range(7) for v in seven(*(o[k] for o in outer))]


def _packed49(blk, part):
    lo, hi = (_nested(_rhs7, [[b[e] for b in row] for row in blk]) for e in range(2))
    return [(n, _pack(lo[n], hi[n])) for n in range(7 * part, 7 * part + 7)]


def _out16(product):
    inner = [_out4([product(7 * k + n) for n in range(7)]) for k in range(7)]
    outer = [_out4([v[e] for v in inner]) for e in range(4)]
    return [[outer[2 * (r % 2) + c % 2][2 * (r // 2) + c // 2] for c in range(4)]
            for r in range(4)]


def _body(x_hbm, mem0_ref, wq_hbm, wk_hbm, wv_hbm, wo_hbm, w1_hbm, w3_hbm, w2_hbm, c_ref,
          wmod_hbm, out_hbm,
          xs, wq, wk, wv, wo, mod, pre, hbuf, obuf, ring_u, ring_d, ring_m,
          sem_x, sem_mod, sem_w, sem_o, sem_ring, sem_out):
    n_seg, seg, D = xs.shape
    H, _, Dh = wq.shape
    M = mem0_ref.shape[0]
    L = M + seg
    F = w1_hbm.shape[2]
    HP = H // 2
    T = _TAIL
    n_it = n_seg // 2
    wqkv = (wq, wk, wv)
    wmod_w = wmod_hbm.bitcast(U32)

    cv = c_ref[...].astype(F32)
    sc = jnp.broadcast_to(_silu(cv), (8, D))

    def mod_row(j):
        per = D // _LANES
        return jnp.concatenate([mod[j * per + n, 0:1, :] for n in range(per)], axis=1)

    def attended(j):
        return pre.at[0, :, pl.ds(pl.multiple_of(j * T, T), T)]

    def ln1(xv):
        return _normalize(xv.astype(F32)) * (1.0 + mod_row(1)) + mod_row(0)

    NT = F // (4 * _LANES)
    n_out = n_it // _INNER
    urows = D // 8 // n_out
    drows = _LANES // 2 // _INNER

    def x_cp(part):
        first = 4 * _INNER
        blk = pl.ds(first, n_seg - first) if part else pl.ds(0, first)
        return pltpu.make_async_copy(x_hbm.at[blk], xs.at[blk], sem_x.at[0])

    def ring_cps(o):
        slot = o % 2
        rows = pl.ds(pl.multiple_of(o * urows, urows), urows)
        cps = [(src.bitcast(U32).at[:, rows], ring_u.at[pl.ds(slot * 8 + n * 4, 4)])
               for n, src in enumerate((w1_hbm, w3_hbm))]
        cps += [(w2_hbm.bitcast(U32).at[half * NT + jnp.minimum(o, NT - 1)],
                 ring_d.at[pl.ds(pl.multiple_of((slot * 2 + half) * _LANES, _LANES), _LANES)])
                for half in range(2)]
        mc = _INNER * _LANES
        cps.append((wmod_w.at[:, pl.ds(pl.multiple_of(2 * D + o * mc, mc), mc)],
                    ring_m.at[slot]))
        return [pltpu.make_async_copy(s, d, sem_ring.at[slot]) for s, d in cps]

    def arrival(xt, wmod, nt, ht):
        n_mod = wmod.shape[0]

        def mod_cp(j):
            return pltpu.make_async_copy(wmod_w.at[:, pl.ds(j * _MC, _MC)], wmod.at[j],
                                         sem_mod.at[j])

        xt_cp = pltpu.make_async_copy(x_hbm.at[:, pl.ds(seg - T, T), :], xt, sem_x.at[1])

        def pair_cps(i):
            return [pltpu.make_async_copy(src.bitcast(U32).at[:, odd * HP + i, :],
                                          dst.at[2 * i + odd], sem_w.at[i])
                    for src, dst in zip((wq_hbm, wk_hbm, wv_hbm), wqkv) for odd in range(2)]

        def wo_cp(i):
            rows = pl.ds(pl.multiple_of(i * Dh, Dh), Dh)
            return pltpu.make_async_copy(wo_hbm.bitcast(U32).at[rows], wo.at[rows], sem_o)

        xt_cp.start()
        for j in range(n_mod):
            mod_cp(j).start()
        xt_cp.wait()
        _start(pair_cps(0))
        nt[...] = _normalize(xt[...].astype(F32).reshape(n_seg * T, D))
        for j in range(n_mod):
            mod_cp(j).wait()
            if j == n_mod - 1:
                _start(pair_cps(1))
            r = _mm(sc, pltpu.bitcast(wmod[j], BF16))
            for n in range(_MC // _LANES):
                mod[j * (_MC // _LANES) + n] = r[:, n * _LANES:(n + 1) * _LANES]
        hn = (nt[...] * (1.0 + mod_row(1)) + mod_row(0)).reshape(n_it, 2 * T, D)
        h_ev = hn[:, 0:T].reshape(n_it * T, D)
        h_od = hn[:, T:2 * T].reshape(n_it * T, D)
        for k, v in enumerate(_lhs7(h_ev[:, 0:D // 2], h_ev[:, D // 2:D],
                                    h_od[:, 0:D // 2], h_od[:, D // 2:D])):
            ht[k] = v
        for i in range(2, _AHEAD):
            _start(pair_cps(i))
        wo_cp(0).start()

        def retile(w, i):
            a = w[2 * i]
            b = w[2 * i + 1]
            even = (a & _LO16) | (b << 16)
            odd = (a >> 16) | (b & _HI16)
            w[2 * i] = even
            w[2 * i + 1] = odd
            halves = [_rhs7(*_unpack(v[0:D // 4]), *_unpack(v[D // 4:D // 2])) for v in (a, b)]
            rhs = [_pack(lo, hi) for lo, hi in zip(*halves)]
            rhs[1], rhs[4] = even[0:D // 4], odd[D // 4:D // 2]
            return rhs

        def arrive(i, carry):
            for m in range(3):
                rhs = retile(wqkv[m], i)
                c11, c12, c21, c22 = _out4(
                    {k: _mm(ht[k], pltpu.bitcast(rhs[k], BF16)) for k in (1, 4, 0, 2, 3, 5, 6)})
                if m == 2:
                    pl.when(i + _AHEAD < HP)(lambda: _start(pair_cps(i + _AHEAD)))
                    pl.when(i + _AHEAD == HP)(lambda: _start(ring_cps(0) + [x_cp(0)]))

                    @pl.when(i + 1 < HP)
                    def _():
                        wo_cp(i + 1).start()
                        _wait(pair_cps(i + 1))

                pre[m, 2 * i] = _pack(c11, c21)
                pre[m, 2 * i + 1] = _pack(c12, c22)
            return carry

        _wait(pair_cps(0))
        lax.fori_loop(0, HP, arrive, 0)
        x_cp(0).wait()
        for i in range(HP):
            wo_cp(i).wait()

    pl.run_scoped(arrival, pltpu.VMEM((n_seg, T, D), BF16),
                  pltpu.VMEM((2 * D // _MC, D // 2, _MC), U32),
                  pltpu.VMEM((n_seg * T, D), F32), pltpu.VMEM((7, n_it * T, D // 2), F32))

    def recurrence(wu, wd):
        x_cp(1).start()
        hbuf[0:M] = mem0_ref[...].astype(F32)
        hbuf[M:L - T] = ln1(xs[0, 0:seg - T])

        def weight_jobs(j):
            slot = j // _INNER % 2
            src_u = ring_u.at[pl.ds(slot * 8 + j % 2 * 4, 4),
                              pl.ds(pl.multiple_of(j % _INNER // 2 * 8, 8), 8)]
            dst_u = wu.at[:, j % 2, pl.ds(pl.multiple_of(j // 2 * 8, 8), 8)]
            r0 = j % _INNER * drows
            src_d = ring_d.at[pl.ds(pl.multiple_of(slot * 2 * _LANES + r0, drows),
                                    3 * _LANES // 2 + drows)]
            tile = jnp.minimum(j // _INNER, NT - 1)
            dst_d = wd.at[:, pl.ds(pl.multiple_of(tile * (_LANES // 2) + r0, drows), drows)]

            def up(t, part, anchor):
                ring_u[16, 0:8, 0:_LANES] = lax.bitcast_convert_type(anchor, U32)
                blk = [[_unpack(src_u[kq, :, pl.ds(half * (F // 2) + (2 * t + par) * _LANES,
                                                   _LANES)])
                        for half in range(2) for par in range(2)] for kq in range(4)]
                for n, v in _packed49(blk, part):
                    dst_u[n, :, pl.ds(t * _LANES, _LANES)] = v

            def down(r, t, part, anchor):
                ring_d[4 * _LANES:, 0:_LANES] = lax.bitcast_convert_type(anchor, U32)
                blk = [[_unpack(src_d[pl.ds(kq * (_LANES // 2) + r, 8),
                                      pl.ds(nq * (D // 4) + t * _LANES, _LANES)])
                        for nq in range(4)] for kq in range(4)]
                for n, v in _packed49(blk, part):
                    dst_d[n, pl.ds(r, 8), pl.ds(t * _LANES, _LANES)] = v

            return ([functools.partial(up, t, part) for t in range(NT) for part in range(7)]
                    + [functools.partial(down, r, t, part) for r in range(0, drows, 8)
                       for t in range(D // 4 // _LANES) for part in range(7)])

        def step(j, u, jobs):
            row = lax.broadcasted_iota(jnp.int32, (L, L), 0)
            col = lax.broadcasted_iota(jnp.int32, (L, L), 1)
            mask = (row < M) | (row >= col)
            h = hbuf[...].astype(BF16)
            tail = pl.ds(pl.multiple_of(j * T, T), T)

            def proj(m, g):
                heads = range(g * _HG, (g + 1) * _HG)
                r = _mm(h, jnp.concatenate([pltpu.bitcast(wqkv[m][hd], BF16) for hd in heads],
                                           axis=1))
                return [jnp.concatenate([r[:, n * Dh:(n + 1) * Dh],
                                         _unpack(pre[m, hd, tail, :])[u]], axis=0)
                        for n, hd in enumerate(heads)]

            def probs(qs, ks):
                res = []
                for q, k in zip(qs, ks):
                    sco = jnp.where(mask, _mm_nt(q, k.astype(BF16)) * (Dh ** -0.5 * _LOG2E),
                                    -1e9 * _LOG2E)
                    e = jnp.exp2(sco - jnp.max(sco, axis=-1, keepdims=True))
                    den = jnp.sum(e, axis=-1, keepdims=True)
                    res.append((e, pl.reciprocal(den, full_range=False)))
                return res

            def mix(g, ps, vs):
                for n, ((e, inv), v) in enumerate(zip(ps, vs)):
                    obuf[:, pl.ds((g * _HG + n) * Dh, Dh)] = _mm(e, v.astype(BF16)) * inv

            def out_proj(g, acc):
                kk = _HG * Dh
                part = _mm(obuf[:, pl.ds(g * kk, kk)],
                           pltpu.bitcast(wo[pl.ds(g * kk // 2, kk // 2), :], BF16))
                mine = jobs[g::H // _HG]
                for n, job in enumerate(mine):
                    lane = n * _NA // len(mine) * _LANES
                    job(part[0:8, lane:lane + _LANES])
                return part if acc is None else acc + part

            NG = H // _HG
            acc = ps = vs = None
            for g in range(NG + 1):
                if g < NG:
                    ks, qs = proj(1, g), proj(0, g)
                if g > _LAG:
                    acc = out_proj(g - 1 - _LAG, acc)
                prev = ps, vs
                if g < NG:
                    vs = proj(2, g)
                    ps = probs(qs, ks)
                if g > 0:
                    mix(g - 1, *prev)
            for g in range(NG - _LAG, NG):
                acc = out_proj(g, acc)

            hbuf[M:L - T] = ln1(xs[jnp.minimum(2 * j + u + 1, n_seg - 1), 0:seg - T])
            hbuf[0:M] = acc[0:M]
            return acc[M:L]

        def steps(j, carry):
            jobs = weight_jobs(j)
            first = step(j, 0, jobs[0::2])
            mod[2 * D // _LANES + j] = _mm(sc, pltpu.bitcast(ring_m[
                j // _INNER % 2, :, pl.ds(pl.multiple_of(j % _INNER * _LANES, _LANES), _LANES)], BF16))
            both = _pack(first, step(j, 1, jobs[1::2]))
            dst = attended(j)
            for r in range(seg // T):
                for n in range(D // Dh):
                    dst[r * (D // Dh) + n] = both[r * T:(r + 1) * T, n * Dh:(n + 1) * Dh]
            return carry

        def outer(o, carry):
            _wait(ring_cps(o))
            pl.when(o == 1)(x_cp(1).wait)
            pl.when(o + 1 < n_out)(lambda: _start(ring_cps(o + 1)))
            return lax.fori_loop(o * _INNER, (o + 1) * _INNER, steps, carry)

        lax.fori_loop(0, n_out, outer, 0)

    def feed_forward(wu, wd):
        n_blk = n_seg // 4

        def out_cp(i):
            blk = pl.ds(i * 4, 4)
            return pltpu.make_async_copy(xs.at[blk], out_hbm.at[blk], sem_out)

        def residual(i, q):
            src = attended(2 * i + q // 2)
            a = jnp.concatenate(
                [jnp.concatenate([_unpack(src[g * (D // Dh) + n])[q % 2] for n in range(D // Dh)],
                                 axis=1) for g in range(seg // T)], axis=0)
            return xs[4 * i + q].astype(F32) + mod_row(2) * a

        def operands(slot):
            return wo.at[pl.ds(pl.multiple_of(slot * 7 * seg, seg), 7 * seg)]

        def place(n):
            return pl.ds(n // 4 * (seg // 2), seg // 2), pl.ds(n % 4 * (D // 4), D // 4)

        def ln2(i, dst):
            hs = [_normalize(residual(i, q)) * (1.0 + mod_row(4)) + mod_row(3)
                  for q in range(4)]
            blk = [[v[:, kq * (D // 4):(kq + 1) * (D // 4)] for kq in range(4)] for v in hs]
            for n, v in enumerate(_nested(_lhs7, blk)):
                dst[place(n)] = pltpu.bitcast(v.astype(BF16), U32)

        def ffn(i, carry):
            cur, nxt = operands(i % 2), operands((i + 1) % 2)

            def project(mat, t):
                if 2 * t + mat == _LPOS:
                    ln2(jnp.minimum(i + 1, n_blk - 1), nxt)
                return _out16(lambda n: _mm(
                    pltpu.bitcast(cur[place(n)], BF16),
                    pltpu.bitcast(wu[n, mat, :, pl.ds(t * _LANES, _LANES)], BF16)))

            def hidden(t):
                gate = [[_silu(v) for v in row] for row in project(0, t)]
                return [[g * u for g, u in zip(*rows)] for rows in zip(gate, project(1, t))]

            acc = [None] * 49
            ops = None
            for t0 in range(0, NT + _DT, _DT):
                prev = ops
                ts = range(t0, min(t0 + _DT, NT))
                if ts:
                    acts = [hidden(t) for t in ts]
                    ops = _nested(_lhs7, [[jnp.concatenate([a[q][kq] for a in acts],
                                                           axis=1)
                                           for kq in range(4)] for q in range(4)])
                if prev is not None:
                    rows = pl.ds((t0 - _DT) * _LANES // 2, prev[0].shape[1] // 2)
                    for n in range(49):
                        part = _mm(prev[n], pltpu.bitcast(wd[n, rows, :], BF16))
                        acc[n] = part if acc[n] is None else acc[n] + part
            down = _out16(lambda n: acc[n])
            ys = [residual(i, q) + mod_row(5) * jnp.concatenate(down[q], axis=1)
                  for q in range(4)]
            for q in range(4):
                xs[4 * i + q] = ys[q].astype(xs.dtype)
            out_cp(i).start()
            return carry

        ln2(0, operands(0))
        lax.fori_loop(0, n_blk, ffn, 0)
        for i in range(n_blk):
            out_cp(i).wait()

    def main(wu, wd):
        recurrence(wu, wd)
        feed_forward(wu, wd)

    pl.run_scoped(main, pltpu.VMEM((49, 2, D // 8, F // 4), U32),
                  pltpu.VMEM((49, F // 8, D // 4), U32))


@functools.partial(jax.jit, static_argnames=("A_seg_len",))
def pallas_adaLN_cond__memory_aug_recurrent_mem_tr__glu_gated_swiglu__prompt_kernel(
        A_x, A_mem0, A_Wq, A_Wk, A_Wv, A_Wo, A_seg_len, B_x, B_w1, B_w3, B_w2, c, w_mod):
    del B_x
    B, S, D = A_x.shape
    _, H, Dh = A_Wq.shape
    M = A_mem0.shape[1]
    F = B_w1.shape[1]
    seg = int(A_seg_len)
    n_seg = S // seg
    assert (B, S, D, H, Dh, M, F, seg) == (1, 2048, 1024, 32, 128, 8, 3584, 32)
    hbm = pl.BlockSpec(memory_space=pl.ANY)
    vmem = pl.BlockSpec(memory_space=pltpu.VMEM)
    dma = pltpu.SemaphoreType.DMA
    out = pl.pallas_call(
        _body,
        out_shape=jax.ShapeDtypeStruct((n_seg, seg, D), A_x.dtype),
        in_specs=[hbm, vmem, hbm, hbm, hbm, hbm, hbm, hbm, hbm, vmem, hbm],
        out_specs=hbm,
        scratch_shapes=[
            pltpu.VMEM((n_seg, seg, D), BF16),
            pltpu.VMEM((H, D // 2, Dh), U32),
            pltpu.VMEM((H, D // 2, Dh), U32),
            pltpu.VMEM((H, D // 2, Dh), U32),
            pltpu.VMEM((H * Dh // 2, D), U32),
            pltpu.VMEM((6 * D // _LANES, 8, _LANES), F32),
            pltpu.VMEM((3, H, n_seg // 2 * _TAIL, Dh), U32),
            pltpu.VMEM((M + seg - _TAIL, D), F32),
            pltpu.VMEM((M + seg, H * Dh), F32),
            pltpu.VMEM((17, D // 4 * _INNER // n_seg, F), U32),
            pltpu.VMEM((4 * _LANES + 8, D), U32),
            pltpu.VMEM((2, D // 2, _INNER * _LANES), U32),
            dma((2,)), dma((2 * D // _MC,)), dma((H // 2,)), dma(()), dma((2,)), dma(()),
        ],
        compiler_params=pltpu.CompilerParams(vmem_limit_bytes=127 * 1024 * 1024,
                                             disable_bounds_checks=True),
    )(A_x.reshape(n_seg, seg, D), A_mem0.reshape(M, D), A_Wq.reshape(D // 2, 2 * H, Dh),
      A_Wk.reshape(D // 2, 2 * H, Dh), A_Wv.reshape(D // 2, 2 * H, Dh), A_Wo.reshape(H * Dh, D),
      B_w1.reshape(4, D // 4, F), B_w3.reshape(4, D // 4, F),
      B_w2.reshape(F // (2 * _LANES), 2 * _LANES, D), c, w_mod)
    return out.reshape(B, S, D)
```
